```python
import jax
import jax.numpy as jnp

def _softmax(x, axis=-1):
    return jax.nn.softmax(x, axis=axis)
def _gelu(x):
    return jax.nn.gelu(x, approximate=True)
def _silu(x):
    return jax.nn.silu(x)
def _sigmoid(x):
    return jax.nn.sigmoid(x)
def _layernorm(x, axis=-1, eps=1e-5):
    m = jnp.mean(x, axis=axis, keepdims=True)
    v = jnp.var(x, axis=axis, keepdims=True)
    return (x - m) / jnp.sqrt(v + eps)
def _scatter_add(tgt, idx, src, axis=0):
    return tgt.at[idx].add(src)
def _segment_sum(src, seg, n):
    return jax.ops.segment_sum(src, seg, n)
class _Rng:
    def __init__(self, key):
        self._k = key
    def _next(self):
        self._k, sub = jax.random.split(self._k)
        return sub
    def normal(self, shape):
        return jax.random.normal(self._next(), shape, dtype=jnp.bfloat16)
    def randint(self, lo, hi, shape):
        return jax.random.randint(self._next(), shape, lo, hi, dtype=jnp.int32)
    def uniform(self, shape, lo=0.0, hi=1.0):
        return jax.random.uniform(self._next(), shape, jnp.bfloat16, lo, hi)
    def permutation(self, n):
        return jax.random.permutation(self._next(), n)


kernel_name = 'interleave_layers__linear_attn_block__mixer_channel_mlp__prompt'

def _fwd_setup_inputs():
    _rng = _Rng(jax.random.key(int.from_bytes(__import__("os").urandom(4), "little")))
    _w = (lambda a: (lambda t: t.astype(jnp.bfloat16) if jnp.issubdtype(t.dtype, jnp.floating) else t)(jnp.asarray(a)))
    def _A_setup():
        B, S, D = 1, 2048, 576
        return {
            "x": _w((lambda *s: _rng.normal(s) * 0.05)(B, S, D)),
            "wqkv": _w((lambda *s: _rng.normal(s) * 0.05)(D, 3 * D)),
            "wo": _w((lambda *s: _rng.normal(s) * 0.05)(D, D)),
        }
    _A_in = _A_setup()

    def _B_setup():
        B, S, D, F = 1, 2048, 576, 4608
        return {
            "x": _w((lambda *s: _rng.normal(s) * 0.05)(B, S, D)),
            "w1": _w((lambda *s: _rng.normal(s) * 0.05)(D, F) * (D ** -0.5)),
            "b1": _w((lambda *s: _rng.normal(s) * 0.05)(F)),
            "w2": _w((lambda *s: _rng.normal(s) * 0.05)(F, D) * (F ** -0.5)),
            "b2": _w((lambda *s: _rng.normal(s) * 0.05)(D)),
        }
    _B_in = _B_setup()

    return {
        "A_x": _A_in["x"],
        "A_wqkv": _A_in["wqkv"],
        "A_wo": _A_in["wo"],
        "B_x": _B_in["x"],
        "B_w1": _B_in["w1"],
        "B_b1": _B_in["b1"],
        "B_w2": _B_in["w2"],
        "B_b2": _B_in["b2"],
    }

def _fwd_reference(A_x, A_wqkv, A_wo, B_x, B_w1, B_b1, B_w2, B_b2):
    def _A_ref(x, wqkv, wo):
        B, S, D = x.shape
        H = 32; Dh = D // H
        qkv = (lambda x, *d: x.transpose(*d))((x @ wqkv).reshape(B, S, 3, H, Dh), 2, 0, 3, 1, 4)
        q, k, v = qkv[0], qkv[1], qkv[2]
        phi = lambda t: jnp.where(t > 0, t + 1, jnp.exp(t)) + 1e-6
        pq, pk = phi(q), phi(k)
        kv = jnp.einsum("bhsd,bhse->bhde", pk, v)
        z = jnp.einsum("bhsd->bhd", pk)
        num = jnp.einsum("bhqd,bhde->bhqe", pq, kv)
        den = jnp.einsum("bhqd,bhd->bhq", pq, z)[..., None] + 1e-6
        o = num / den
        return (lambda x, *d: x.transpose(*d))(o, 0, 2, 1, 3).reshape(B, S, D) @ wo

    def _B_ref(x, w1, b1, w2, b2):
        y = _layernorm(x, axis=-1)
        h = _gelu(jnp.einsum("bsd,df->bsf", y, w1) + b1)
        return jnp.einsum("bsf,fd->bsd", h, w2) + b2

    x = A_x
    x = x + _A_ref(_layernorm(x, axis=-1), A_wqkv, A_wo)
    x = x + _B_ref(_layernorm(x, axis=-1), B_w1, B_b1, B_w2, B_b2)
    x = x + _A_ref(_layernorm(x, axis=-1), A_wqkv, A_wo)
    x = x + _B_ref(_layernorm(x, axis=-1), B_w1, B_b1, B_w2, B_b2)
    return x


def setup_inputs():
    _inp = _fwd_setup_inputs()
    _gk = jax.random.fold_in(jax.random.key(int.from_bytes(__import__("os").urandom(4), "little")), 2**31 - 1)
    _shapes = [[1, 2048, 576]]
    _dtypes = ['bfloat16']
    _gks = jax.random.split(_gk, len(_shapes))
    _gs = [jax.random.normal(k, s, dtype=jnp.dtype(d)) * 0.05 for k, s, d in zip(_gks, _shapes, _dtypes)]
    _inp["grad_out"] = _gs[0]
    return _inp

def reference(A_x, A_wqkv, A_wo, B_w1, B_b1, B_w2, B_b2, B_x, grad_out):
    _const = dict(B_x=B_x)
    def _f(*_d):
        return _fwd_reference(**{'A_x': _d[0], 'A_wqkv': _d[1], 'A_wo': _d[2], 'B_w1': _d[3], 'B_b1': _d[4], 'B_w2': _d[5], 'B_b2': _d[6], **_const})
    _out, _vjp = jax.vjp(_f, A_x, A_wqkv, A_wo, B_w1, B_b1, B_w2, B_b2)
    _grads = _vjp(grad_out)
    _out0 = jnp.asarray(_out)
    return (_out0, *[jnp.asarray(_g) for _g in _grads])
```

```python
import jax
import jax.numpy as jnp
from jax import lax
import jax.experimental.pallas as pl
import jax.experimental.pallas.tpu as pltpu

S, D, F = 2048, 576, 4608
H, DH = 32, 18
D3 = 3 * D
DA = 592
T = 128
NT_ = S // T
TB = 512
NB = S // TB
FH = F // 2
FQ = F // 4
QA = 768
W1C = F // 3
QC = 256
NG = 5
WSTEP = 112
HEAD_LO = (0, 7, 13, 19, 25)
HEAD_HI = (6, 12, 18, 24, 31)

LN_EPS = 1e-5
PHI_EPS = 1e-6
GC0 = 0.7978845608028654
GC1 = 0.044715

BF = jnp.bfloat16
F32 = jnp.float32
_NN = (((1,), (0,)), ((), ()))
_NT = (((1,), (1,)), ((), ()))


def _dot(a, b):
    return lax.dot_general(a, b, _NN, preferred_element_type=F32)


def _dot_nt(a, b):
    return lax.dot_general(a, b, _NT, preferred_element_type=F32)


def _colmean(x):
    n = x.shape[1]
    p = jnp.sum(x.reshape(9, 64, n), axis=0)
    p = p[0:32] + p[32:64]
    p = p[0:16] + p[16:32]
    p = p[0:8] + p[8:16]
    return jnp.sum(p, axis=0, keepdims=True) * (1.0 / D)


def _ln(x):
    m = _colmean(x)
    xc = x - m
    v = _colmean(xc * xc)
    rs = lax.rsqrt(v + LN_EPS)
    return xc * rs, rs


def _ln_bwd(dy, y, rs):
    a = _colmean(dy)
    b = _colmean(dy * y)
    return (dy - a - y * b) * rs


def _phi(t):
    return jnp.where(t > 0, t + 1.0, jnp.exp(t)) + PHI_EPS


def _dphi_from_phi(p):
    return jnp.minimum(p - PHI_EPS, 1.0)


def _win(x, g):
    return x[WSTEP * g:WSTEP * g + 128]


def _assemble(parts):
    pieces = [parts[0][:WSTEP]]
    for g in range(NG - 1):
        pieces.append(parts[g][WSTEP:128] + parts[g + 1][0:16])
        pieces.append(parts[g + 1][16:WSTEP] if g + 1 < NG - 1 else parts[g + 1][16:128])
    return jnp.concatenate(pieces, axis=0)


def _head_mask(g):
    r = lax.broadcasted_iota(jnp.int32, (128, 128), 0) + WSTEP * g
    c = lax.broadcasted_iota(jnp.int32, (128, 128), 1) + WSTEP * g
    hr = (r * 3641) >> 16
    hc = (c * 3641) >> 16
    return (hr == hc) & (hr >= HEAD_LO[g]) & (hr <= HEAD_HI[g])


def _lane_fold(x):
    acc = x[:, 0:128]
    for j in range(1, x.shape[1] // 128):
        acc = acc + x[:, 128 * j:128 * (j + 1)]
    return acc


def _lane_tile(x128, n):
    if n == 128:
        return x128
    return jnp.concatenate([x128] * (n // 128), axis=1)


def _gelu_parts(pre):
    x2 = pre * pre
    t = jnp.tanh(pre * (GC0 + (GC0 * GC1) * x2))
    hp = 0.5 + 0.5 * t
    return x2, t, hp


def _cols(s, n):
    if isinstance(s, int):
        return pl.ds(s * n, n)
    return pl.ds(pl.multiple_of(s * n, n), n)


def _kernel(
    x_hbm, wqkv_hbm, wo_hbm, w1_hbm, b1_hbm, w2_hbm, b2_hbm, g_hbm,
    out_hbm, dx_hbm, dwqkv_hbm, dwo_hbm, dw1_hbm, db1_hbm, dw2_hbm, db2_hbm,
    xs, gs, wqkv, wqkvT, wo, w1c, w1T, w2c, w2T, b1v, b2v, b2col,
    dw1a, dw2Ta, pre2, stream, u_s, qkv_s, wq_s, y2_s, u2_s, stat,
    ycur, ucur, oacc, dyacc, hcar,
    kvT, zacc, zb, mm, mmT, zm, bm, pacc, dkv, dkvT, dwo_a, db2a,
    sem_in, sem_out,
):
    def cp_x(s):
        return pltpu.make_async_copy(x_hbm.at[0, :, _cols(s, TB)], xs.at[:, _cols(s, TB)], sem_in.at[s])

    k0 = NB
    cp_wqkv = pltpu.make_async_copy(wqkv_hbm, wqkv, sem_in.at[k0])
    cp_wo = pltpu.make_async_copy(wo_hbm, wo, sem_in.at[k0 + 1])
    cp_b1 = pltpu.make_async_copy(b1_hbm, b1v, sem_in.at[k0 + 2])
    cp_b2 = pltpu.make_async_copy(b2_hbm, b2v, sem_in.at[k0 + 3])
    cp_w2 = pltpu.make_async_copy(w2_hbm, w2T, sem_in.at[k0 + 4])
    cp_g = pltpu.make_async_copy(g_hbm.at[0], gs, sem_in.at[k0 + 5])
    k1 = k0 + 6

    def cp_w1(c):
        return pltpu.make_async_copy(w1_hbm.at[:, _cols(c, W1C)], w1c.at[pl.ds(0, D), _cols(c, W1C)],
                                     sem_in.at[k1 + c])

    cp_x(0).start()
    cp_wqkv.start()
    cp_b1.start()
    cp_b2.start()
    for s in range(1, NB):
        cp_x(s).start()
        cp_w1(s - 1).start()
    cp_wo.start()
    cp_w2.start()
    cp_g.start()

    def front_a(l, cs, x):
        u, rs = _ln(x)
        ub = u.astype(BF)
        u_s[l, :, cs] = ub
        stat[l:l + 1, cs] = rs
        return ub

    def front_b(l, cs, ub):
        qkv = _dot(wqkvT[...], ub)
        pq = _phi(qkv[:D])
        pk = _phi(qkv[D:2 * D])
        pkb = pk.astype(BF)
        vb = qkv[2 * D:].astype(BF)
        qkv_s[l, 0:D, cs] = pq.astype(BF)
        qkv_s[l, D:2 * D, cs] = pkb
        qkv_s[l, 2 * D:, cs] = vb
        zacc[...] += _lane_fold(pk)
        return pkb, vb

    def front_c(l, pkb, vb):
        for g in range(NG):
            kvT[l, g] += _dot_nt(_win(vb, g), _win(pkb, g))

    def attn_fwd_finalize(l):
        z = jnp.sum(zacc[...], axis=1, keepdims=True)
        zbv = jnp.broadcast_to(z, (D, 128))
        zb[l] = zbv
        parts = []
        for g in range(NG):
            msk = _head_mask(g)
            kt = jnp.where(msk, kvT[l, g], 0.0)
            kvT[l, g] = kt
            parts.append(_dot(kt.T.astype(BF), wo[WSTEP * g:WSTEP * g + 128, :]))
            zm[g] = jnp.where(msk, _win(zbv, g), 0.0).T.astype(BF)
        m = _assemble(parts)
        mm[l] = m.astype(BF)
        mmT[...] = m.T.astype(BF)
        zacc[...] = jnp.zeros_like(zacc)

    def back_a(l, cs):
        pqb = qkv_s[l, 0:D, cs]
        den = _assemble([_dot(zm[g], _win(pqb, g)) for g in range(NG)]) + PHI_EPS
        rden = 1.0 / den
        pq = pqb.astype(F32)
        pqn = (pq * rden).astype(BF)
        qkv_s[l, 0:D, cs] = pqn
        wq_s[l, :, cs] = (_dphi_from_phi(pq) * rden).astype(BF)
        return pqn

    def back_b(x, pqn):
        x1 = x + _dot(mmT[...], pqn)
        u, rs1 = _ln(x1)
        y, rs2 = _ln(u)
        return x1, u.astype(BF), aug(y), rs1, rs2

    def bwd1_a(l, cs, g):
        gb = g.astype(BF)
        pqnb = qkv_s[l, 0:D, cs]
        dpqn = _dot(mm[l], gb)
        pacc[...] += _dot_nt(pqnb, gb)
        return dpqn, pqnb.astype(F32)

    def bwd1_b(l, cs, dpqn, pqn):
        tb = (dpqn * pqn).astype(BF)
        r = _assemble([_dot(bm[gg], _win(tb, gg)) for gg in range(NG)])
        dq = (dpqn - r * _lane_tile(zb[l], pqn.shape[1])) * wq_s[l, :, cs].astype(F32)
        qkv_s[l, 0:D, cs] = dq.astype(BF)
        zacc[...] += _lane_fold(r * pqn)

    def attn_bwd_finalize(l, first):
        dz = -jnp.sum(zacc[...], axis=1, keepdims=True)
        zb[l] = jnp.broadcast_to(dz, (D, 128))
        pb = pacc[...].astype(BF)
        parts = []
        for g in range(NG):
            msk = _head_mask(g)
            pw = _win(pb, g)
            d = jnp.where(msk, _dot_nt(pw, wo[WSTEP * g:WSTEP * g + 128, :]), 0.0)
            dkv[g] = d.astype(BF)
            dkvT[g] = d.T.astype(BF)
        for g in range(NG):
            parts.append(_dot(kvT[l, g].astype(BF), _win(pb, g)))
        dwo = _assemble(parts)
        if first:
            dwo_a[...] = dwo
            zacc[...] = jnp.zeros_like(zacc)
            pacc[...] = jnp.zeros_like(pacc)
        else:
            dwo_a[...] += dwo

    def bwd2_a(l, cs, n):
        pkb = qkv_s[l, D:2 * D, cs]
        vb = qkv_s[l, 2 * D:, cs]
        dpk = _assemble([_dot(dkv[gg], _win(vb, gg)) for gg in range(NG)]) + _lane_tile(zb[l], n)
        dk = (dpk * _dphi_from_phi(pkb.astype(F32))).astype(BF)
        dv = _assemble([_dot(dkvT[gg], _win(pkb, gg)) for gg in range(NG)]).astype(BF)
        qkv_s[l, D:2 * D, cs] = dk
        qkv_s[l, 2 * D:, cs] = dv
        return jnp.concatenate([qkv_s[l, 0:D, cs], dk, dv], axis=0)

    def bwd2_b(l, cs, dqkv):
        du = _dot(wqkv[...], dqkv)
        return stream[:, cs] + _ln_bwd(du, u_s[l, :, cs].astype(F32), stat[l:l + 1, cs])

    def aug(y):
        r = lax.broadcasted_iota(jnp.int32, (DA - D, T), 0)
        return jnp.concatenate([y.astype(BF), jnp.where(r == 0, 1.0, 0.0).astype(BF)], axis=0)

    def hs(h):
        return pl.ds(h * FH, FH)

    def qs(c):
        return pl.ds(c * FQ, FQ)

    def f_pre(y, cs, c):
        pre = _dot(w1T[qs(c), :], y)
        pre2[qs(c), cs] = pre.astype(BF)
        _, _, hp = _gelu_parts(pre)
        return (pre * hp).astype(BF)

    def f_out(hh, c):
        return _dot(w2T[:, qs(c)], hh)

    def gelu_bwd(pre):
        x2, t, hp = _gelu_parts(pre)
        hh = (pre * hp).astype(BF)
        gp = hp + (0.5 * pre) * (1.0 - t * t) * (GC0 + (3.0 * GC0 * GC1) * x2)
        return hh, gp

    def m_dh(gb, h):
        return _dot(w2c[hs(h), :], gb)

    def m_pre(y, h):
        return _dot(w1T[hs(h), :], y)

    def m_dy(dpre, h):
        return _dot(w1c[0:D, hs(h)], dpre)

    def m_out(hh, h):
        return _dot(w2T[:, hs(h)], hh)

    def acc_to(ref, h, val, keep):
        if keep is True:
            ref[:, hs(h)] += val
        elif keep is False:
            ref[:, hs(h)] = val
        else:
            ref[:, hs(h)] = jnp.where(keep, ref[:, hs(h)], 0.0) + val

    def m_w1(y, dpre, h, keep=True):
        acc_to(dw1a, h, _dot_nt(y, dpre), keep)

    def m_w2(gb, hh, h, keep=True):
        acc_to(dw2Ta, h, _dot_nt(gb, hh), keep)

    zacc[...] = jnp.zeros_like(zacc)
    kvT[...] = jnp.zeros_like(kvT)
    pacc[...] = jnp.zeros_like(pacc)
    db2a[...] = jnp.zeros_like(db2a)
    for g in range(NG):
        bm[g] = jnp.where(_head_mask(g), 1.0, 0.0).astype(BF)
    cp_b1.wait()
    cp_b2.wait()
    b2col[...] = jnp.broadcast_to(b2v[...].reshape(1, D).astype(F32), (128, D)).T
    rid = lax.broadcasted_iota(jnp.int32, (DA - D, F), 0)
    w1c[D:DA, :] = jnp.where(
        rid == 0, jnp.broadcast_to(b1v[...].reshape(1, F).astype(F32), (DA - D, F)), 0.0).astype(BF)
    cp_x(0).wait()
    cp_wqkv.wait()
    wqkvT[...] = wqkv[...].T

    def front(l, cs, x):
        front_c(l, *front_b(l, cs, front_a(l, cs, x)))

    front(0, _cols(0, TB), xs[:, _cols(0, TB)].astype(F32))

    def p1(s, c):
        cp_x(s).wait()
        cp_w1(s - 1).wait()
        w1T[_cols(s - 1, W1C), :] = w1c[:, _cols(s - 1, W1C)].T
        front(0, _cols(s, TB), xs[:, _cols(s, TB)].astype(F32))
        return c

    lax.fori_loop(1, NB, p1, 0)

    def save_2(cs, u, y, rs1, rs2):
        u2_s[:, cs] = u
        y2_s[:, cs] = y
        stat[2:3, cs] = rs1
        stat[3:4, cs] = rs2

    def step_2(s, first=False, last=False):
        cs = _cols(s, T)
        cn = _cols(s + 1, T)
        if not first:
            y = y2_s[:, cs]
            o = oacc[...]
            h1 = hcar[...]
        if not last:
            pqn = back_a(0, cn)
        if not first:
            h2 = f_pre(y, cs, 2)
        if not last:
            x1, un, yn, rs1, rs2 = back_b(xs[:, cn].astype(F32), pqn)
            save_2(cn, un, yn, rs1, rs2)
        if not first:
            o = o + f_out(h1, 1)
            h3 = f_pre(y, cs, 3)
            o = o + f_out(h2, 2)
        if not last:
            h0n = f_pre(yn, cn, 0)
        if not first:
            x2 = o + f_out(h3, 3)
            stream[:, cs] = x2
            ub = front_a(1, cs, x2)
        if not last:
            hcar[...] = f_pre(yn, cn, 1)
        if not first:
            pkb, vb = front_b(1, cs, ub)
        if not last:
            oacc[...] = x1 + b2col[...] + f_out(h0n, 0)
        if not first:
            front_c(1, pkb, vb)

    cp_wo.wait()
    cp_w2.wait()
    attn_fwd_finalize(0)
    step_2(-1, first=True)

    def p2(s, carry):
        j = pl.ds(pl.multiple_of(jnp.minimum(s, 11) * 384, 384), 384)
        w2c[j, :] = w2T[:, j].T
        step_2(s)
        return carry

    lax.fori_loop(0, NT_ - 1, p2, 0)

    def step_3(s, first=False, last=False):
        cs = _cols(s, T)
        cn = _cols(s + 1, T)
        if not first:
            y = ycur[...]
            u = ucur[...]
            gb = gs[:, cs]
            rs1 = stat[4:5, cs]
            rs2 = stat[5:6, cs]
            o0 = oacc[...]
            dy0 = dyacc[...]
        if not last:
            gn = gs[:, cn]
            pqn = back_a(1, cn)
        if not first:
            dh = m_dh(gb, 1)
        if not last:
            x3, un, yn, rs1n, rs2n = back_b(stream[:, cn], pqn)
            stat[4:5, cn] = rs1n
            stat[5:6, cn] = rs2n
            ycur[...] = yn
            ucur[...] = un
        if not first:
            hh, gp = gelu_bwd(m_pre(y, 1))
            dpre = (dh * gp).astype(BF)
            dy = dy0 + m_dy(dpre, 1)
            g = gb.astype(F32)
            db2a[...] += g
            du = _ln_bwd(dy, y[0:D].astype(F32), rs2)
            g3 = g + _ln_bwd(du, u.astype(F32), rs1)
            stream[:, cs] = g3
            xs[:, cs] = (o0 + m_out(hh, 1)).astype(BF)
            keep = True if last else s > 0
            m_w1(y, dpre, 1, keep)
            m_w2(gb, hh, 1, keep)
        if not last:
            dhn = m_dh(gn, 0)
        if not first:
            dpqn, pq = bwd1_a(1, cs, g3)
        if not last:
            hn, gpn = gelu_bwd(m_pre(yn, 0))
            dpren = (dhn * gpn).astype(BF)
        if not first:
            bwd1_b(1, cs, dpqn, pq)
        if not last:
            dyacc[...] = m_dy(dpren, 0)
            oacc[...] = x3 + b2col[...] + m_out(hn, 0)
            m_w1(yn, dpren, 0, not first)
            m_w2(gn, hn, 0, not first)

    cp_g.wait()
    step_2(NT_ - 1, last=True)
    attn_fwd_finalize(1)
    step_3(-1, first=True)

    def p3(s, carry):
        step_3(s)
        return carry

    lax.fori_loop(0, NT_ - 1, p3, 0)

    def step_4(s, first=False, last=False):
        cs = _cols(s, T)
        cn = _cols(s + 1, T)
        if not first:
            y = y2_s[:, cs]
            gb = ucur[...]
            g2 = oacc[...]
            dy0 = dyacc[...]
        if not last:
            yn = y2_s[:, cn]
            dqkv = bwd2_a(1, cn, T)
        if not first:
            dh = m_dh(gb, 1)
        if not last:
            g2n = bwd2_b(1, cn, dqkv)
            gn = g2n.astype(BF)
            db2a[...] += g2n
            ucur[...] = gn
            oacc[...] = g2n
        if not first:
            hh, gp = gelu_bwd(pre2[hs(1), cs].astype(F32))
            dpre = (dh * gp).astype(BF)
            m_w2(gb, hh, 1)
            dy = dy0 + m_dy(dpre, 1)
            du = _ln_bwd(dy, y[0:D].astype(F32), stat[3:4, cs])
            g1 = g2 + _ln_bwd(du, u2_s[:, cs].astype(F32), stat[2:3, cs])
            stream[:, cs] = g1
            m_w1(y, dpre, 1)
        if not last:
            dhn = m_dh(gn, 0)
            hn, gpn = gelu_bwd(pre2[hs(0), cn].astype(F32))
            dpren = (dhn * gpn).astype(BF)
        if not first:
            dpqn, pq = bwd1_a(0, cs, g1)
        if not last:
            m_w2(gn, hn, 0)
        if not first:
            bwd1_b(0, cs, dpqn, pq)
        if not last:
            dyacc[...] = m_dy(dpren, 0)
            m_w1(yn, dpren, 0)

    cp_out = pltpu.make_async_copy(xs, out_hbm.at[0], sem_out.at[0])

    step_3(NT_ - 1, last=True)
    attn_bwd_finalize(1, True)
    step_4(-1, first=True)
    cp_out.start()

    def p4(s, carry):
        step_4(s)
        return carry

    lax.fori_loop(0, NT_ - 1, p4, 0)

    w1c[0:D, hs(0)] = dw1a[0:D, hs(0)].astype(BF)
    w2T[:, hs(0)] = dw2Ta[:, hs(0)].astype(BF)
    step_4(NT_ - 1, last=True)
    dw2Ta[:, 0:QA] = _dot_nt(u_s[1, :, 0:TB], qkv_s[1, 0:QA, 0:TB])
    attn_bwd_finalize(0, False)
    dw2Ta[:, QA:D3] = _dot_nt(u_s[1, :, 0:TB], qkv_s[1, QA:D3, 0:TB])
    b1v[...] = dw1a[D:D + 1, :].astype(BF).reshape(F)
    b2v[...] = jnp.sum(db2a[...].T, axis=0, keepdims=True).astype(BF).reshape(D)
    wo[...] = dwo_a[...].astype(BF)
    cp_dw1a = pltpu.make_async_copy(w1c.at[pl.ds(0, D), hs(0)], dw1_hbm.at[:, hs(0)], sem_out.at[1])
    cp_dw2a = pltpu.make_async_copy(w2T.at[:, hs(0)], dw2_hbm.at[:, hs(0)], sem_out.at[2])
    cp_db1 = pltpu.make_async_copy(b1v, db1_hbm, sem_out.at[3])
    cp_db2 = pltpu.make_async_copy(b2v, db2_hbm, sem_out.at[4])
    cp_dwo = pltpu.make_async_copy(wo, dwo_hbm, sem_out.at[5])
    cp_dw1a.start()
    cp_dw2a.start()
    cp_db1.start()
    cp_db2.start()
    cp_dwo.start()
    o3 = 6
    RQ = D // NB

    def cp_dx(s):
        return pltpu.make_async_copy(gs.at[:, _cols(s, TB)], dx_hbm.at[0, :, _cols(s, TB)], sem_out.at[o3 + s])

    def cp_dw1b(s):
        return pltpu.make_async_copy(w1c.at[_cols(s, RQ), hs(1)], dw1_hbm.at[_cols(s, RQ), hs(1)],
                                     sem_out.at[o3 + NB + s])

    def cp_dw2b(s):
        return pltpu.make_async_copy(w2T.at[_cols(s, RQ), hs(1)], dw2_hbm.at[_cols(s, RQ), hs(1)],
                                     sem_out.at[o3 + 2 * NB + s])

    def p5(s, carry):
        cs = _cols(s, TB)
        ks = pl.ds(pl.multiple_of(TB + s * 384, 128), 384)
        w1c[_cols(s, RQ), hs(1)] = dw1a[_cols(s, RQ), hs(1)].astype(BF)
        w2T[_cols(s, RQ), hs(1)] = dw2Ta[_cols(s, RQ), hs(1)].astype(BF)
        u3 = u_s[1, :, ks]
        dqkv = bwd2_a(0, cs, TB)
        dw2Ta[:, 0:QA] += _dot_nt(u3, qkv_s[1, 0:QA, ks])
        dx = bwd2_b(0, cs, dqkv)
        gs[:, cs] = dx.astype(BF)
        dw2Ta[:, QA:D3] += _dot_nt(u3, qkv_s[1, QA:D3, ks])
        cp_dx(s).start()
        cp_dw1b(s).start()
        cp_dw2b(s).start()
        return carry

    lax.fori_loop(0, NB, p5, 0)

    o4 = o3 + 3 * NB
    qchunks = [(c0, min(QC, D3 - c0)) for c0 in range(0, D3, QC)]

    def cp_dwqkv(i):
        c0, w = qchunks[i]
        return pltpu.make_async_copy(wqkv.at[:, pl.ds(c0, w)], dwqkv_hbm.at[:, pl.ds(c0, w)], sem_out.at[o4 + i])

    for i, (c0, w) in enumerate(qchunks):
        acc = dw2Ta[:, c0:c0 + w] + _dot_nt(u_s[0], qkv_s[0, c0:c0 + w, :])
        wqkv[:, c0:c0 + w] = acc.astype(BF)
        cp_dwqkv(i).start()

    cp_out.wait()
    cp_dw1a.wait()
    cp_dw2a.wait()
    cp_db1.wait()
    cp_db2.wait()
    cp_dwo.wait()
    for s in range(NB):
        cp_dx(s).wait()
        cp_dw1b(s).wait()
        cp_dw2b(s).wait()
    for i in range(len(qchunks)):
        cp_dwqkv(i).wait()


@jax.jit
def pallas_interleave_layers__linear_attn_block__mixer_channel_mlp__prompt_kernel(
    A_x: jax.Array,
    A_wqkv: jax.Array,
    A_wo: jax.Array,
    B_x: jax.Array,
    B_w1: jax.Array,
    B_b1: jax.Array,
    B_w2: jax.Array,
    B_b2: jax.Array,
    grad_out: jax.Array,
):
    del B_x
    V = pltpu.VMEM
    n_in = NB + 6 + 3
    n_out = 6 + 3 * NB + (-(-D3 // QC))
    scratch = [
        V((D, S), BF),
        V((D, S), BF),
        V((D, D3), BF),
        V((D3, D), BF),
        V((D, D), BF),
        V((DA, F), BF),
        V((F, DA), BF),
        V((F, D), BF),
        V((D, F), BF),
        V((F,), BF),
        V((D,), BF),
        V((D, 128), F32),
        V((DA, F), F32),
        V((D, F), F32),
        V((F, S), BF),
        V((D, S), F32),
        V((2, D, S), BF),
        V((2, D3, S), BF),
        V((2, D, S), BF),
        V((DA, S), BF),
        V((D, S), BF),
        V((8, S), F32),
        V((DA, T), BF),
        V((D, T), BF),
        V((D, T), F32),
        V((D, T), F32),
        V((FQ, T), BF),
        V((2, NG, 128, 128), F32),
        V((D, 128), F32),
        V((2, D, 128), F32),
        V((2, D, D), BF),
        V((D, D), BF),
        V((NG, 128, 128), BF),
        V((NG, 128, 128), BF),
        V((D, D), F32),
        V((NG, 128, 128), BF),
        V((NG, 128, 128), BF),
        V((D, D), F32),
        V((D, 128), F32),
        pltpu.SemaphoreType.DMA((n_in,)),
        pltpu.SemaphoreType.DMA((n_out,)),
    ]
    any_spec = pl.BlockSpec(memory_space=pl.ANY)
    out_shape = (
        jax.ShapeDtypeStruct((1, D, S), BF),
        jax.ShapeDtypeStruct((1, D, S), BF),
        jax.ShapeDtypeStruct((D, D3), BF),
        jax.ShapeDtypeStruct((D, D), BF),
        jax.ShapeDtypeStruct((D, F), BF),
        jax.ShapeDtypeStruct((F,), BF),
        jax.ShapeDtypeStruct((D, F), BF),
        jax.ShapeDtypeStruct((D,), BF),
    )
    outT, dxT, dwqkv, dwo, dw1, db1, dw2T, db2 = pl.pallas_call(
        _kernel,
        out_shape=out_shape,
        in_specs=[any_spec] * 8,
        out_specs=tuple([any_spec] * 8),
        scratch_shapes=scratch,
        compiler_params=pltpu.CompilerParams(vmem_limit_bytes=127 * 1024 * 1024),
    )(jnp.swapaxes(A_x, 1, 2), A_wqkv, A_wo, B_w1, B_b1, B_w2.T, B_b2, jnp.swapaxes(grad_out, 1, 2))
    return (jnp.swapaxes(outT, 1, 2), jnp.swapaxes(dxT, 1, 2), dwqkv, dwo, dw1, db1, dw2T.T, db2)
```

```python
import jax
import jax.numpy as jnp
from jax import lax
import jax.experimental.pallas as pl
import jax.experimental.pallas.tpu as pltpu

S, D, F = 2048, 576, 4608
H, DH = 32, 18
D3 = 3 * D
DA = 592
T = 128
NT_ = S // T
TB = 512
NB = S // TB
FH = F // 2
FQ = F // 4
D2 = 2 * D
DR = D + H
QA = 512
W1C = F // 3
NG = 5
WSTEP = 112
HEAD_LO = (0, 7, 13, 19, 25)
HEAD_HI = (6, 12, 18, 24, 31)

LN_EPS = 1e-5
PHI_EPS = 1e-6
GC0 = 0.7978845608028654
GC1 = 0.044715

BF = jnp.bfloat16
F32 = jnp.float32
_NN = (((1,), (0,)), ((), ()))
_NT = (((1,), (1,)), ((), ()))


def _dot(a, b):
    return lax.dot_general(a, b, _NN, preferred_element_type=F32)


def _dot_nt(a, b):
    return lax.dot_general(a, b, _NT, preferred_element_type=F32)


def _colmean(x):
    n = x.shape[1]
    p = jnp.sum(x.reshape(9, 64, n), axis=0)
    p = p[0:32] + p[32:64]
    p = p[0:16] + p[16:32]
    p = p[0:8] + p[8:16]
    return jnp.sum(p, axis=0, keepdims=True) * (1.0 / D)


def _ln(x):
    m = _colmean(x)
    xc = x - m
    v = _colmean(xc * xc)
    rs = lax.rsqrt(v + LN_EPS)
    return xc * rs, rs


def _ln_bwd(dy, y, rs):
    a = _colmean(dy)
    b = _colmean(dy * y)
    return (dy - a - y * b) * rs


def _ln2(x):
    m = _colmean(x)
    xc = x - m
    s1 = _colmean(xc)
    s2 = _colmean(xc * xc)
    rs1 = lax.rsqrt(s2 + LN_EPS)
    m2 = s1 * rs1
    v2 = s2 * rs1 * rs1 - m2 * m2
    rs2 = lax.rsqrt(v2 + LN_EPS)
    rs12 = rs1 * rs2
    return xc * rs12 - m2 * rs2, rs12


def _ln2_bwd(dy, y, rs12):
    a = _colmean(dy)
    b = _colmean(dy * y) * (1.0 + LN_EPS)
    return (dy - a - y * b) * rs12


def _headsum(x):
    n = x.shape[1]
    p = x.reshape(DH, H, n)
    p = p[0:9] + p[9:18]
    q = (p[0] + p[1]) + (p[2] + p[3])
    r = (p[4] + p[5]) + (p[6] + p[7])
    return (q + r) + p[8]


def _headmul(x, c):
    n = x.shape[1]
    return (x.reshape(DH, H, n) * c[None]).reshape(D, n)


_LT = ((0, 128), (128, 128), (256, 128), (384, 128), (512, 64))


def _to_perm(scr, val):
    for c, (o, w) in enumerate(_LT):
        scr[c, :, 0:w] = val[:, o:o + w]
    return jnp.concatenate(
        [jnp.concatenate([scr[c, pl.ds(j, H, stride=DH), 0:w] for c, (o, w) in enumerate(_LT)], axis=1)
         for j in range(DH)], axis=0)


def _from_perm(scr, val):
    for j in range(DH):
        for c, (o, w) in enumerate(_LT):
            scr[c, pl.ds(j, H, stride=DH), 0:w] = val[H * j:H * j + H, o:o + w]
    return jnp.concatenate([scr[c, :, 0:w] for c, (o, w) in enumerate(_LT)], axis=1)


def _aug(y):
    r = lax.broadcasted_iota(jnp.int32, (DA - D, y.shape[1]), 0)
    return jnp.concatenate([y.astype(BF), jnp.where(r < 2, 1.0, 0.0).astype(BF)], axis=0)


def _phi(t):
    return jnp.where(t > 0, t + 1.0, jnp.exp(t)) + PHI_EPS


def _dphi_from_phi(p):
    return jnp.minimum(p - PHI_EPS, 1.0)


def _win(x, g):
    return x[WSTEP * g:WSTEP * g + 128]


def _assemble(parts):
    pieces = [parts[0][:WSTEP]]
    for g in range(NG - 1):
        pieces.append(parts[g][WSTEP:128] + parts[g + 1][0:16])
        pieces.append(parts[g + 1][16:WSTEP] if g + 1 < NG - 1 else parts[g + 1][16:128])
    return jnp.concatenate(pieces, axis=0)


def _head_mask(g):
    r = lax.broadcasted_iota(jnp.int32, (128, 128), 0) + WSTEP * g
    c = lax.broadcasted_iota(jnp.int32, (128, 128), 1) + WSTEP * g
    hr = (r * 3641) >> 16
    hc = (c * 3641) >> 16
    return (hr == hc) & (hr >= HEAD_LO[g]) & (hr <= HEAD_HI[g])


def _lane_fold(x):
    acc = x[:, 0:128]
    for j in range(1, x.shape[1] // 128):
        acc = acc + x[:, 128 * j:128 * (j + 1)]
    return acc


def _lane_tile(x128, n):
    if n == 128:
        return x128
    return jnp.concatenate([x128] * (n // 128), axis=1)


def _gelu_parts(pre):
    x2 = pre * pre
    t = jnp.tanh(pre * (GC0 + (GC0 * GC1) * x2))
    hp = 0.5 + 0.5 * t
    return x2, t, hp


def _cols(s, n):
    if isinstance(s, int):
        return pl.ds(s * n, n)
    return pl.ds(pl.multiple_of(s * n, n), n)


def _kernel(
    x_hbm, wqkv_hbm, wo_hbm, w1_hbm, b1_hbm, w2_hbm, b2_hbm, g_hbm,
    out_hbm, dx_hbm, dwqkv_hbm, dwo_hbm, dw1_hbm, db1_hbm, dw2_hbm, db2_hbm,
    xs, gs, wraw, wx, wT, wo, w1c, w1T, w2c, w2T, b1v, b2v, b2col,
    dw1a, dw2Ta, pre2, stream, u_s, qk_s, rd_s, y2_s, y4_s, stat,
    oacc, dyacc, hcar,
    kvT, cacc, ctb, zb, mm, mmT, pacc, dctb, dwv_a, dwo_a, db2a, ps0, ps1,
    sem_in, sem_out,
):
    def cp_x(s):
        return pltpu.make_async_copy(x_hbm.at[0, :, _cols(s, TB)], xs.at[:, _cols(s, TB)], sem_in.at[s])

    k0 = NB
    cp_wqkv = pltpu.make_async_copy(wqkv_hbm, wraw, sem_in.at[k0])
    cp_wo = pltpu.make_async_copy(wo_hbm, wo, sem_in.at[k0 + 1])
    cp_b1 = pltpu.make_async_copy(b1_hbm, b1v, sem_in.at[k0 + 2])
    cp_b2 = pltpu.make_async_copy(b2_hbm, b2v, sem_in.at[k0 + 3])
    cp_w2 = pltpu.make_async_copy(w2_hbm, w2T, sem_in.at[k0 + 4])
    cp_g = pltpu.make_async_copy(g_hbm.at[0], gs, sem_in.at[k0 + 5])
    k1 = k0 + 6

    def cp_w1(c):
        return pltpu.make_async_copy(w1_hbm.at[:, _cols(c, W1C)], w1c.at[pl.ds(0, D), _cols(c, W1C)],
                                     sem_in.at[k1 + c])

    cp_wqkv.start()
    cp_x(0).start()
    cp_b1.start()
    cp_b2.start()
    for s in range(1, NB):
        cp_x(s).start()
        cp_w1(s - 1).start()
    cp_wo.start()
    cp_w2.start()
    cp_g.start()

    def wrow(ref, g, base=0):
        return ref[base + WSTEP * g:base + WSTEP * g + 128, :]

    def front_a(l, cs, x):
        u, rs = _ln(x)
        ub = _aug(u)
        u_s[l, :, cs] = ub
        stat[l:l + 1, cs] = rs
        return ub

    def front_b(l, cs, ub):
        qk = _dot(wT[0:D2, :], ub[0:D])
        pkb = _phi(qk[D:]).astype(BF)
        qk_s[l, 0:D, cs] = _phi(qk[:D]).astype(BF)
        qk_s[l, D2:D3, cs] = pkb
        return pkb

    def front_c(pkb, ub, first=False):
        c = _dot_nt(pkb, ub)
        if first:
            cacc[...] = c
        else:
            cacc[...] += c

    def ff_a(l):
        c = cacc[...]
        zb[l] = jnp.broadcast_to(c[:, D:D + 1], (D, 128))
        ct = _from_perm(ps0, c[:, 0:D]).astype(BF)
        ctb[l] = ct
        if l == 0:
            cacc[...] = jnp.zeros_like(cacc)
        return ct

    def ff_b(l, ct):
        kvs = []
        for g in range(NG):
            kv = jnp.where(_head_mask(g), _dot_nt(_win(ct, g), wrow(wT, g, D2)), 0.0)
            kvT[l, g] = kv.T.astype(BF)
            kvs.append(kv.astype(BF))
        return kvs

    def ff_c(l, kvs):
        m = _assemble([_dot(kvs[g], wrow(wo, g)) for g in range(NG)])
        mp = _to_perm(ps1, m).astype(BF)
        mm[l] = mp
        mmT[...] = mp.T

    def back_a(l, cs):
        pq = qk_s[l, 0:D, cs].astype(F32)
        rden = 1.0 / (_headsum(pq * zb[l]) + PHI_EPS)
        rd_s[l, :, cs] = rden
        return _headmul(pq, rden).astype(BF)

    def back_b(x, pqn):
        x1 = x + _dot(mmT[...], pqn)
        y, rs12 = _ln2(x1)
        return x1, _aug(y), rs12

    def bwd1_a(l, g):
        gb = g.astype(BF)
        return gb, _dot(mm[l], gb)

    def bwd1_b(l, cs, gb, dpqn):
        pq = qk_s[l, 0:D, cs].astype(F32)
        rden = rd_s[l, :, cs]
        pqn = _headmul(pq, rden)
        r = _headsum(dpqn * pqn)
        dq = _headmul((dpqn - _headmul(zb[l], r)) * _dphi_from_phi(pq), rden)
        qk_s[l, 0:D, cs] = dq.astype(BF)
        pacc[...] += _dot_nt(pqn.astype(BF), jnp.concatenate([gb, r.astype(BF)], axis=0))

    def bf_a(l):
        p = pacc[...]
        tl = p[:, 512:DR]
        rr = lax.broadcasted_iota(jnp.int32, tl.shape, 0)
        cc = lax.broadcasted_iota(jnp.int32, tl.shape, 1)
        dz = -jnp.sum(jnp.where(cc - (D - 512) == (rr & (H - 1)), tl, 0.0), axis=1, keepdims=True)
        hi = dz.astype(BF).astype(F32)
        ce = lax.broadcasted_iota(jnp.int32, (D, DA - D), 1)
        dctb[:, D:DA] = jnp.where(ce == 0, hi, jnp.where(ce == 1, dz - hi, 0.0)).astype(BF)
        pb = _from_perm(ps0, p[:, 0:D]).astype(BF)
        if l == 1:
            pacc[...] = jnp.zeros_like(pacc)
        return pb

    def acc_l(ref, l, val):
        if l == 1:
            ref[...] = val
        else:
            ref[...] += val

    def bf_b(l, pb):
        ds_ = [jnp.where(_head_mask(g), _dot_nt(_win(pb, g), wrow(wo, g)), 0.0) for g in range(NG)]
        acc_l(dwo_a, l, _assemble([_dot(kvT[l, g], _win(pb, g)) for g in range(NG)]))
        return ds_

    def bf_c(l, ds_):
        dct = _assemble([_dot(ds_[g].astype(BF), wrow(wT, g, D2)) for g in range(NG)])
        dp = _to_perm(ps1, dct).astype(BF)
        dctb[:, 0:D] = dp
        wx[:, D2:D3] = dp.T
        acc_l(dwv_a, l, _assemble([_dot(ds_[g].T.astype(BF), wrow(ctb.at[l], g)) for g in range(NG)]))

    def bwd2_a(l, cs):
        dpk = _dot(dctb[...], u_s[l, :, cs])
        dk = (dpk * _dphi_from_phi(qk_s[l, D2:D3, cs].astype(F32))).astype(BF)
        qk_s[l, D:D2, cs] = dk
        return dk

    def bwd2_b(l, cs, dk=None):
        if dk is None:
            rhs = qk_s[l, :, cs]
        else:
            rhs = jnp.concatenate([qk_s[l, 0:D, cs], dk, qk_s[l, D2:D3, cs]], axis=0)
        du = _dot(wx[...], rhs)
        return stream[:, cs] + _ln_bwd(du, u_s[l, 0:D, cs].astype(F32), stat[l:l + 1, cs])

    def hs(h):
        return pl.ds(h * FH, FH)

    def qs(c):
        return pl.ds(c * FQ, FQ)

    def f_pre(y, cs, c):
        pre = _dot(w1T[qs(c), :], y)
        pre2[qs(c), cs] = pre.astype(BF)
        _, _, hp = _gelu_parts(pre)
        return (pre * hp).astype(BF)

    def f_out(hh, c):
        return _dot(w2T[:, qs(c)], hh)

    def gelu_bwd(pre):
        x2, t, hp = _gelu_parts(pre)
        hh = (pre * hp).astype(BF)
        gp = hp + (0.5 * pre) * (1.0 - t * t) * (GC0 + (3.0 * GC0 * GC1) * x2)
        return hh, gp

    def m_dh(gb, h):
        return _dot(w2c[hs(h), :], gb)

    def m_dhq(gb, c):
        return _dot(w2c[qs(c), :], gb)

    def m_pre(y, h):
        return _dot(w1T[hs(h), :], y)

    def m_dy(dpre, h):
        return _dot(w1c[0:D, hs(h)], dpre)

    def m_out(hh, h):
        return _dot(w2T[:, hs(h)], hh)

    def acc_to(ref, sl, val, keep):
        if keep is True:
            ref[:, sl] += val
        elif keep is False:
            ref[:, sl] = val
        else:
            ref[:, sl] = jnp.where(keep, ref[:, sl], 0.0) + val

    def m_w1(y, dpre, h, keep=True):
        acc_to(dw1a, hs(h), _dot_nt(y, dpre), keep)

    def m_w2(gb, hh, h, keep=True):
        acc_to(dw2Ta, hs(h), _dot_nt(gb, hh), keep)

    def m_wq(ref, a, b, c):
        acc_to(ref, qs(c), _dot_nt(a, b[(c - 2) * FQ:(c - 1) * FQ]), True)

    pacc[...] = jnp.zeros_like(pacc)
    db2a[...] = jnp.zeros_like(db2a)
    cp_b1.wait()
    cp_b2.wait()
    b2col[...] = jnp.broadcast_to(b2v[...].reshape(1, D).astype(F32), (128, D)).T
    rid = lax.broadcasted_iota(jnp.int32, (DA - D, F), 0)
    w1c[D:DA, :] = jnp.where(
        rid == 0, jnp.broadcast_to(b1v[...].reshape(1, F).astype(F32), (DA - D, F)), 0.0).astype(BF)
    cp_wqkv.wait()
    cp_x(0).wait()
    wt = wraw[...].T
    wT[0:D, :] = _to_perm(ps0, wt[0:D].astype(F32)).astype(BF)
    wT[D:D2, :] = _to_perm(ps1, wt[D:D2].astype(F32)).astype(BF)
    wT[D2:D3, :] = wt[D2:D3]

    def front(l, cs, x, first=False):
        ub = front_a(l, cs, x)
        front_c(front_b(l, cs, ub), ub, first)

    front(0, _cols(0, TB), xs[:, _cols(0, TB)].astype(F32), True)

    def p1(s, c):
        cp_x(s).wait()
        cp_w1(s - 1).wait()
        w1T[_cols(s - 1, W1C), :] = w1c[:, _cols(s - 1, W1C)].T
        front(0, _cols(s, TB), xs[:, _cols(s, TB)].astype(F32))
        return c

    lax.fori_loop(1, NB, p1, 0)

    def step_2(s, first=False):
        cs = _cols(s, T)
        cn = _cols(s + 1, T)
        pqn = back_a(0, cn)
        if not first:
            y = y2_s[:, cs]
            h2 = f_pre(y, cs, 2)
        x1, yn, rs12 = back_b(xs[:, cn].astype(F32), pqn)
        if not first:
            o = oacc[...] + f_out(hcar[...], 1)
            h3 = f_pre(y, cs, 3)
            o = o + f_out(h2, 2)
        y2_s[:, cn] = yn
        stat[2:3, cn] = rs12
        h0n = f_pre(yn, cn, 0)
        if not first:
            x2 = o + f_out(h3, 3)
            stream[:, cs] = x2
            ub = front_a(1, cs, x2)
        hcar[...] = f_pre(yn, cn, 1)
        if not first:
            pkb = front_b(1, cs, ub)
        oacc[...] = x1 + b2col[...] + f_out(h0n, 0)
        if not first:
            front_c(pkb, ub)

    cp_wo.wait()
    cp_w2.wait()
    ff_c(0, ff_b(0, ff_a(0)))
    step_2(-1, first=True)

    def p2(s, carry):
        j = pl.ds(pl.multiple_of(jnp.minimum(s, 11) * 384, 384), 384)
        w2c[j, :] = w2T[:, j].T
        step_2(s)
        return carry

    lax.fori_loop(0, NT_ - 1, p2, 0)

    cp_g.wait()
    cl = _cols(NT_ - 1, T)
    c0 = _cols(0, T)
    y = y2_s[:, cl]
    gn = gs[:, c0]
    h2 = f_pre(y, cl, 2)
    o = oacc[...] + f_out(hcar[...], 1)
    h3 = f_pre(y, cl, 3)
    o = o + f_out(h2, 2)
    x2 = o + f_out(h3, 3)
    stream[:, cl] = x2
    ub = front_a(1, cl, x2)
    FE = FQ // 2
    dhe = []

    def fill_dh():
        e = len(dhe)
        dhe.append(_dot(w2c[e * FE:(e + 1) * FE, :], gn))

    fill_dh()
    pkb = front_b(1, cl, ub)
    front_c(pkb, ub)
    ct = ff_a(1)
    fill_dh()
    kvs = ff_b(1, ct)
    ff_c(1, kvs)
    fill_dh()
    x3, yn, rs12 = back_b(stream[:, c0], back_a(1, c0))
    y4_s[:, c0] = yn
    stat[3:4, c0] = rs12
    fill_dh()
    hn, gpn = gelu_bwd(m_pre(yn, 0))
    dpren = (jnp.concatenate(dhe, axis=0) * gpn).astype(BF)
    oacc[...] = x3 + b2col[...] + m_out(hn, 0)
    dyacc[...] = m_dy(dpren, 0)
    m_w1(yn, dpren, 0, False)
    m_w2(gn, hn, 0, False)

    def p3(s, carry):
        j = pl.ds(pl.multiple_of(jnp.minimum(s, 8) * 128, 128), 128)
        wx[:, j] = wT[j, :].T
        cs = _cols(s, T)
        cn = _cols(s + 1, T)
        gb = gs[:, cs]
        gn = gs[:, cn]
        pqn = back_a(1, cn)
        dh = m_dh(gb, 1)
        x3, yn, rs12 = back_b(stream[:, cn], pqn)
        hh, gp = gelu_bwd(m_pre(y4_s[:, cs], 1))
        y4_s[:, cn] = yn
        stat[3:4, cn] = rs12
        dpre = (dh * gp).astype(BF)
        dy = dyacc[...] + m_dy(dpre, 1)
        g = gb.astype(F32)
        db2a[...] += g
        g3 = g + _ln2_bwd(dy, y4_s[0:D, cs].astype(F32), stat[3:4, cs])
        stream[:, cs] = g3
        xs[:, cs] = (oacc[...] + m_out(hh, 1)).astype(BF)
        m_w1(y4_s[:, cs], dpre, 1, s > 0)
        m_w2(gb, hh, 1, s > 0)
        dhn = m_dh(gn, 0)
        g3b, dpqn = bwd1_a(1, g3)
        hn, gpn = gelu_bwd(m_pre(yn, 0))
        dpren = (dhn * gpn).astype(BF)
        bwd1_b(1, cs, g3b, dpqn)
        dyacc[...] = m_dy(dpren, 0)
        oacc[...] = x3 + b2col[...] + m_out(hn, 0)
        m_w1(yn, dpren, 0)
        m_w2(gn, hn, 0)
        return carry

    lax.fori_loop(0, NT_ - 1, p3, 0)

    cp_out = pltpu.make_async_copy(xs, out_hbm.at[0], sem_out.at[0])
    gb = gs[:, cl]
    y = y4_s[:, cl]
    hh, gp = gelu_bwd(m_pre(y, 1))
    dh = m_dh(gb, 1)
    dpre = (dh * gp).astype(BF)
    dy = dyacc[...] + m_dy(dpre, 1)
    g = gb.astype(F32)
    db2a[...] += g
    g3 = g + _ln2_bwd(dy, y[0:D].astype(F32), stat[3:4, cl])
    stream[:, cl] = g3
    xs[:, cl] = (oacc[...] + m_out(hh, 1)).astype(BF)
    g3b, dpqn = bwd1_a(1, g3)
    m_wq(dw1a, y, dpre, 2)
    bwd1_b(1, cl, g3b, dpqn)
    pb = bf_a(1)
    m_wq(dw1a, y, dpre, 3)
    bf_c(1, bf_b(1, pb))
    m_wq(dw2Ta, gb, hh, 2)
    dk = bwd2_a(1, c0)
    m_wq(dw2Ta, gb, hh, 3)
    g2n = bwd2_b(1, c0, dk)
    gn = g2n.astype(BF)
    db2a[...] += g2n
    gs[:, c0] = gn
    stream[:, c0] = g2n
    hn, gpn = gelu_bwd(pre2[hs(0), c0].astype(F32))
    dhn = m_dh(gn, 0)
    dpren = (dhn * gpn).astype(BF)
    m_w2(gn, hn, 0)
    dyacc[...] = m_dy(dpren, 0)
    m_w1(y2_s[:, c0], dpren, 0)
    cp_out.start()

    def p4(s, carry):
        cs = _cols(s, T)
        cn = _cols(s + 1, T)
        dk = bwd2_a(1, cn)
        dh = m_dh(gs[:, cs], 1)
        g2n = bwd2_b(1, cn, dk)
        hh, gp = gelu_bwd(pre2[hs(1), cs].astype(F32))
        dpre = (dh * gp).astype(BF)
        m_w2(gs[:, cs], hh, 1)
        gn = g2n.astype(BF)
        db2a[...] += g2n
        gs[:, cn] = gn
        stream[:, cn] = g2n
        y = y2_s[:, cs]
        dy = dyacc[...] + m_dy(dpre, 1)
        g1 = stream[:, cs] + _ln2_bwd(dy, y[0:D].astype(F32), stat[2:3, cs])
        stream[:, cs] = g1
        m_w1(y, dpre, 1)
        dhn = m_dh(gn, 0)
        hn, gpn = gelu_bwd(pre2[hs(0), cn].astype(F32))
        dpren = (dhn * gpn).astype(BF)
        g1b, dpqn = bwd1_a(0, g1)
        m_w2(gn, hn, 0)
        bwd1_b(0, cs, g1b, dpqn)
        dyacc[...] = m_dy(dpren, 0)
        m_w1(y2_s[:, cn], dpren, 0)
        return carry

    lax.fori_loop(0, NT_ - 1, p4, 0)

    w1c[0:D, hs(0)] = dw1a[0:D, hs(0)].astype(BF)
    w2T[:, hs(0)] = dw2Ta[:, hs(0)].astype(BF)
    gb = gs[:, cl]
    y = y2_s[:, cl]
    dh = m_dh(gb, 1)
    hh, gp = gelu_bwd(pre2[hs(1), cl].astype(F32))
    dpre = (dh * gp).astype(BF)
    m_wq(dw2Ta, gb, hh, 2)
    dy = dyacc[...] + m_dy(dpre, 1)
    g1 = stream[:, cl] + _ln2_bwd(dy, y[0:D].astype(F32), stat[2:3, cl])
    stream[:, cl] = g1
    m_wq(dw2Ta, gb, hh, 3)
    g1b, dpqn = bwd1_a(0, g1)
    m_wq(dw1a, y, dpre, 2)
    bwd1_b(0, cl, g1b, dpqn)
    pb = bf_a(0)
    m_wq(dw1a, y, dpre, 3)
    bf_c(0, bf_b(0, pb))
    dw2Ta[:, 0:D2] = _dot_nt(u_s[1, 0:D, 0:TB], qk_s[1, 0:D2, 0:TB])
    b1v[...] = dw1a[D:D + 1, :].astype(BF).reshape(F)
    b2v[...] = jnp.sum(db2a[...].T, axis=0, keepdims=True).astype(BF).reshape(D)
    wo[...] = dwo_a[...].astype(BF)
    cp_dw1a = pltpu.make_async_copy(w1c.at[pl.ds(0, D), hs(0)], dw1_hbm.at[:, hs(0)], sem_out.at[1])
    cp_dw2a = pltpu.make_async_copy(w2T.at[:, hs(0)], dw2_hbm.at[:, hs(0)], sem_out.at[2])
    cp_db1 = pltpu.make_async_copy(b1v, db1_hbm, sem_out.at[3])
    cp_db2 = pltpu.make_async_copy(b2v, db2_hbm, sem_out.at[4])
    cp_dwo = pltpu.make_async_copy(wo, dwo_hbm, sem_out.at[5])
    cp_dwqkv = pltpu.make_async_copy(wraw, dwqkv_hbm, sem_out.at[6])
    cp_dw1a.start()
    cp_dw2a.start()
    cp_db1.start()
    cp_db2.start()
    cp_dwo.start()
    o3 = 7
    RQ = D // NB

    def cp_dx(s):
        return pltpu.make_async_copy(gs.at[:, _cols(s, TB)], dx_hbm.at[0, :, _cols(s, TB)], sem_out.at[o3 + s])

    def cp_dw1b(s):
        return pltpu.make_async_copy(w1c.at[_cols(s, RQ), hs(1)], dw1_hbm.at[_cols(s, RQ), hs(1)],
                                     sem_out.at[o3 + NB + s])

    def cp_dw2b(s):
        return pltpu.make_async_copy(w2T.at[_cols(s, RQ), hs(1)], dw2_hbm.at[_cols(s, RQ), hs(1)],
                                     sem_out.at[o3 + 2 * NB + s])

    def p5a(s, carry):
        cs = _cols(s, TB)
        ks = pl.ds(pl.multiple_of(TB + s * 384, 128), 384)
        w1c[_cols(s, RQ), hs(1)] = dw1a[_cols(s, RQ), hs(1)].astype(BF)
        w2T[_cols(s, RQ), hs(1)] = dw2Ta[_cols(s, RQ), hs(1)].astype(BF)
        dk = bwd2_a(0, cs)
        dw2Ta[:, 0:D2] += _dot_nt(u_s[1, 0:D, ks], qk_s[1, 0:D2, ks])
        dw2Ta[:, 0:D2] += _dot_nt(u_s[0, 0:D, cs], jnp.concatenate([qk_s[0, 0:D, cs], dk], axis=0))
        cp_dw1b(s).start()
        cp_dw2b(s).start()
        return carry

    lax.fori_loop(0, NB, p5a, 0)

    def dx_tile(s):
        for k in range(TB // T):
            if isinstance(s, int):
                cs = pl.ds(s * TB + k * T, T)
            else:
                cs = pl.ds(pl.multiple_of(s * TB + k * T, T), T)
            gs[:, cs] = bwd2_b(0, cs).astype(BF)
        cp_dx(s).start()

    dwt = dw2Ta[:, 0:D2].astype(BF).T.astype(F32)
    dwq = _from_perm(ps0, dwt[0:D]).astype(BF)
    dwk = _from_perm(ps1, dwt[D:D2]).astype(BF)
    wraw[...] = jnp.concatenate([dwq, dwk, dwv_a[...].astype(BF)], axis=0).T
    dx_tile(0)
    cp_dwqkv.start()

    def p5b(s, carry):
        dx_tile(s)
        return carry

    lax.fori_loop(1, NB, p5b, 0)

    cp_out.wait()
    cp_dw1a.wait()
    cp_dw2a.wait()
    cp_db1.wait()
    cp_db2.wait()
    cp_dwo.wait()
    cp_dwqkv.wait()
    for s in range(NB):
        cp_dw1b(s).wait()
        cp_dw2b(s).wait()
    for s in range(NB):
        cp_dx(s).wait()


@jax.jit
def pallas_interleave_layers__linear_attn_block__mixer_channel_mlp__prompt_kernel(
    A_x: jax.Array,
    A_wqkv: jax.Array,
    A_wo: jax.Array,
    B_x: jax.Array,
    B_w1: jax.Array,
    B_b1: jax.Array,
    B_w2: jax.Array,
    B_b2: jax.Array,
    grad_out: jax.Array,
):
    del B_x
    V = pltpu.VMEM
    n_in = NB + 6 + 3
    n_out = 7 + 3 * NB
    scratch = [
        V((D, S), BF),
        V((D, S), BF),
        V((D, D3), BF),
        V((D, D3), BF),
        V((D3, D), BF),
        V((D, D), BF),
        V((DA, F), BF),
        V((F, DA), BF),
        V((F, D), BF),
        V((D, F), BF),
        V((F,), BF),
        V((D,), BF),
        V((D, 128), F32),
        V((DA, F), F32),
        V((D, F), F32),
        V((F, S), BF),
        V((D, S), F32),
        V((2, DA, S), BF),
        V((2, D3, S), BF),
        V((2, H, S), F32),
        V((DA, S), BF),
        V((DA, S), BF),
        V((8, S), F32),
        V((D, T), F32),
        V((D, T), F32),
        V((FQ, T), BF),
        V((2, NG, 128, 128), BF),
        V((D, DA), F32),
        V((2, D, D), BF),
        V((2, D, 128), F32),
        V((2, D, D), BF),
        V((D, D), BF),
        V((D, DR), F32),
        V((D, DA), BF),
        V((D, D), F32),
        V((D, D), F32),
        V((D, 128), F32),
        V((5, D, 128), F32),
        V((5, D, 128), F32),
        pltpu.SemaphoreType.DMA((n_in,)),
        pltpu.SemaphoreType.DMA((n_out,)),
    ]
    any_spec = pl.BlockSpec(memory_space=pl.ANY)
    out_shape = (
        jax.ShapeDtypeStruct((1, D, S), BF),
        jax.ShapeDtypeStruct((1, D, S), BF),
        jax.ShapeDtypeStruct((D, D3), BF),
        jax.ShapeDtypeStruct((D, D), BF),
        jax.ShapeDtypeStruct((D, F), BF),
        jax.ShapeDtypeStruct((F,), BF),
        jax.ShapeDtypeStruct((D, F), BF),
        jax.ShapeDtypeStruct((D,), BF),
    )
    outT, dxT, dwqkv, dwo, dw1, db1, dw2T, db2 = pl.pallas_call(
        _kernel,
        out_shape=out_shape,
        in_specs=[any_spec] * 8,
        out_specs=tuple([any_spec] * 8),
        scratch_shapes=scratch,
        compiler_params=pltpu.CompilerParams(vmem_limit_bytes=127 * 1024 * 1024),
    )(jnp.swapaxes(A_x, 1, 2), A_wqkv, A_wo, B_w1, B_b1, B_w2.T, B_b2, jnp.swapaxes(grad_out, 1, 2))
    return (jnp.swapaxes(outT, 1, 2), jnp.swapaxes(dxT, 1, 2), dwqkv, dwo, dw1, db1, dw2T.T, db2)
```

```python
import jax
import jax.numpy as jnp
from jax import lax
import jax.experimental.pallas as pl
import jax.experimental.pallas.tpu as pltpu

S, D, F = 2048, 576, 4608
H, DH = 32, 18
D3 = 3 * D
DA = 592
T = 128
NT_ = S // T
TB = 512
NB = S // TB
FH = F // 2
FQ = F // 4
D2 = 2 * D
DR = D + H
QA = 512
W1C = F // 3
NG = 5
WSTEP = 112
HEAD_LO = (0, 7, 13, 19, 25)
HEAD_HI = (6, 12, 18, 24, 31)

LN_EPS = 1e-5
PHI_EPS = 1e-6
GC0 = 0.7978845608028654
GC1 = 0.044715

BF = jnp.bfloat16


def on(name):
    return True


F32 = jnp.float32
U32 = jnp.uint32
_NN = (((1,), (0,)), ((), ()))
_NT = (((1,), (1,)), ((), ()))


def _dot(a, b):
    return lax.dot_general(a, b, _NN, preferred_element_type=F32)


def _dot_nt(a, b):
    return lax.dot_general(a, b, _NT, preferred_element_type=F32)


def _colmean(x):
    n = x.shape[1]
    p = jnp.sum(x.reshape(9, 64, n), axis=0)
    p = p[0:32] + p[32:64]
    p = p[0:16] + p[16:32]
    p = p[0:8] + p[8:16]
    return jnp.sum(p, axis=0, keepdims=True) * (1.0 / D)


def _ln(x):
    m = _colmean(x)
    xc = x - m
    v = _colmean(xc * xc)
    rs = lax.rsqrt(v + LN_EPS)
    return xc * rs, rs


def _ln_bwd(dy, y, rs):
    a = _colmean(dy)
    b = _colmean(dy * y)
    return (dy - a - y * b) * rs


CR = 8
NCH = D // CR


def _fold(p):
    while p.shape[0] > 8:
        h = p.shape[0] // 2
        p = p[0:h] + p[h:2 * h]
    return jnp.sum(p, axis=0, keepdims=True) * (1.0 / D)


def _ch(x, c):
    return x[c * CR:(c + 1) * CR]


PR = 32


def _b8(c, rows=PR):
    return jnp.broadcast_to(c, (rows, c.shape[1]))


def _pace(c, v):
    return c + 0.0 * v[0:1]


def _ln2(x):
    acc = _ch(x, 0)
    for c in range(1, NCH):
        acc = acc + _ch(x, c)
    m = _fold(acc)
    a1 = a2 = None
    for c in range(NCH):
        xc = _ch(x, c) - m
        a1 = xc if a1 is None else a1 + xc
        a2 = xc * xc if a2 is None else a2 + xc * xc
    s1 = _fold(a1)
    s2 = _fold(a2)
    rs1 = lax.rsqrt(s2 + LN_EPS)
    m2 = s1 * rs1
    v2 = s2 * rs1 * rs1 - m2 * m2
    rs2 = lax.rsqrt(v2 + LN_EPS)
    rs12 = rs1 * rs2
    mc = _pace(m + s1, rs12)
    out = []
    for c in range(D // PR):
        y = (x[PR * c:PR * c + PR] - mc) * rs12
        mc = _pace(mc, y)
        out.append(y.astype(BF))
    return jnp.concatenate(out, axis=0), rs12


def _ln2_bwd(g, dy, y, rs12, k=1.0 + LN_EPS):
    a1 = a2 = None
    y = y.astype(F32)
    for c in range(NCH):
        d = _ch(dy, c)
        t = d * _ch(y, c)
        a1 = d if a1 is None else a1 + d
        a2 = t if a2 is None else a2 + t
    t = g + dy * rs12
    a = _fold(a1) * rs12
    b = _fold(a2) * (k * rs12)
    out = []
    for c in range(D // PR):
        o = (t[PR * c:PR * c + PR] - y[PR * c:PR * c + PR] * b) - a
        b = _pace(b, o)
        out.append(o)
    return jnp.concatenate(out, axis=0)


def _lnp(x):
    acc = _ch(x, 0)
    for c in range(1, NCH):
        acc = acc + _ch(x, c)
    m = _fold(acc)
    a2 = None
    for c in range(NCH):
        xc = _ch(x, c) - m
        a2 = xc * xc if a2 is None else a2 + xc * xc
    rs = lax.rsqrt(_fold(a2) + LN_EPS)
    mc = _pace(m, rs)
    out = []
    for c in range(D // PR):
        y = (x[PR * c:PR * c + PR] - mc) * rs
        mc = _pace(mc, y)
        out.append(y.astype(BF))
    return jnp.concatenate(out, axis=0), rs


def _headsum(x):
    n = x.shape[1]
    p = x.reshape(DH, H, n)
    p = p[0:9] + p[9:18]
    q = (p[0] + p[1]) + (p[2] + p[3])
    r = (p[4] + p[5]) + (p[6] + p[7])
    return (q + r) + p[8]


def _headmul(x, c):
    n = x.shape[1]
    return (x.reshape(DH, H, n) * c[None]).reshape(D, n)


_LT = ((0, 128), (128, 128), (256, 128), (384, 128), (512, 64))


def _to_perm(scr, val):
    for c, (o, w) in enumerate(_LT):
        scr[c, :, 0:w] = val[:, o:o + w]
    return jnp.concatenate(
        [jnp.concatenate([scr[c, pl.ds(j, H, stride=DH), 0:w] for c, (o, w) in enumerate(_LT)], axis=1)
         for j in range(DH)], axis=0)


def _from_perm(scr, val):
    for j in range(DH):
        for c, (o, w) in enumerate(_LT):
            scr[c, pl.ds(j, H, stride=DH), 0:w] = val[H * j:H * j + H, o:o + w]
    return jnp.concatenate([scr[c, :, 0:w] for c, (o, w) in enumerate(_LT)], axis=1)


class _Pk:
    def __init__(self, ref):
        self.ref = ref

    def _idx(self, idx):
        nd = len(self.ref.shape)
        if idx is Ellipsis:
            return idx
        if not isinstance(idx, tuple):
            idx = (idx,)
        idx = list(idx) + [slice(None)] * (nd - len(idx))
        r = idx[nd - 2]
        if isinstance(r, slice):
            if r.start is not None or r.stop is not None:
                r = slice(r.start // 2, r.stop // 2)
        elif isinstance(r.start, int):
            r = pl.ds(r.start // 2, r.size // 2)
        else:
            r = pl.ds(pl.multiple_of(r.start // 2, 8), r.size // 2)
        idx[nd - 2] = r
        return tuple(idx)

    def __getitem__(self, idx):
        return pltpu.bitcast(self.ref[self._idx(idx)], BF)

    def __setitem__(self, idx, val):
        self.ref[self._idx(idx)] = pltpu.bitcast(val, U32)


def _aug(y):
    r = lax.broadcasted_iota(jnp.int32, (DA - D, y.shape[1]), 0)
    return jnp.concatenate([y.astype(BF), jnp.where(r < 2, 1.0, 0.0).astype(BF)], axis=0)


def _phi(t):
    return jnp.where(t > 0, t + 1.0, jnp.exp(t)) + PHI_EPS


def _dphi_from_phi(p):
    return jnp.minimum(p - PHI_EPS, 1.0)


def _win(x, g):
    return x[WSTEP * g:WSTEP * g + 128]


def _assemble(parts):
    pieces = [parts[0][:WSTEP]]
    for g in range(NG - 1):
        pieces.append(parts[g][WSTEP:128] + parts[g + 1][0:16])
        pieces.append(parts[g + 1][16:WSTEP] if g + 1 < NG - 1 else parts[g + 1][16:128])
    return jnp.concatenate(pieces, axis=0)


def _head_mask(g):
    r = lax.broadcasted_iota(jnp.int32, (128, 128), 0) + WSTEP * g
    c = lax.broadcasted_iota(jnp.int32, (128, 128), 1) + WSTEP * g
    hr = (r * 3641) >> 16
    hc = (c * 3641) >> 16
    return (hr == hc) & (hr >= HEAD_LO[g]) & (hr <= HEAD_HI[g])


def _lane_fold(x):
    acc = x[:, 0:128]
    for j in range(1, x.shape[1] // 128):
        acc = acc + x[:, 128 * j:128 * (j + 1)]
    return acc


def _lane_tile(x128, n):
    if n == 128:
        return x128
    return jnp.concatenate([x128] * (n // 128), axis=1)


def _gelu_parts(pre):
    x2 = pre * pre
    t = jnp.tanh(pre * (GC0 + (GC0 * GC1) * x2))
    hp = 0.5 + 0.5 * t
    return x2, t, hp


def _cols(s, n):
    if isinstance(s, int):
        return pl.ds(s * n, n)
    return pl.ds(pl.multiple_of(s * n, n), n)


def _kernel(
    x_hbm, wqkv_hbm, wo_hbm, w1_hbm, b1_hbm, w2_hbm, b2_hbm, g_hbm,
    out_hbm, dx_hbm, dwqkv_hbm, dwo_hbm, dw1_hbm, db1_hbm, dw2_hbm, db2_hbm,
    xs, gs, wraw, wx, wT, wo, w1c, w1T, w2c, w2T, b1v, b2v, b2col,
    dw1a, dw2Ta, pre2, stream, u_s, qk_s, rd_s, y2_s, y4_s, stat,
    oacc, dyacc, hcar,
    kvT, cacc, ctb, zb, mm, mmT, pacc, dctb, dwv_a, dwo_a, db2a, ps0, ps1,
    sem_in, sem_out,
):
    wx, wT, w1T, w2c, pre2, u_s, qk_s, hcar, kvT, ctb, mm, mmT, dctb = [
        _Pk(r) for r in (wx, wT, w1T, w2c, pre2, u_s, qk_s, hcar, kvT, ctb, mm, mmT, dctb)]

    def cp_x(s):
        return pltpu.make_async_copy(x_hbm.at[0, :, _cols(s, TB)], xs.at[:, _cols(s, TB)], sem_in.at[s])

    k0 = NB
    cp_wqkv = pltpu.make_async_copy(wqkv_hbm, wraw, sem_in.at[k0])
    cp_wo = pltpu.make_async_copy(wo_hbm, wo, sem_in.at[k0 + 1])
    cp_b1 = pltpu.make_async_copy(b1_hbm, b1v, sem_in.at[k0 + 2])
    cp_b2 = pltpu.make_async_copy(b2_hbm, b2v, sem_in.at[k0 + 3])
    cp_w2 = pltpu.make_async_copy(w2_hbm, w2T, sem_in.at[k0 + 4])
    cp_g = pltpu.make_async_copy(g_hbm.at[0], gs, sem_in.at[k0 + 5])
    k1 = k0 + 6

    def cp_w1(c):
        return pltpu.make_async_copy(w1_hbm.at[:, _cols(c, W1C)], w1c.at[pl.ds(0, D), _cols(c, W1C)],
                                     sem_in.at[k1 + c])

    cp_wqkv.start()
    cp_x(0).start()
    cp_b1.start()
    cp_b2.start()
    for s in range(1, NB):
        cp_x(s).start()
        cp_w1(s - 1).start()
    cp_wo.start()
    cp_w2.start()
    cp_g.start()

    def wrow(ref, g, base=0):
        return ref[base + WSTEP * g:base + WSTEP * g + 128, :]

    def front_a(l, cs, x):
        u, rs = _lnp(x) if x.shape[1] == T else _ln(x)
        ub = _aug(u)
        u_s[l, :, cs] = ub
        stat[l:l + 1, cs] = rs
        return ub

    def front_b(l, cs, ub):
        pkb = _phi(_dot(wT[D:D2, :], ub[0:D])).astype(BF)
        qk_s[l, D2:D3, cs] = pkb
        qk_s[l, 0:D, cs] = _phi(_dot(wT[0:D, :], ub[0:D])).astype(BF)
        return pkb

    def front_c(pkb, ub, first=False):
        c = _dot_nt(pkb, ub)
        if first:
            cacc[...] = c
        else:
            cacc[...] += c

    def ff_a(l):
        c = cacc[...]
        zb[l] = jnp.broadcast_to(c[:, D:D + 1], (D, 128))
        ct = _from_perm(ps0, c[:, 0:D]).astype(BF)
        ctb[l] = ct
        if l == 0:
            cacc[...] = jnp.zeros_like(cacc)
        return ct

    def ff_b(l, ct):
        kvs = []
        for g in range(NG):
            kv = jnp.where(_head_mask(g), _dot_nt(_win(ct, g), wrow(wT, g, D2)), 0.0)
            kvT[l, g] = kv.T.astype(BF)
            kvs.append(kv.astype(BF))
        return kvs

    def ff_c(l, kvs):
        m = _assemble([_dot(kvs[g], wrow(wo, g)) for g in range(NG)])
        mp = _to_perm(ps1, m).astype(BF)
        mm[l] = mp
        mmT[...] = mp.T

    def back_a(l, cs):
        pq = qk_s[l, 0:D, cs].astype(F32)
        rden = 1.0 / (_headsum(pq * zb[l]) + PHI_EPS)
        rd_s[l, :, cs] = rden
        return _headmul(pq, rden).astype(BF)

    def back_b(x, pqn):
        x1 = x + _dot(mmT[...], pqn)
        y, rs12 = _ln2(x1)
        return x1, _aug(y), rs12

    def bwd1_a(l, g):
        gb = g.astype(BF)
        return gb, _dot(mm[l], gb)

    def bwd1_b(l, cs, gb, dpqn):
        pq = qk_s[l, 0:D, cs].astype(F32)
        rden = rd_s[l, :, cs]
        z = zb[l]
        rd = rden
        r = None
        pqn, w = [], []
        for j in range(DH):
            pj = pq[H * j:H * j + H]
            t = pj * rd
            pqn.append(t.astype(BF))
            w.append(_dphi_from_phi(pj) * rd)
            t = dpqn[H * j:H * j + H] * t
            r = t if r is None else r + t
            rd = _pace(rden, r)
        rb = r.astype(BF)
        dq = []
        for j in range(DH):
            t = (dpqn[H * j:H * j + H] - z[H * j:H * j + H] * r) * w[j]
            r = _pace(r, t)
            dq.append(t.astype(BF))
        qk_s[l, 0:D, cs] = jnp.concatenate(dq, axis=0)
        pacc[...] += _dot_nt(jnp.concatenate(pqn, axis=0), jnp.concatenate([gb, rb], axis=0))

    def bf_a(l):
        p = pacc[...]
        tl = p[:, 512:DR]
        rr = lax.broadcasted_iota(jnp.int32, tl.shape, 0)
        cc = lax.broadcasted_iota(jnp.int32, tl.shape, 1)
        dz = -jnp.sum(jnp.where(cc - (D - 512) == (rr & (H - 1)), tl, 0.0), axis=1, keepdims=True)
        hi = dz.astype(BF).astype(F32)
        ce = lax.broadcasted_iota(jnp.int32, (D, DA - D), 1)
        dctb[:, D:DA] = jnp.where(ce == 0, hi, jnp.where(ce == 1, dz - hi, 0.0)).astype(BF)
        pb = _from_perm(ps0, p[:, 0:D]).astype(BF)
        if l == 1:
            pacc[...] = jnp.zeros_like(pacc)
        return pb

    def acc_l(ref, l, val):
        if l == 1:
            ref[...] = val
        else:
            ref[...] += val

    def bf_b(l, pb):
        ds_ = [jnp.where(_head_mask(g), _dot_nt(_win(pb, g), wrow(wo, g)), 0.0) for g in range(NG)]
        acc_l(dwo_a, l, _assemble([_dot(kvT[l, g], _win(pb, g)) for g in range(NG)]))
        return ds_

    def bf_c(l, ds_):
        dct = _assemble([_dot(ds_[g].astype(BF), wrow(wT, g, D2)) for g in range(NG)])
        dp = _to_perm(ps1, dct).astype(BF)
        dctb[:, 0:D] = dp
        wx[:, D2:D3] = dp.T
        acc_l(dwv_a, l, _assemble([_dot(ds_[g].T.astype(BF), ctb[l, WSTEP * g:WSTEP * g + 128, :]) for g in range(NG)]))

    def bwd2_a(l, cs):
        dpk = _dot(dctb[...], u_s[l, :, cs])
        dk = (dpk * _dphi_from_phi(qk_s[l, D2:D3, cs].astype(F32))).astype(BF)
        qk_s[l, D:D2, cs] = dk
        return dk

    def bwd2_b(l, cs, dk=None):
        if dk is None:
            rhs = qk_s[l, :, cs]
        else:
            rhs = jnp.concatenate([qk_s[l, 0:D, cs], dk, qk_s[l, D2:D3, cs]], axis=0)
        du = _dot(wx[...], rhs)
        return _ln2_bwd(stream[:, cs], du, u_s[l, 0:D, cs], stat[l:l + 1, cs], 1.0)

    def hs(h):
        return pl.ds(h * FH, FH)

    def qs(c):
        return pl.ds(c * FQ, FQ)

    def f_pre(y, cs, c):
        pre = _dot(w1T[qs(c), :], y)
        pre2[qs(c), cs] = pre.astype(BF)
        _, _, hp = _gelu_parts(pre)
        return (pre * hp).astype(BF)

    def f_out(hh, c):
        return _dot(w2T[:, qs(c)], hh)

    def gelu_bwd(pre):
        x2, t, hp = _gelu_parts(pre)
        hh = (pre * hp).astype(BF)
        gp = hp + (0.5 * pre) * (1.0 - t * t) * (GC0 + (3.0 * GC0 * GC1) * x2)
        return hh, gp

    def gelu_bwd_p(h, cs):
        GR = 64
        hs_, gs_ = [], []
        k = jnp.full((1, T), GC0, F32)
        for c in range(FH // GR):
            pre = pre2[h * FH + c * GR:h * FH + (c + 1) * GR, cs].astype(F32)
            x2 = pre * pre
            t = jnp.tanh(pre * (k + (GC0 * GC1) * x2))
            k = _pace(k, t)
            hp = 0.5 + 0.5 * t
            hs_.append((pre * hp).astype(BF))
            gs_.append(hp + (0.5 * pre) * (1.0 - t * t) * (GC0 + (3.0 * GC0 * GC1) * x2))
        return jnp.concatenate(hs_, axis=0), jnp.concatenate(gs_, axis=0)

    def m_dh(gb, h):
        return _dot(w2c[hs(h), :], gb)

    def m_dhq(gb, c):
        return _dot(w2c[qs(c), :], gb)

    def m_pre(y, h):
        return _dot(w1T[hs(h), :], y)

    def m_dy(dpre, h):
        return _dot(w1c[0:D, hs(h)], dpre)

    def m_out(hh, h):
        return _dot(w2T[:, hs(h)], hh)

    def acc_to(ref, sl, val, keep):
        if keep is True:
            ref[:, sl] += val
        elif keep is False:
            ref[:, sl] = val
        else:
            ref[:, sl] = jnp.where(keep, ref[:, sl], 0.0) + val

    def m_w1(y, dpre, h, keep=True):
        acc_to(dw1a, hs(h), _dot_nt(y, dpre), keep)

    def m_w2(gb, hh, h, keep=True):
        acc_to(dw2Ta, hs(h), _dot_nt(gb, hh), keep)

    def m_wq(ref, a, b, c):
        acc_to(ref, qs(c), _dot_nt(a, b[(c - 2) * FQ:(c - 1) * FQ]), True)

    pacc[...] = jnp.zeros_like(pacc)
    db2a[...] = jnp.zeros_like(db2a)
    cp_b1.wait()
    cp_b2.wait()
    b2col[...] = jnp.broadcast_to(b2v[...].reshape(1, D).astype(F32), (128, D)).T
    rid = lax.broadcasted_iota(jnp.int32, (DA - D, F), 0)
    w1c[D:DA, :] = jnp.where(
        rid == 0, jnp.broadcast_to(b1v[...].reshape(1, F).astype(F32), (DA - D, F)), 0.0).astype(BF)
    cp_wqkv.wait()
    cp_x(0).wait()
    if on('b0'):
        wt = wraw[...].T
        wT[0:D, :] = _to_perm(ps0, wt[0:D].astype(F32)).astype(BF)
        wT[D:D2, :] = _to_perm(ps1, wt[D:D2].astype(F32)).astype(BF)
        wT[D2:D3, :] = wt[D2:D3]

    def front(l, cs, x, first=False):
        ub = front_a(l, cs, x)
        front_c(front_b(l, cs, ub), ub, first)

    if on('b0'):
        front(0, _cols(0, TB), xs[:, _cols(0, TB)].astype(F32), True)

    def p1(s, c):
        cp_x(s).wait()
        cp_w1(s - 1).wait()
        w1T[_cols(s - 1, W1C), :] = w1c[:, _cols(s - 1, W1C)].T
        front(0, _cols(s, TB), xs[:, _cols(s, TB)].astype(F32))
        return c

    if on('p1'):
        lax.fori_loop(1, NB, p1, 0)
    else:
        for s in range(1, NB):
            cp_x(s).wait()
            cp_w1(s - 1).wait()

    def step_2(s, first=False):
        cs = _cols(s, T)
        cn = _cols(s + 1, T)
        pqn = back_a(0, cn)
        if not first:
            y = y2_s[:, cs]
            h2 = f_pre(y, cs, 2)
        x1, yn, rs12 = back_b(xs[:, cn].astype(F32), pqn)
        if not first:
            o = oacc[...] + f_out(hcar[...], 1)
            h3 = f_pre(y, cs, 3)
            o = o + f_out(h2, 2)
        y2_s[:, cn] = yn
        stat[2:3, cn] = rs12
        h0n = f_pre(yn, cn, 0)
        if not first:
            x2 = o + f_out(h3, 3)
            stream[:, cs] = x2
            ub = front_a(1, cs, x2)
        hcar[...] = f_pre(yn, cn, 1)
        oacc[...] = x1 + b2col[...] + f_out(h0n, 0)
        if not first:
            front_c(front_b(1, cs, ub), ub)

    cp_wo.wait()
    cp_w2.wait()
    if on('b1'):
        ff_c(0, ff_b(0, ff_a(0)))
        step_2(-1, first=True)

    def p2(s, carry):
        j = pl.ds(pl.multiple_of(jnp.minimum(s, 11) * 384, 384), 384)
        w2c[j, :] = w2T[:, j].T
        step_2(s)
        return carry

    if on('p2'):
        lax.fori_loop(0, NT_ - 1, p2, 0)

    cp_g.wait()
    cl = _cols(NT_ - 1, T)
    c0 = _cols(0, T)
    if on('b2'):
        y = y2_s[:, cl]
        gn = gs[:, c0]
        h2 = f_pre(y, cl, 2)
        o = oacc[...] + f_out(hcar[...], 1)
        h3 = f_pre(y, cl, 3)
        o = o + f_out(h2, 2)
        x2 = o + f_out(h3, 3)
        stream[:, cl] = x2
        ub = front_a(1, cl, x2)
        FE = FQ // 2
        dhe = []

        def fill_dh():
            e = len(dhe)
            dhe.append(_dot(w2c[e * FE:(e + 1) * FE, :], gn))

        fill_dh()
        pkb = front_b(1, cl, ub)
        front_c(pkb, ub)
        ct = ff_a(1)
        fill_dh()
        kvs = ff_b(1, ct)
        ff_c(1, kvs)
        fill_dh()
        x3, yn, rs12 = back_b(stream[:, c0], back_a(1, c0))
        y4_s[:, c0] = yn
        stat[3:4, c0] = rs12
        fill_dh()
        hn, gpn = gelu_bwd(m_pre(yn, 0))
        dpren = (jnp.concatenate(dhe, axis=0) * gpn).astype(BF)
        oacc[...] = x3 + b2col[...] + m_out(hn, 0)
        dyacc[...] = m_dy(dpren, 0)
        m_w1(yn, dpren, 0, False)
        m_w2(gn, hn, 0, False)

    def p3(s, carry):
        j = pl.ds(pl.multiple_of(jnp.minimum(s, 8) * 128, 128), 128)
        wx[:, j] = wT[j, :].T
        cs = _cols(s, T)
        cn = _cols(s + 1, T)
        gb = gs[:, cs]
        gn = gs[:, cn]
        pqn = back_a(1, cn)
        dh = m_dh(gb, 1)
        x3, yn, rs12 = back_b(stream[:, cn], pqn)
        hh, gp = gelu_bwd(m_pre(y4_s[:, cs], 1))
        y4_s[:, cn] = yn
        stat[3:4, cn] = rs12
        dpre = (dh * gp).astype(BF)
        dy = dyacc[...] + m_dy(dpre, 1)
        g = gb.astype(F32)
        db2a[...] += g
        g3 = _ln2_bwd(g, dy, y4_s[0:D, cs], stat[3:4, cs])
        stream[:, cs] = g3
        xs[:, cs] = (oacc[...] + m_out(hh, 1)).astype(BF)
        m_w1(y4_s[:, cs], dpre, 1, s > 0)
        m_w2(gb, hh, 1, s > 0)
        dhn = m_dh(gn, 0)
        g3b, dpqn = bwd1_a(1, g3)
        hn, gpn = gelu_bwd(m_pre(yn, 0))
        dpren = (dhn * gpn).astype(BF)
        bwd1_b(1, cs, g3b, dpqn)
        dyacc[...] = m_dy(dpren, 0)
        oacc[...] = x3 + b2col[...] + m_out(hn, 0)
        m_w1(yn, dpren, 0)
        m_w2(gn, hn, 0)
        return carry

    if on('p3'):
        lax.fori_loop(0, NT_ - 1, p3, 0)

    cp_out = pltpu.make_async_copy(xs, out_hbm.at[0], sem_out.at[0])
    if on('b3'):
        gb = gs[:, cl]
        y = y4_s[:, cl]
        hh, gp = gelu_bwd(m_pre(y, 1))
        dh = m_dh(gb, 1)
        dpre = (dh * gp).astype(BF)
        dy = dyacc[...] + m_dy(dpre, 1)
        g = gb.astype(F32)
        db2a[...] += g
        g3 = _ln2_bwd(g, dy, y[0:D], stat[3:4, cl])
        stream[:, cl] = g3
        xs[:, cl] = (oacc[...] + m_out(hh, 1)).astype(BF)
        g3b, dpqn = bwd1_a(1, g3)
        m_wq(dw1a, y, dpre, 2)
        bwd1_b(1, cl, g3b, dpqn)
        pb = bf_a(1)
        m_wq(dw1a, y, dpre, 3)
        bf_c(1, bf_b(1, pb))
        m_wq(dw2Ta, gb, hh, 2)
        dk = bwd2_a(1, c0)
        m_wq(dw2Ta, gb, hh, 3)
        g2n = bwd2_b(1, c0, dk)
        gn = g2n.astype(BF)
        gs[:, c0] = gn
        stream[:, c0] = g2n
        hn, gpn = gelu_bwd(pre2[hs(0), c0].astype(F32))
        dhn = m_dh(gn, 0)
        dpren = (dhn * gpn).astype(BF)
        m_w2(gn, hn, 0)
        dyacc[...] = m_dy(dpren, 0)
        m_w1(y2_s[:, c0], dpren, 0)
    cp_out.start()

    def p4(s, carry):
        cs = _cols(s, T)
        cn = _cols(s + 1, T)
        dk = bwd2_a(1, cn)
        gb = gs[:, cs]
        dh = m_dh(gb, 1)
        db2a[...] += gb.astype(F32)
        g2n = bwd2_b(1, cn, dk)
        hh, gp = gelu_bwd_p(1, cs)
        dpre = (dh * gp).astype(BF)
        m_w2(gb, hh, 1)
        gn = g2n.astype(BF)
        gs[:, cn] = gn
        stream[:, cn] = g2n
        y = y2_s[:, cs]
        dy = dyacc[...] + m_dy(dpre, 1)
        g1 = _ln2_bwd(stream[:, cs], dy, y[0:D], stat[2:3, cs])
        stream[:, cs] = g1
        m_w1(y, dpre, 1)
        dhn = m_dh(gn, 0)
        hn, gpn = gelu_bwd_p(0, cn)
        dpren = (dhn * gpn).astype(BF)
        g1b, dpqn = bwd1_a(0, g1)
        m_w2(gn, hn, 0)
        bwd1_b(0, cs, g1b, dpqn)
        dyacc[...] = m_dy(dpren, 0)
        m_w1(y2_s[:, cn], dpren, 0)
        return carry

    if on('p4'):
        lax.fori_loop(0, NT_ - 1, p4, 0)

    if on('b4'):
        w1c[0:D, hs(0)] = dw1a[0:D, hs(0)].astype(BF)
        w2T[:, hs(0)] = dw2Ta[:, hs(0)].astype(BF)
        gb = gs[:, cl]
        y = y2_s[:, cl]
        db2a[...] += gb.astype(F32)
        dh = m_dh(gb, 1)
        hh, gp = gelu_bwd(pre2[hs(1), cl].astype(F32))
        dpre = (dh * gp).astype(BF)
        m_wq(dw2Ta, gb, hh, 2)
        dy = dyacc[...] + m_dy(dpre, 1)
        g1 = _ln2_bwd(stream[:, cl], dy, y[0:D], stat[2:3, cl])
        stream[:, cl] = g1
        m_wq(dw2Ta, gb, hh, 3)
        g1b, dpqn = bwd1_a(0, g1)
        m_wq(dw1a, y, dpre, 2)
        bwd1_b(0, cl, g1b, dpqn)
        pb = bf_a(0)
        m_wq(dw1a, y, dpre, 3)
        bf_c(0, bf_b(0, pb))
        dw2Ta[:, 0:D2] = _dot_nt(u_s[1, 0:D, 0:TB], qk_s[1, 0:D2, 0:TB])
        b1v[...] = dw1a[D:D + 1, :].astype(BF).reshape(F)
        b2v[...] = jnp.sum(db2a[...].T, axis=0, keepdims=True).astype(BF).reshape(D)
        wo[...] = dwo_a[...].astype(BF)
    cp_dw1a = pltpu.make_async_copy(w1c.at[pl.ds(0, D), hs(0)], dw1_hbm.at[:, hs(0)], sem_out.at[1])
    cp_dw2a = pltpu.make_async_copy(w2T.at[:, hs(0)], dw2_hbm.at[:, hs(0)], sem_out.at[2])
    cp_db1 = pltpu.make_async_copy(b1v, db1_hbm, sem_out.at[3])
    cp_db2 = pltpu.make_async_copy(b2v, db2_hbm, sem_out.at[4])
    cp_dwo = pltpu.make_async_copy(wo, dwo_hbm, sem_out.at[5])
    cp_dwqkv = pltpu.make_async_copy(wraw, dwqkv_hbm, sem_out.at[6])
    cp_dw1a.start()
    cp_dw2a.start()
    cp_db1.start()
    cp_db2.start()
    cp_dwo.start()
    o3 = 7
    RQ = D // NB

    def cp_dx(s):
        return pltpu.make_async_copy(gs.at[:, _cols(s, TB)], dx_hbm.at[0, :, _cols(s, TB)], sem_out.at[o3 + s])

    def cp_dw1b(s):
        return pltpu.make_async_copy(w1c.at[_cols(s, RQ), hs(1)], dw1_hbm.at[_cols(s, RQ), hs(1)],
                                     sem_out.at[o3 + NB + s])

    def cp_dw2b(s):
        return pltpu.make_async_copy(w2T.at[_cols(s, RQ), hs(1)], dw2_hbm.at[_cols(s, RQ), hs(1)],
                                     sem_out.at[o3 + 2 * NB + s])

    def p5a(s, carry):
        cs = _cols(s, TB)
        ks = pl.ds(pl.multiple_of(TB + s * 384, 128), 384)
        w1c[_cols(s, RQ), hs(1)] = dw1a[_cols(s, RQ), hs(1)].astype(BF)
        w2T[_cols(s, RQ), hs(1)] = dw2Ta[_cols(s, RQ), hs(1)].astype(BF)
        dk = bwd2_a(0, cs)
        dw2Ta[:, 0:D2] += _dot_nt(u_s[1, 0:D, ks], qk_s[1, 0:D2, ks])
        dw2Ta[:, 0:D2] += _dot_nt(u_s[0, 0:D, cs], jnp.concatenate([qk_s[0, 0:D, cs], dk], axis=0))
        cp_dw1b(s).start()
        cp_dw2b(s).start()
        return carry

    if on('p5a'):
        lax.fori_loop(0, NB, p5a, 0)
    else:
        for s in range(NB):
            cp_dw1b(s).start()
            cp_dw2b(s).start()

    def dx_tile(s):
        for k in range(TB // T):
            if isinstance(s, int):
                cs = pl.ds(s * TB + k * T, T)
            else:
                cs = pl.ds(pl.multiple_of(s * TB + k * T, T), T)
            gs[:, cs] = bwd2_b(0, cs).astype(BF)
        cp_dx(s).start()

    if on('b5'):
        dwt = dw2Ta[:, 0:D2].astype(BF).T.astype(F32)
        dwq = _from_perm(ps0, dwt[0:D]).astype(BF)
        dwk = _from_perm(ps1, dwt[D:D2]).astype(BF)
        wraw[...] = jnp.concatenate([dwq, dwk, dwv_a[...].astype(BF)], axis=0).T
        dx_tile(0)
    else:
        cp_dx(0).start()
    cp_dwqkv.start()

    def p5b(s, carry):
        dx_tile(s)
        return carry

    if on('p5b'):
        lax.fori_loop(1, NB, p5b, 0)
    else:
        for s in range(1, NB):
            cp_dx(s).start()

    cp_out.wait()
    cp_dw1a.wait()
    cp_dw2a.wait()
    cp_db1.wait()
    cp_db2.wait()
    cp_dwo.wait()
    cp_dwqkv.wait()
    for s in range(NB):
        cp_dw1b(s).wait()
        cp_dw2b(s).wait()
    for s in range(NB):
        cp_dx(s).wait()


@jax.jit
def pallas_interleave_layers__linear_attn_block__mixer_channel_mlp__prompt_kernel(
    A_x: jax.Array,
    A_wqkv: jax.Array,
    A_wo: jax.Array,
    B_x: jax.Array,
    B_w1: jax.Array,
    B_b1: jax.Array,
    B_w2: jax.Array,
    B_b2: jax.Array,
    grad_out: jax.Array,
):
    del B_x
    V = pltpu.VMEM
    n_in = NB + 6 + 3
    n_out = 7 + 3 * NB
    scratch = [
        V((D, S), BF),
        V((D, S), BF),
        V((D, D3), BF),
        V((D // 2, D3), U32),
        V((D3 // 2, D), U32),
        V((D, D), BF),
        V((DA, F), BF),
        V((F // 2, DA), U32),
        V((F // 2, D), U32),
        V((D, F), BF),
        V((F,), BF),
        V((D,), BF),
        V((D, 128), F32),
        V((DA, F), F32),
        V((D, F), F32),
        V((F // 2, S), U32),
        V((D, S), F32),
        V((2, DA // 2, S), U32),
        V((2, D3 // 2, S), U32),
        V((2, H, S), F32),
        V((DA, S), BF),
        V((DA, S), BF),
        V((8, S), F32),
        V((D, T), F32),
        V((D, T), F32),
        V((FQ // 2, T), U32),
        V((2, NG, 64, 128), U32),
        V((D, DA), F32),
        V((2, D // 2, D), U32),
        V((2, D, 128), F32),
        V((2, D // 2, D), U32),
        V((D // 2, D), U32),
        V((D, DR), F32),
        V((D // 2, DA), U32),
        V((D, D), F32),
        V((D, D), F32),
        V((D, 128), F32),
        V((5, D, 128), F32),
        V((5, D, 128), F32),
        pltpu.SemaphoreType.DMA((n_in,)),
        pltpu.SemaphoreType.DMA((n_out,)),
    ]
    any_spec = pl.BlockSpec(memory_space=pl.ANY)
    out_shape = (
        jax.ShapeDtypeStruct((1, D, S), BF),
        jax.ShapeDtypeStruct((1, D, S), BF),
        jax.ShapeDtypeStruct((D, D3), BF),
        jax.ShapeDtypeStruct((D, D), BF),
        jax.ShapeDtypeStruct((D, F), BF),
        jax.ShapeDtypeStruct((F,), BF),
        jax.ShapeDtypeStruct((D, F), BF),
        jax.ShapeDtypeStruct((D,), BF),
    )
    outT, dxT, dwqkv, dwo, dw1, db1, dw2T, db2 = pl.pallas_call(
        _kernel,
        out_shape=out_shape,
        in_specs=[any_spec] * 8,
        out_specs=tuple([any_spec] * 8),
        scratch_shapes=scratch,
        compiler_params=pltpu.CompilerParams(vmem_limit_bytes=127 * 1024 * 1024),
    )(jnp.swapaxes(A_x, 1, 2), A_wqkv, A_wo, B_w1, B_b1, B_w2.T, B_b2, jnp.swapaxes(grad_out, 1, 2))
    return (jnp.swapaxes(outT, 1, 2), jnp.swapaxes(dxT, 1, 2), dwqkv, dwo, dw1, db1, dw2T.T, db2)
```

```python
import jax
import jax.numpy as jnp
from jax import lax
import jax.experimental.pallas as pl
import jax.experimental.pallas.tpu as pltpu

S, D, F = 2048, 576, 4608
H, DH = 32, 18
D3 = 3 * D
DA = 592
T = 128
NT_ = S // T
TB = 512
NB = S // TB
FH = F // 2
FQ = F // 4
D2 = 2 * D
DR = D + H
QA = 512
W1C = F // 3
NG = 5
WSTEP = 112
HEAD_LO = (0, 7, 13, 19, 25)
HEAD_HI = (6, 12, 18, 24, 31)

R3 = ()
R4 = ()
LN_EPS = 1e-5
PHI_EPS = 1e-6
GC0 = 0.7978845608028654
GC1 = 0.044715

BF = jnp.bfloat16


def on(name):
    return True


F32 = jnp.float32
U32 = jnp.uint32
_NN = (((1,), (0,)), ((), ()))
_NT = (((1,), (1,)), ((), ()))


def _dot(a, b):
    return lax.dot_general(a, b, _NN, preferred_element_type=F32)


def _dot_nt(a, b):
    return lax.dot_general(a, b, _NT, preferred_element_type=F32)


def _rows(m, nt):
    p = {1: 4, 2: 2}[nt % 4]
    return [slice(m // p * i, m // p * (i + 1)) for i in range(p)]


def _dot5(a, b, split, head=False):
    k = a.shape[1]
    nt = (k + 127) // 128
    if not split or nt % 4 == 0:
        return _dot(a, b)
    if head:
        odd, main = slice(0, nt % 4 * 128), slice(nt % 4 * 128, k)
    else:
        odd, main = slice(nt // 4 * 512, k), slice(0, nt // 4 * 512)
    tail = [_dot(a[r, odd], b[odd]) for r in _rows(a.shape[0], nt)]
    return _dot(a[:, main], b[main]) + jnp.concatenate(tail, axis=0)


def _dot5_nt(a, b):
    n = b.shape[0]
    nt = (n + 127) // 128
    n0 = nt // 4 * 512
    main = _dot_nt(a, b[0:n0])
    tail = [_dot_nt(a[r], b[n0:n]) for r in _rows(a.shape[0], nt)]
    return jnp.concatenate([main, jnp.concatenate(tail, axis=0)], axis=1)


def _colmean(x):
    n = x.shape[1]
    p = jnp.sum(x.reshape(9, 64, n), axis=0)
    p = p[0:32] + p[32:64]
    p = p[0:16] + p[16:32]
    p = p[0:8] + p[8:16]
    return jnp.sum(p, axis=0, keepdims=True) * (1.0 / D)


def _ln(x):
    m = _colmean(x)
    xc = x - m
    v = _colmean(xc * xc)
    rs = lax.rsqrt(v + LN_EPS)
    return xc * rs, rs


def _ln_bwd(dy, y, rs):
    a = _colmean(dy)
    b = _colmean(dy * y)
    return (dy - a - y * b) * rs


CR = 8
NCH = D // CR


def _fold(p):
    while p.shape[0] > 8:
        h = p.shape[0] // 2
        p = p[0:h] + p[h:2 * h]
    return jnp.sum(p, axis=0, keepdims=True) * (1.0 / D)


def _ch(x, c):
    return x[c * CR:(c + 1) * CR]


PR = 32


_PO = (16, 17) + tuple(range(16))


def _cat(out):
    return jnp.concatenate(out[2:] + out[:2], axis=0)


def _b8(c, rows=PR):
    return jnp.broadcast_to(c, (rows, c.shape[1]))


def _pace(c, v):
    return c + 0.0 * v[0:1]


def _ln2(x, ld):
    acc = _ch(x, 0)
    for c in range(1, NCH):
        acc = acc + _ch(x, c)
    m = _fold(acc)
    a1 = a2 = None
    x = ld(0)
    for c in range(NCH):
        xc = _ch(x, c) - m
        a1 = xc if a1 is None else a1 + xc
        a2 = xc * xc if a2 is None else a2 + xc * xc
    s1 = _fold(a1)
    s2 = _fold(a2)
    rs1 = lax.rsqrt(s2 + LN_EPS)
    m2 = s1 * rs1
    v2 = s2 * rs1 * rs1 - m2 * m2
    rs2 = lax.rsqrt(v2 + LN_EPS)
    rs12 = rs1 * rs2
    mc = _pace(m + s1, rs12)
    out = []
    x = ld(1)
    for c in _PO:
        y = (x[PR * c:PR * c + PR] - mc) * rs12
        mc = _pace(mc, y)
        out.append(y.astype(BF))
    return _cat(out), rs12


def _ln2_bwd(g, dy, y, rs12, home, k=1.0 + LN_EPS, keep=True):
    st, ld_t, ld_y = home
    a1 = a2 = None
    y = y.astype(F32)
    for c in range(NCH):
        d = _ch(dy, c)
        t = d * _ch(y, c)
        a1 = d if a1 is None else a1 + d
        a2 = t if a2 is None else a2 + t
    t = g + dy * rs12
    if ld_t is None:
        ld_t, ld_y = (lambda r: t[r]), (lambda r: y[r])
    else:
        st(slice(0, D), t)
    a = _fold(a1) * rs12
    b = _fold(a2) * (k * rs12)
    out = []
    for c in _PO:
        r = slice(PR * c, PR * c + PR)
        o = (ld_t(r) - ld_y(r).astype(F32) * b) - a
        b = _pace(b, o)
        if keep:
            st(r, o)
        out.append(o.astype(BF))
    return _cat(out)


def _lnp(x, link=None, ld=None):
    acc = _ch(x, 0)
    if link is not None:
        acc = acc + 0.0 * link
    for c in range(1, NCH):
        acc = acc + _ch(x, c)
    m = _fold(acc)
    a2 = None
    if ld is not None:
        x = ld(0)
    for c in range(NCH):
        xc = _ch(x, c) - m
        a2 = xc * xc if a2 is None else a2 + xc * xc
    rs = lax.rsqrt(_fold(a2) + LN_EPS)
    mc = _pace(m, rs)
    out = []
    if ld is not None:
        x = ld(1)
    for c in _PO:
        y = (x[PR * c:PR * c + PR] - mc) * rs
        mc = _pace(mc, y)
        out.append(y.astype(BF))
    return _cat(out), rs, jnp.minimum(jnp.abs(y[0:1]), 1.0)


def _headsum(x):
    n = x.shape[1]
    p = x.reshape(DH, H, n)
    p = p[0:9] + p[9:18]
    q = (p[0] + p[1]) + (p[2] + p[3])
    r = (p[4] + p[5]) + (p[6] + p[7])
    return (q + r) + p[8]


def _headmul(x, c):
    n = x.shape[1]
    return (x.reshape(DH, H, n) * c[None]).reshape(D, n)


_LT = ((0, 128), (128, 128), (256, 128), (384, 128), (512, 64))


def _to_perm(scr, val):
    for c, (o, w) in enumerate(_LT):
        scr[c, :, 0:w] = val[:, o:o + w]
    return jnp.concatenate(
        [jnp.concatenate([scr[c, pl.ds(j, H, stride=DH), 0:w] for c, (o, w) in enumerate(_LT)], axis=1)
         for j in range(DH)], axis=0)


def _from_perm(scr, val):
    for j in range(DH):
        for c, (o, w) in enumerate(_LT):
            scr[c, pl.ds(j, H, stride=DH), 0:w] = val[H * j:H * j + H, o:o + w]
    return jnp.concatenate([scr[c, :, 0:w] for c, (o, w) in enumerate(_LT)], axis=1)


class _Pk:
    def __init__(self, ref):
        self.ref = ref

    def _idx(self, idx):
        nd = len(self.ref.shape)
        if idx is Ellipsis:
            return idx
        if not isinstance(idx, tuple):
            idx = (idx,)
        idx = list(idx) + [slice(None)] * (nd - len(idx))
        r = idx[nd - 2]
        if isinstance(r, slice):
            if r.start is not None or r.stop is not None:
                r = slice(r.start // 2, r.stop // 2)
        elif isinstance(r.start, int):
            r = pl.ds(r.start // 2, r.size // 2)
        else:
            r = pl.ds(pl.multiple_of(r.start // 2, 8), r.size // 2)
        idx[nd - 2] = r
        return tuple(idx)

    def __getitem__(self, idx):
        return pltpu.bitcast(self.ref[self._idx(idx)], BF)

    def __setitem__(self, idx, val):
        self.ref[self._idx(idx)] = pltpu.bitcast(val, U32)


class _L2:
    def __init__(self, a, b):
        self.r = (a, b)

    def __getitem__(self, idx):
        return self.r[idx[0]][idx[1:]]

    def __setitem__(self, idx, val):
        self.r[idx[0]][idx[1:]] = val


def _aug(y):
    r = lax.broadcasted_iota(jnp.int32, (DA - D, y.shape[1]), 0)
    return jnp.concatenate([y.astype(BF), jnp.where(r < 2, 1.0, 0.0).astype(BF)], axis=0)


def _phi(t):
    return jnp.where(t > 0, t + 1.0, jnp.exp(t)) + PHI_EPS


def _dphi_from_phi(p):
    return jnp.minimum(p - PHI_EPS, 1.0)


def _win(x, g):
    return x[WSTEP * g:WSTEP * g + 128]


def _assemble(parts):
    pieces = [parts[0][:WSTEP]]
    for g in range(NG - 1):
        pieces.append(parts[g][WSTEP:128] + parts[g + 1][0:16])
        pieces.append(parts[g + 1][16:WSTEP] if g + 1 < NG - 1 else parts[g + 1][16:128])
    return jnp.concatenate(pieces, axis=0)


def _head_mask(g):
    r = lax.broadcasted_iota(jnp.int32, (128, 128), 0) + WSTEP * g
    c = lax.broadcasted_iota(jnp.int32, (128, 128), 1) + WSTEP * g
    hr = (r * 3641) >> 16
    hc = (c * 3641) >> 16
    return (hr == hc) & (hr >= HEAD_LO[g]) & (hr <= HEAD_HI[g])


def _lane_fold(x):
    acc = x[:, 0:128]
    for j in range(1, x.shape[1] // 128):
        acc = acc + x[:, 128 * j:128 * (j + 1)]
    return acc


def _lane_tile(x128, n):
    if n == 128:
        return x128
    return jnp.concatenate([x128] * (n // 128), axis=1)


def _gelu_parts(pre):
    x2 = pre * pre
    t = jnp.tanh(pre * (GC0 + (GC0 * GC1) * x2))
    hp = 0.5 + 0.5 * t
    return x2, t, hp


def _cols(s, n):
    if isinstance(s, int):
        return pl.ds(s * n, n)
    return pl.ds(pl.multiple_of(s * n, n), n)


def _kernel(
    x_hbm, wqkv_hbm, wo_hbm, w1_hbm, b1_hbm, w2_hbm, b2_hbm, g_hbm,
    out_hbm, dx_hbm, dwqkv_hbm, dwo_hbm, dw1_hbm, db1_hbm, dw2_hbm, db2_hbm,
    xs, gs, wraw, wx, wT, wo, w1c, w1T, w2c, w2T, b1v, b2v, b2col,
    dw1a, dw2Ta, pre2, stream, u_0, u_1, qk_0, qk_1, rd_0, rd_1, y2_s, y4_s, stat, db1a, dbrow,
    oacc, dyacc, hcar,
    kvT, cacc, ctb, zb, mm, mmT, pacc, dctb, dwv_a, dwo_a, db2a, ps0, ps1, dtmp, zs,
    sem_in, sem_out,
):
    wx, wT, w1T, w2c, pre2, hcar, kvT, ctb, mm, mmT, dctb = [
        _Pk(r) for r in (wx, wT, w1T, w2c, pre2, hcar, kvT, ctb, mm, mmT, dctb)]
    u_s = _L2(_Pk(u_0), _Pk(u_1))
    qk_s = _L2(_Pk(qk_0), _Pk(qk_1))
    rd_s = _L2(rd_0, rd_1)

    ALLR = (0, 1, 2, 3, 4)
    env = {'r': ALLR}

    def zero(k):
        if k not in env['r']:
            return 0
        return env['z'] >> (20 + k)

    def _alt(cs, k):
        if k not in env['r']:
            return cs
        return pl.ds(pl.multiple_of(cs.start + (zero(k) << 7), 128), cs.size)

    def home(cs, yref):
        def st(r, v):
            stream[r, cs] = v
        if 3 not in env['r']:
            return st, None, None
        return st, (lambda r: stream[r, _alt(cs, 3)]), (lambda r: yref[r, _alt(cs, 3)])

    zs[0] = 0

    def cp_x(s):
        return pltpu.make_async_copy(x_hbm.at[0, :, _cols(s, TB)], xs.at[:, _cols(s, TB)], sem_in.at[s])

    k0 = NB
    def cp_wpart(lo, hi, k):
        return pltpu.make_async_copy(wqkv_hbm.at[:, pl.ds(lo, hi - lo)], wraw.at[:, pl.ds(lo, hi - lo)], sem_in.at[k])

    cp_wk = cp_wpart(512, D2, k0)
    cp_wq = cp_wpart(0, 512, k0 + 9)
    cp_wv = cp_wpart(D2, D3, k0 + 10)
    cp_wo = pltpu.make_async_copy(wo_hbm, wo, sem_in.at[k0 + 1])
    cp_b1 = pltpu.make_async_copy(b1_hbm, b1v, sem_in.at[k0 + 2])
    cp_b2 = pltpu.make_async_copy(b2_hbm, b2v, sem_in.at[k0 + 3])
    cp_w2 = pltpu.make_async_copy(w2_hbm, w2T, sem_in.at[k0 + 4])
    cp_g = pltpu.make_async_copy(g_hbm.at[0], gs, sem_in.at[k0 + 5])
    k1 = k0 + 6

    def cp_w1(c):
        return pltpu.make_async_copy(w1_hbm.at[:, _cols(c, W1C)], w1c.at[pl.ds(0, D), _cols(c, W1C)],
                                     sem_in.at[k1 + c])

    cp_x(0).start()
    cp_wk.start()
    cp_wq.start()
    cp_x(1).start()
    cp_b1.start()
    cp_b2.start()
    cp_wv.start()
    cp_x(2).start()
    cp_x(3).start()
    for s in range(3):
        cp_w1(s).start()
    cp_wo.start()
    cp_w2.start()
    cp_g.start()

    def wrow(ref, g, base=0):
        return ref[base + WSTEP * g:base + WSTEP * g + 128, :]

    def front_a(l, cs, x, link=None):
        u, rs, lk = _lnp(x, link, (lambda k: stream[:, _alt(cs, k)]) if l == 1 else None)
        ub = _aug(u)
        u_s[l, :, cs] = ub
        stat[l:l + 1, cs] = rs
        return ub if link is None else lk

    def front_k(l, cs, ub):
        pkb = _phi(_dot5(wT[D:D2, :], ub[0:D], True)).astype(BF)
        qk_s[l, D2:D3, cs] = pkb
        return pkb

    def front_q(l, cs, ub):
        qk_s[l, 0:D, cs] = _phi(_dot5(wT[0:D, :], ub[0:D], True)).astype(BF)

    def front_b(l, cs, ub):
        pkb = front_k(l, cs, ub)
        front_q(l, cs, ub)
        return pkb

    def front_c(pkb, ub, first=False):
        if pkb.shape[1] == T:
            for m in range(4):
                cacc[144 * m:144 * m + 144, 512:DA] += _dot_nt(pkb[144 * m:144 * m + 144], ub[512:DA])
            cacc[:, 0:512] += _dot_nt(pkb, ub[0:512])
            return
        c = _dot_nt(pkb, ub)
        if first:
            cacc[...] = c
        else:
            cacc[...] += c

    def ff_a(l):
        c = cacc[...]
        zb[l] = jnp.broadcast_to(c[:, D:D + 1], (D, 128))
        ct = _from_perm(ps0, c[:, 0:D]).astype(BF)
        ctb[l] = ct
        if l == 0:
            cacc[...] = jnp.zeros_like(cacc)
        return ct

    def ff_b(l, ct):
        kvs = []
        for g in range(NG):
            kv = jnp.where(_head_mask(g), _dot_nt(_win(ct, g), wrow(wT, g, D2)), 0.0)
            kvT[l, g] = kv.T.astype(BF)
            kvs.append(kv.astype(BF))
        return kvs

    def ff_c(l, kvs):
        m = _assemble([_dot(kvs[g], wrow(wo, g)) for g in range(NG)])
        mp = _to_perm(ps1, m).astype(BF)
        mm[l] = mp
        mmT[...] = mp.T

    def back_a(l, cs):
        pq = qk_s[l, 0:D, cs].astype(F32)
        rden = 1.0 / (_headsum(pq * zb[l]) + PHI_EPS)
        rd_s[l, :, cs] = rden
        return _headmul(pq, rden).astype(BF)

    def back_b(x, cs, pqn, split=False):
        x1 = x + _dot5(mmT[...], pqn, split)
        env['x'] = x1
        if 0 in env['r']:
            stream[:, cs] = x1
            y, rs12 = _ln2(x1, lambda k: stream[:, _alt(cs, k)])
        else:
            y, rs12 = _ln2(x1, lambda k: x1)
        return _aug(y), rs12

    def res(cs):
        return (stream[:, _alt(cs, 2)] if 0 in env['r'] else env['x']) + b2col[...]

    def bwd1_a(l, gb, split=False):
        return gb, _dot5(mm[l], gb, split)

    def bwd1_b(l, cs, gb, dpqn, split=False):
        pq = qk_s[l, 0:D, cs].astype(F32)
        rden = rd_s[l, :, cs]
        z = zb[l]
        rd = rden
        r = None
        pqn = []
        rl = 4 in env['r']
        if rl:
            dtmp[0] = dpqn
        for j in range(DH):
            t = pq[H * j:H * j + H] * rd
            pqn.append(t.astype(BF))
            t = dpqn[H * j:H * j + H] * t
            r = t if r is None else r + t
            rd = _pace(rden, r)
        rb = r.astype(BF)
        for j in range(DH):
            rj = slice(H * j, H * j + H)
            w = _dphi_from_phi(qk_s[l, rj, _alt(cs, 4)].astype(F32) if rl else pq[rj]) * rden
            t = ((dtmp[zero(4), rj, :] if rl else dpqn[rj]) - z[rj] * r) * w
            r = _pace(r, t)
            qk_s[l, rj, cs] = t.astype(BF)
        pqn = jnp.concatenate(pqn, axis=0)
        gr = jnp.concatenate([gb, rb], axis=0)
        if split:
            pacc[:, 0:512] += _dot_nt(pqn, gr[0:512])
            for m in range(4):
                pacc[144 * m:144 * m + 144, 512:DR] += _dot_nt(pqn[144 * m:144 * m + 144], gr[512:DR])
        else:
            pacc[...] += _dot_nt(pqn, gr)

    def bf_a(l):
        p = pacc[...]
        tl = p[:, 512:DR]
        rr = lax.broadcasted_iota(jnp.int32, tl.shape, 0)
        cc = lax.broadcasted_iota(jnp.int32, tl.shape, 1)
        dz = -jnp.sum(jnp.where(cc - (D - 512) == (rr & (H - 1)), tl, 0.0), axis=1, keepdims=True)
        hi = dz.astype(BF).astype(F32)
        ce = lax.broadcasted_iota(jnp.int32, (D, DA - D), 1)
        dctb[:, D:DA] = jnp.where(ce == 0, hi, jnp.where(ce == 1, dz - hi, 0.0)).astype(BF)
        pb = _from_perm(ps0, p[:, 0:D]).astype(BF)
        if l == 1:
            pacc[...] = jnp.zeros_like(pacc)
        return pb

    def acc_l(ref, l, val):
        if l == 1:
            ref[...] = val
        else:
            ref[...] += val

    def bf_b(l, pb):
        ds_ = [jnp.where(_head_mask(g), _dot_nt(_win(pb, g), wrow(wo, g)), 0.0) for g in range(NG)]
        acc_l(dwo_a, l, _assemble([_dot(kvT[l, g], _win(pb, g)) for g in range(NG)]))
        return ds_

    def bf_c(l, ds_):
        dct = _assemble([_dot(ds_[g].astype(BF), wrow(wT, g, D2)) for g in range(NG)])
        dp = _to_perm(ps1, dct).astype(BF)
        dctb[:, 0:D] = dp
        wx[:, D2:D3] = dp.T
        acc_l(dwv_a, l, _assemble([_dot(ds_[g].T.astype(BF), ctb[l, WSTEP * g:WSTEP * g + 128, :]) for g in range(NG)]))

    def bwd2_a(l, cs, split=False):
        dpk = _dot5(dctb[...], u_s[l, :, cs], split)
        dk = (dpk * _dphi_from_phi(qk_s[l, D2:D3, cs].astype(F32))).astype(BF)
        qk_s[l, D:D2, cs] = dk
        return dk

    def bwd2_b(l, cs, dk=None, keep=True, bal=False):
        if dk is None:
            rhs = qk_s[l, :, cs]
        else:
            rhs = jnp.concatenate([qk_s[l, 0:D, cs], dk, qk_s[l, D2:D3, cs]], axis=0)
        du = _dot5(wx[...], rhs, bal)
        return _ln2_bwd(stream[:, cs], du, u_s[l, 0:D, cs], stat[l:l + 1, cs], home(cs, u_s.r[l]), 1.0, keep)

    def hs(h):
        return pl.ds(h * FH, FH)

    def qs(c):
        return pl.ds(c * FQ, FQ)

    def f_pre(y, cs, c):
        pre = _dot5(w1T[qs(c), :], y, True)
        pre2[qs(c), cs] = pre.astype(BF)
        _, _, hp = _gelu_parts(pre)
        return (pre * hp).astype(BF)

    def f_out(hh, c):
        return _dot5(w2T[:, qs(c)], hh, True, True)

    def gelu_bwd(pre):
        x2, t, hp = _gelu_parts(pre)
        hh = (pre * hp).astype(BF)
        gp = hp + (0.5 * pre) * (1.0 - t * t) * (GC0 + (3.0 * GC0 * GC1) * x2)
        return hh, gp

    def gelu_bwd_p(h, cs):
        GR = 64
        hs_, gs_ = [], []
        k = jnp.full((1, T), GC0, F32)
        for c in range(FH // GR):
            pre = pre2[h * FH + c * GR:h * FH + (c + 1) * GR, cs].astype(F32)
            x2 = pre * pre
            t = jnp.tanh(pre * (k + (GC0 * GC1) * x2))
            k = _pace(k, t)
            hp = 0.5 + 0.5 * t
            hs_.append((pre * hp).astype(BF))
            gs_.append(hp + (0.5 * pre) * (1.0 - t * t) * (GC0 + (3.0 * GC0 * GC1) * x2))
        return jnp.concatenate(hs_, axis=0), jnp.concatenate(gs_, axis=0)

    def m_dh(gb, h):
        return _dot5(w2c[hs(h), :], gb, True)

    def m_dhq(gb, c):
        return _dot(w2c[qs(c), :], gb)

    def m_pre(y, h):
        return _dot5(w1T[hs(h), :], y, True)

    def m_dy(dpre, h, bal=False):
        return _dot5(w1c[0:D, hs(h)], dpre, bal, True)

    def m_out(hh, h):
        return _dot(w2T[:, hs(h)], hh)

    def acc_to(ref, sl, val, keep):
        if keep is True:
            ref[:, sl] += val
        elif keep is False:
            ref[:, sl] = val
        else:
            ref[:, sl] = jnp.where(keep, ref[:, sl], 0.0) + val

    def m_w1(y, dpre, h, keep=True):
        acc_to(dw1a, hs(h), _dot_nt(y[0:D], dpre), keep)

    def mk_dpre(dh, gp, h):
        dp = dh * gp
        db1a[hs(h), :] += dp
        return dp.astype(BF)

    def m_w2(gb, hh, h, keep=True):
        acc_to(dw2Ta, hs(h), _dot_nt(gb, hh), keep)

    def m_wq(ref, a, b, c):
        acc_to(ref, qs(c), _dot5_nt(a, b[(c - 2) * FQ:(c - 1) * FQ]), True)

    def m_fin(dst, ref, a, b, sl):
        val = ref[:, sl] + _dot_nt(a, b)
        dst[0:D, sl] = val.astype(BF)

    def m_wq_fin(dst, ref, a, b, c):
        m_fin(dst, ref, a, b[(c - 2) * FQ:(c - 1) * FQ], qs(c))

    pacc[...] = jnp.zeros_like(pacc)
    db2a[...] = jnp.zeros_like(db2a)
    db1a[...] = jnp.zeros_like(db1a)

    def ln0(s, chain=4, lk=None):
        for k in range(TB // T):
            cs = pl.ds(s * TB + k * T, T)
            if k % chain == 0 and (k or lk is None):
                lk = jnp.zeros((1, T), F32)
            lk = front_a(0, cs, xs[:, cs].astype(F32), lk)
        return lk

    def k_part(s):
        cs = _cols(s, TB)
        qk_s[0, D2:D3, cs] = _phi(_dot(wT[D:D2, :], u_s[0, 0:D, cs])).astype(BF)

    def q_part(lo, hi):
        cs = pl.ds(lo * T, (hi - lo) * T)
        qk_s[0, 0:D, cs] = _phi(_dot(wT[0:D, :], u_s[0, 0:D, cs])).astype(BF)

    def c_part(s):
        cs = _cols(s, TB)
        front_c(qk_s[0, D2:D3, cs], u_s[0, :, cs], s == 0)

    def w1_t(c):
        w1T[_cols(c, W1C), :] = w1c[:, _cols(c, W1C)].T

    cp_x(0).wait()
    ln0(0, 2)
    cp_wk.wait()
    wtk = wraw[:, 512:D2].T
    wT[D:D2, :] = _to_perm(ps1, wtk[64:640].astype(F32)).astype(BF)
    k_part(0)
    cp_wq.wait()
    cp_x(1).wait()
    cp_b1.wait()
    cp_b2.wait()
    wtq = jnp.concatenate([wraw[:, 0:512].T, wtk[0:64]], axis=0)
    wT[0:D, :] = _to_perm(ps0, wtq.astype(F32)).astype(BF)
    c_part(0)
    b2col[...] = jnp.broadcast_to(b2v[...].reshape(1, D).astype(F32), (128, D)).T
    rid = lax.broadcasted_iota(jnp.int32, (DA - D, F), 0)
    w1c[D:DA, :] = jnp.where(
        rid == 0, jnp.broadcast_to(b1v[...].reshape(1, F).astype(F32), (DA - D, F)), 0.0).astype(BF)
    ln0(1)
    q_part(0, 4)
    k_part(1)
    c_part(1)
    cp_wv.wait()
    cp_x(2).wait()
    cp_x(3).wait()
    cp_w1(0).wait()
    cp_w1(1).wait()
    lk = ln0(2)
    q_part(4, 8)
    wT[D2:D3, :] = wraw[:, D2:D3].T
    w1_t(0)
    ln0(3, 4, lk)
    k_part(2)
    c_part(2)
    w1_t(1)
    k_part(3)
    q_part(8, 12)
    c_part(3)
    cp_w1(2).wait()
    cp_wo.wait()
    cp_w2.wait()

    def step_2(s, first=False, last=False):
        cs = _cols(s, T)
        cn = _cols(s + 1, T)
        pqn = back_a(0, cn)
        if not first:
            y = y2_s[:, cs]
            h2 = f_pre(y, cs, 2)
        yn, rs12 = back_b(xs[:, cn].astype(F32), cn, pqn, True)
        if first:
            q_part(15, 16)
        else:
            o = oacc[...] + f_out(hcar[...], 1)
            h3 = f_pre(y, cs, 3)
            o = o + f_out(h2, 2)
        y2_s[:, cn] = yn
        stat[2:3, cn] = rs12
        h0n = f_pre(yn, cn, 0)
        if not first:
            x2 = o + f_out(h3, 3)
            stream[:, cs] = x2
            ub = front_a(1, cs, x2)
        hcar[...] = f_pre(yn, cn, 1)
        if last:
            pkb = front_k(1, cs, ub)
        oacc[...] = res(cn) + f_out(h0n, 0)
        if last:
            front_c(pkb, ub)
        elif not first:
            front_c(front_b(1, cs, ub), ub)

    env['z'] = zs[0]
    if on('b1'):
        ct = ff_a(0)
        q_part(12, 13)
        ff_c(0, ff_b(0, ct))
        q_part(13, 15)
        w1_t(2)
        step_2(-1, first=True)

    def p2(s, carry):
        env['z'] = s
        j = pl.ds(pl.multiple_of(jnp.minimum(s, 11) * 384, 384), 384)
        w2c[j, :] = w2T[:, j].T
        step_2(s)
        return s

    if on('p2'):
        env['z'] = \
            lax.fori_loop(0, NT_ - 2, p2, 0)

    cp_g.wait()
    cl = _cols(NT_ - 1, T)
    c0 = _cols(0, T)
    if on('b2'):
        step_2(NT_ - 2, last=True)
        cp_ = _cols(NT_ - 2, T)
        y = y2_s[:, cl]
        gn = gs[:, c0]
        h2 = f_pre(y, cl, 2)
        o = oacc[...] + f_out(hcar[...], 1)
        h3 = f_pre(y, cl, 3)
        o = o + f_out(h2, 2)
        x2 = o + f_out(h3, 3)
        stream[:, cl] = x2
        ub = front_a(1, cl, x2)
        FE = FH // 8
        dhe = []

        def fill_dh(n):
            e = len(dhe)
            for i in range(e, e + n):
                dhe.append(_dot(w2c[i * FE:(i + 1) * FE, 0:512], gn[0:512]))

        front_q(1, cp_, u_s[1, :, cp_])
        fill_dh(1)
        pkb = front_k(1, cl, ub)
        fill_dh(1)
        front_c(pkb, ub)
        ct = ff_a(1)
        front_q(1, cl, ub)
        kvs = ff_b(1, ct)
        fill_dh(1)
        ff_c(1, kvs)
        dht = jnp.concatenate([_dot(w2c[r, 512:D], gn[512:D]) for r in _rows(FH, 1)], axis=0)
        fill_dh(1)
        yn, rs12 = back_b(stream[:, c0], c0, back_a(1, c0), True)
        y4_s[:, c0] = yn
        stat[3:4, c0] = rs12
        fill_dh(4)
        hn, gpn = gelu_bwd(m_pre(yn, 0))
        dpren = mk_dpre(jnp.concatenate(dhe, axis=0) + dht, gpn, 0)
        oacc[...] = res(c0) + m_out(hn, 0)
        dyacc[...] = m_dy(dpren, 0)
        m_w1(yn, dpren, 0, False)
        m_w2(gn, hn, 0, False)

    def p3(s, carry):
        env['z'] = s
        env['r'] = R3
        j = pl.ds(pl.multiple_of(jnp.minimum(s, 8) * 128, 128), 128)
        wx[:, j] = wT[j, :].T
        cs = _cols(s, T)
        cn = _cols(s + 1, T)
        gb = gs[:, cs]
        gn = gs[:, cn]
        pqn = back_a(1, cn)
        dh = m_dh(gb, 1)
        yn, rs12 = back_b(stream[:, cn], cn, pqn, True)
        hh, gp = gelu_bwd(m_pre(y4_s[:, cs], 1))
        y4_s[:, cn] = yn
        stat[3:4, cn] = rs12
        dpre = mk_dpre(dh, gp, 1)
        dy = dyacc[...] + m_dy(dpre, 1)
        g = gb.astype(F32)
        db2a[...] += g
        g3 = _ln2_bwd(g, dy, y4_s[0:D, cs], stat[3:4, cs], home(cs, y4_s))
        xs[:, cs] = (oacc[...] + m_out(hh, 1)).astype(BF)
        m_w1(y4_s[0:D, cs], dpre, 1, s > 0)
        m_w2(gb, hh, 1, s > 0)
        dhn = m_dh(gn, 0)
        g3b, dpqn = bwd1_a(1, g3, True)
        hn, gpn = gelu_bwd(m_pre(yn, 0))
        dpren = mk_dpre(dhn, gpn, 0)
        bwd1_b(1, cs, g3b, dpqn, True)
        dyacc[...] = m_dy(dpren, 0)
        oacc[...] = res(cn) + m_out(hn, 0)
        m_w1(yn, dpren, 0)
        m_w2(gn, hn, 0)
        env['r'] = ALLR
        return s

    if on('p3'):
        env['z'] = \
            lax.fori_loop(0, NT_ - 1, p3, 0)

    cp_out = pltpu.make_async_copy(xs, out_hbm.at[0], sem_out.at[0])
    if on('b3'):
        gb = gs[:, cl]
        y = y4_s[:, cl]
        hh, gp = gelu_bwd(m_pre(y, 1))
        dh = m_dh(gb, 1)
        dpre = mk_dpre(dh, gp, 1)
        dy = dyacc[...] + m_dy(dpre, 1, True)
        g = gb.astype(F32)
        db2a[...] += g
        g3 = _ln2_bwd(g, dy, y[0:D], stat[3:4, cl], home(cl, y4_s))
        o = oacc[...] + f_out(hh[0:FQ], 2)
        g3b, dpqn = bwd1_a(1, g3, True)
        m_wq(dw1a, y[0:D], dpre, 2)
        bwd1_b(1, cl, g3b, dpqn, True)
        pb = bf_a(1)
        m_wq(dw1a, y[0:D], dpre, 3)
        bf_c(1, bf_b(1, pb))
        m_wq(dw2Ta, gb, hh, 2)
        dk = bwd2_a(1, c0, True)
        m_wq(dw2Ta, gb, hh, 3)
        gn = bwd2_b(1, c0, dk, True, True)
        xs[:, cl] = (o + f_out(hh[FQ:FH], 3)).astype(BF)
        gs[:, c0] = gn
        hn, gpn = gelu_bwd(pre2[hs(0), c0].astype(F32))
        dhn = m_dh(gn, 0)
        dpren = mk_dpre(dhn, gpn, 0)
        m_w2(gn, hn, 0)
        m_w1(y2_s[0:D, c0], dpren, 0)
        dyacc[...] = m_dy(dpren, 0, True)
    cp_out.start()

    def p4(s, carry, last=False):
        if not last:
            env['z'] = s
            env['r'] = R4
        cs = _cols(s, T)
        cn = _cols(s + 1, T)
        dk = bwd2_a(1, cn, True)
        gb = gs[:, cs]
        dh = m_dh(gb, 1)
        db2a[...] += gb.astype(F32)
        gn = bwd2_b(1, cn, dk)
        hh, gp = gelu_bwd_p(1, cs)
        dpre = mk_dpre(dh, gp, 1)
        m_w2(gb, hh, 1)
        gs[:, cn] = gn
        y = y2_s[:, cs]
        dy = dyacc[...] + m_dy(dpre, 1)
        g1 = _ln2_bwd(stream[:, cs], dy, y[0:D], stat[2:3, cs], home(cs, y2_s))
        m_w1(y, dpre, 1)
        dhn = m_dh(gn, 0)
        hn, gpn = gelu_bwd_p(0, cn)
        dpren = mk_dpre(dhn, gpn, 0)
        g1b, dpqn = bwd1_a(0, g1)
        if last:
            m_fin(w2T, dw2Ta, gn, hn, hs(0))
        else:
            m_w2(gn, hn, 0)
        bwd1_b(0, cs, g1b, dpqn)
        dyacc[...] = m_dy(dpren, 0)
        if last:
            m_fin(w1c, dw1a, y2_s[0:D, cn], dpren, hs(0))
        else:
            m_w1(y2_s[0:D, cn], dpren, 0)
        env['r'] = ALLR
        return s

    if on('p4'):
        env['z'] = \
            lax.fori_loop(0, NT_ - 2, p4, 0)

    if on('b4'):
        p4(NT_ - 2, 0, True)
        gb = gs[:, cl]
        y = y2_s[:, cl]
        db2a[...] += gb.astype(F32)
        dh = m_dh(gb, 1)
        hh, gp = gelu_bwd(pre2[hs(1), cl].astype(F32))
        dpre = mk_dpre(dh, gp, 1)
        m_wq_fin(w2T, dw2Ta, gb, hh, 2)
        dy = dyacc[...] + m_dy(dpre, 1)
        g1 = _ln2_bwd(stream[:, cl], dy, y[0:D], stat[2:3, cl], home(cl, y2_s))
        m_wq_fin(w2T, dw2Ta, gb, hh, 3)
        g1b, dpqn = bwd1_a(0, g1)
        m_wq_fin(w1c, dw1a, y[0:D], dpre, 2)
        bwd1_b(0, cl, g1b, dpqn)
        pb = bf_a(0)
        m_wq_fin(w1c, dw1a, y[0:D], dpre, 3)
        bf_c(0, bf_b(0, pb))
        dw2Ta[:, 0:D2] = _dot_nt(u_s[1, 0:D, 0:TB], qk_s[1, 0:D2, 0:TB])
        b2v[...] = jnp.sum(db2a[...].T, axis=0, keepdims=True).astype(BF).reshape(D)
        wo[...] = dwo_a[...].astype(BF)
    cp_dw1a = pltpu.make_async_copy(w1c.at[pl.ds(0, D), :], dw1_hbm, sem_out.at[1])
    cp_dw2a = pltpu.make_async_copy(w2T, dw2_hbm, sem_out.at[2])
    cp_db1 = pltpu.make_async_copy(b1v, db1_hbm, sem_out.at[3])
    cp_db2 = pltpu.make_async_copy(b2v, db2_hbm, sem_out.at[4])
    cp_dwo = pltpu.make_async_copy(wo, dwo_hbm, sem_out.at[5])
    cp_dwqkv = pltpu.make_async_copy(wraw, dwqkv_hbm, sem_out.at[6])
    cp_dw1a.start()
    cp_dw2a.start()
    cp_db2.start()
    cp_dwo.start()
    o3 = 7

    def cp_dx(s):
        if isinstance(s, int):
            lo, hi = max(s * TB - T, 0), min(s * TB + TB - T, S)
            w = pl.ds(lo, hi - lo)
        else:
            w = pl.ds(pl.multiple_of(s * TB - T, T), TB)
        return pltpu.make_async_copy(gs.at[:, w], dx_hbm.at[0, :, w], sem_out.at[o3 + s])

    def p5a(s, carry):
        cs = _cols(s, TB)
        ks = pl.ds(pl.multiple_of(TB + s * 384, 128), 384)
        dbrow[0:1, _cols(s, FQ)] = jnp.sum(db1a[_cols(s, FQ), :].T, axis=0, keepdims=True)
        dk = bwd2_a(0, cs)
        dw2Ta[:, 0:D2] += _dot_nt(u_s[1, 0:D, ks], qk_s[1, 0:D2, ks])
        dw2Ta[:, 0:D2] += _dot_nt(u_s[0, 0:D, cs], jnp.concatenate([qk_s[0, 0:D, cs], dk], axis=0))
        return carry

    if on('p5a'):
        lax.fori_loop(0, NB, p5a, 0)

    def sub(s, k):
        if isinstance(s, int):
            return pl.ds(s * TB + k * T, T)
        return pl.ds(pl.multiple_of(s * TB + k * T, T), T)

    def dx_fin(cs, du):
        gs[:, cs] = _ln2_bwd(stream[:, cs], du, u_s[0, 0:D, cs], stat[0:1, cs], home(cs, u_s.r[0]), 1.0, False)

    def dx_tile(s, first=False):
        if not first:
            dx_fin(sub(s, -1), dyacc[...])
        for k in range(TB // T - 1):
            dx_fin(sub(s, k), _dot(wx[...], qk_s[0, :, sub(s, k)]))
        dyacc[...] = _dot(wx[...], qk_s[0, :, sub(s, TB // T - 1)])
        cp_dx(s).start()

    env['r'] = ()
    if on('b5'):
        dwt = dw2Ta[:, 0:D2].astype(BF).T.astype(F32)
        dwq = _from_perm(ps0, dwt[0:D]).astype(BF)
        dwk = _from_perm(ps1, dwt[D:D2]).astype(BF)
        wraw[...] = jnp.concatenate([dwq, dwk, dwv_a[...].astype(BF)], axis=0).T
        b1v[...] = dbrow[0:1, :].astype(BF).reshape(F)
        dx_tile(0, True)
    else:
        cp_dx(0).start()
    cp_dwqkv.start()
    cp_db1.start()

    def p5b(s, carry):
        env['z'] = s
        dx_tile(s)
        return s

    if on('p5b'):
        env['z'] = \
            lax.fori_loop(1, NB, p5b, 0)
        env['r'] = ()
        dx_fin(cl, dyacc[...])
    else:
        for s in range(1, NB):
            cp_dx(s).start()
    cp_dx(NB).start()

    cp_out.wait()
    cp_dw1a.wait()
    cp_dw2a.wait()
    cp_db1.wait()
    cp_db2.wait()
    cp_dwo.wait()
    cp_dwqkv.wait()
    for s in range(NB + 1):
        cp_dx(s).wait()


@jax.jit
def pallas_interleave_layers__linear_attn_block__mixer_channel_mlp__prompt_kernel(
    A_x: jax.Array,
    A_wqkv: jax.Array,
    A_wo: jax.Array,
    B_x: jax.Array,
    B_w1: jax.Array,
    B_b1: jax.Array,
    B_w2: jax.Array,
    B_b2: jax.Array,
    grad_out: jax.Array,
):
    del B_x
    V = pltpu.VMEM
    n_in = NB + 6 + 3 + 2
    n_out = 7 + NB + 1
    scratch = [
        V((D, S), BF),
        V((D, S), BF),
        V((D, D3), BF),
        V((D // 2, D3), U32),
        V((D3 // 2, D), U32),
        V((D, D), BF),
        V((DA, F), BF),
        V((F // 2, DA), U32),
        V((F // 2, D), U32),
        V((D, F), BF),
        V((F,), BF),
        V((D,), BF),
        V((D, 128), F32),
        V((D, F), F32),
        V((D, F), F32),
        V((F // 2, S), U32),
        V((D, S), F32),
        V((DA // 2, S), U32),
        V((DA // 2, S), U32),
        V((D3 // 2, S), U32),
        V((D3 // 2, S), U32),
        V((H, S), F32),
        V((H, S), F32),
        V((DA, S), BF),
        V((DA, S), BF),
        V((8, S), F32),
        V((F, T), F32),
        V((8, F), F32),
        V((D, T), F32),
        V((D, T), F32),
        V((FQ // 2, T), U32),
        V((2, NG, 64, 128), U32),
        V((D, DA), F32),
        V((2, D // 2, D), U32),
        V((2, D, 128), F32),
        V((2, D // 2, D), U32),
        V((D // 2, D), U32),
        V((D, DR), F32),
        V((D // 2, DA), U32),
        V((D, D), F32),
        V((D, D), F32),
        V((D, 128), F32),
        V((5, D, 128), F32),
        V((5, D, 128), F32),
        V((2, D, T), F32),
        pltpu.SMEM((1,), jnp.int32),
        pltpu.SemaphoreType.DMA((n_in,)),
        pltpu.SemaphoreType.DMA((n_out,)),
    ]
    any_spec = pl.BlockSpec(memory_space=pl.ANY)
    out_shape = (
        jax.ShapeDtypeStruct((1, D, S), BF),
        jax.ShapeDtypeStruct((1, D, S), BF),
        jax.ShapeDtypeStruct((D, D3), BF),
        jax.ShapeDtypeStruct((D, D), BF),
        jax.ShapeDtypeStruct((D, F), BF),
        jax.ShapeDtypeStruct((F,), BF),
        jax.ShapeDtypeStruct((D, F), BF),
        jax.ShapeDtypeStruct((D,), BF),
    )
    outT, dxT, dwqkv, dwo, dw1, db1, dw2T, db2 = pl.pallas_call(
        _kernel,
        out_shape=out_shape,
        in_specs=[any_spec] * 8,
        out_specs=tuple([any_spec] * 8),
        scratch_shapes=scratch,
        compiler_params=pltpu.CompilerParams(vmem_limit_bytes=127 * 1024 * 1024),
    )(jnp.swapaxes(A_x, 1, 2), A_wqkv, A_wo, B_w1, B_b1, B_w2.T, B_b2, jnp.swapaxes(grad_out, 1, 2))
    return (jnp.swapaxes(outT, 1, 2), jnp.swapaxes(dxT, 1, 2), dwqkv, dwo, dw1, db1, dw2T.T, db2)
```

```python
import jax
import jax.numpy as jnp
from jax import lax
import jax.experimental.pallas as pl
import jax.experimental.pallas.tpu as pltpu

S, D, F = 2048, 576, 4608
H, DH = 32, 18
D3 = 3 * D
DA = 592
T = 128
NT_ = S // T
TB = 512
NB = S // TB
FH = F // 2
FQ = F // 4
D2 = 2 * D
DR = D + H
QA = 512
W1C = F // 3
NG = 5
WSTEP = 112
HEAD_LO = (0, 7, 13, 19, 25)
HEAD_HI = (6, 12, 18, 24, 31)

R3 = ()
R4 = ()
LN_EPS = 1e-5
PHI_EPS = 1e-6
GC0 = 0.7978845608028654
GC1 = 0.044715

BF = jnp.bfloat16


def on(name):
    return True


F32 = jnp.float32
U32 = jnp.uint32
_NN = (((1,), (0,)), ((), ()))
_NT = (((1,), (1,)), ((), ()))


def _dot(a, b):
    return lax.dot_general(a, b, _NN, preferred_element_type=F32)


def _dot_nt(a, b):
    return lax.dot_general(a, b, _NT, preferred_element_type=F32)


def _rows(m, nt):
    p = {1: 4, 2: 2}[nt % 4]
    return [slice(m // p * i, m // p * (i + 1)) for i in range(p)]


def _dot5(a, b, split, head=False):
    k = a.shape[1]
    nt = (k + 127) // 128
    if not split or nt % 4 == 0:
        return _dot(a, b)
    if head:
        odd, main = slice(0, nt % 4 * 128), slice(nt % 4 * 128, k)
    else:
        odd, main = slice(nt // 4 * 512, k), slice(0, nt // 4 * 512)
    tail = [_dot(a[r, odd], b[odd]) for r in _rows(a.shape[0], nt)]
    return _dot(a[:, main], b[main]) + jnp.concatenate(tail, axis=0)


def _dot5_nt(a, b):
    n = b.shape[0]
    nt = (n + 127) // 128
    n0 = nt // 4 * 512
    main = _dot_nt(a, b[0:n0])
    tail = [_dot_nt(a[r], b[n0:n]) for r in _rows(a.shape[0], nt)]
    return jnp.concatenate([main, jnp.concatenate(tail, axis=0)], axis=1)


def _colmean(x):
    n = x.shape[1]
    p = jnp.sum(x.reshape(9, 64, n), axis=0)
    p = p[0:32] + p[32:64]
    p = p[0:16] + p[16:32]
    p = p[0:8] + p[8:16]
    return jnp.sum(p, axis=0, keepdims=True) * (1.0 / D)


def _ln(x):
    m = _colmean(x)
    xc = x - m
    v = _colmean(xc * xc)
    rs = lax.rsqrt(v + LN_EPS)
    return xc * rs, rs


def _ln_bwd(dy, y, rs):
    a = _colmean(dy)
    b = _colmean(dy * y)
    return (dy - a - y * b) * rs


CR = 8
NCH = D // CR
FCR = 32


def _fold(p):
    while p.shape[0] > 8:
        h = p.shape[0] // 2
        p = p[0:h] + p[h:2 * h]
    return jnp.sum(p, axis=0, keepdims=True) * (1.0 / D)


def _ch(x, c, cr=CR):
    return x[c * cr:(c + 1) * cr]


def _nop(c, v):
    return c


PR = 32


_PO = (16, 17) + tuple(range(16))


def _cat(out):
    return jnp.concatenate(out[2:] + out[:2], axis=0)


def _b8(c, rows=PR):
    return jnp.broadcast_to(c, (rows, c.shape[1]))


def _pace(c, v):
    return c + 0.0 * v[0:1]


def _ln2(x, ld, fast=False):
    cr, pace = (FCR, _nop) if fast else (CR, _pace)
    acc = _ch(x, 0, cr)
    for c in range(1, D // cr):
        acc = acc + _ch(x, c, cr)
    m = _fold(acc)
    a1 = a2 = None
    x = ld(0)
    for c in range(D // cr):
        xc = _ch(x, c, cr) - m
        a1 = xc if a1 is None else a1 + xc
        a2 = xc * xc if a2 is None else a2 + xc * xc
    s1 = _fold(a1)
    s2 = _fold(a2)
    rs1 = lax.rsqrt(s2 + LN_EPS)
    m2 = s1 * rs1
    v2 = s2 * rs1 * rs1 - m2 * m2
    rs2 = lax.rsqrt(v2 + LN_EPS)
    rs12 = rs1 * rs2
    mc = _pace(m + s1, rs12)
    out = []
    x = ld(1)
    for c in _PO:
        y = (x[PR * c:PR * c + PR] - mc) * rs12
        mc = pace(mc, y)
        out.append(y.astype(BF))
    return _cat(out), rs12


def _ln2_bwd(g, dy, y, rs12, home, k=1.0 + LN_EPS, keep=True, fast=False):
    st, ld_t, ld_y = home
    a1 = a2 = None
    y = y.astype(F32)
    cr, pace = (FCR, _nop) if fast else (CR, _pace)
    for c in range(D // cr):
        d = _ch(dy, c, cr)
        t = d * _ch(y, c, cr)
        a1 = d if a1 is None else a1 + d
        a2 = t if a2 is None else a2 + t
    t = g + dy * rs12
    if ld_t is None:
        ld_t, ld_y = (lambda r: t[r]), (lambda r: y[r])
    else:
        st(slice(0, D), t)
    a = _fold(a1) * rs12
    b = _fold(a2) * (k * rs12)
    out = []
    for c in _PO:
        r = slice(PR * c, PR * c + PR)
        o = (ld_t(r) - ld_y(r).astype(F32) * b) - a
        b = pace(b, o)
        if keep:
            st(r, o)
        out.append(o.astype(BF))
    return _cat(out)


def _lnp(x, link=None, ld=None, fast=False):
    cr, pace = (FCR, _nop) if fast else (CR, _pace)
    acc = _ch(x, 0, cr)
    if link is not None:
        acc = acc + 0.0 * link
    for c in range(1, D // cr):
        acc = acc + _ch(x, c, cr)
    m = _fold(acc)
    a2 = None
    if ld is not None:
        x = ld(0)
    for c in range(D // cr):
        xc = _ch(x, c, cr) - m
        a2 = xc * xc if a2 is None else a2 + xc * xc
    rs = lax.rsqrt(_fold(a2) + LN_EPS)
    mc = _pace(m, rs)
    out = []
    if ld is not None:
        x = ld(1)
    for c in _PO:
        y = (x[PR * c:PR * c + PR] - mc) * rs
        mc = pace(mc, y)
        out.append(y.astype(BF))
    return _cat(out), rs, jnp.minimum(jnp.abs(y[0:1]), 1.0)


def _headsum(x):
    n = x.shape[1]
    p = x.reshape(DH, H, n)
    p = p[0:9] + p[9:18]
    q = (p[0] + p[1]) + (p[2] + p[3])
    r = (p[4] + p[5]) + (p[6] + p[7])
    return (q + r) + p[8]


def _headmul(x, c):
    n = x.shape[1]
    return (x.reshape(DH, H, n) * c[None]).reshape(D, n)


_LT = ((0, 128), (128, 128), (256, 128), (384, 128), (512, 64))


def _to_perm(scr, val, c0=0, c1=5):
    lt = [(c, o - 128 * c0, w) for c, (o, w) in enumerate(_LT)][c0:c1]
    for c, o, w in lt:
        scr[c, :, 0:w] = val[:, o:o + w]
    return jnp.concatenate(
        [jnp.concatenate([scr[c, pl.ds(j, H, stride=DH), 0:w] for c, o, w in lt], axis=1)
         for j in range(DH)], axis=0)


def _from_perm(scr, val):
    for j in range(DH):
        for c, (o, w) in enumerate(_LT):
            scr[c, pl.ds(j, H, stride=DH), 0:w] = val[H * j:H * j + H, o:o + w]
    return jnp.concatenate([scr[c, :, 0:w] for c, (o, w) in enumerate(_LT)], axis=1)


class _Pk:
    def __init__(self, ref):
        self.ref = ref

    def _idx(self, idx):
        nd = len(self.ref.shape)
        if idx is Ellipsis:
            return idx
        if not isinstance(idx, tuple):
            idx = (idx,)
        idx = list(idx) + [slice(None)] * (nd - len(idx))
        r = idx[nd - 2]
        if isinstance(r, slice):
            if r.start is not None or r.stop is not None:
                r = slice(r.start // 2, r.stop // 2)
        elif isinstance(r.start, int):
            r = pl.ds(r.start // 2, r.size // 2)
        else:
            r = pl.ds(pl.multiple_of(r.start // 2, 8), r.size // 2)
        idx[nd - 2] = r
        return tuple(idx)

    def __getitem__(self, idx):
        return pltpu.bitcast(self.ref[self._idx(idx)], BF)

    def __setitem__(self, idx, val):
        self.ref[self._idx(idx)] = pltpu.bitcast(val, U32)


class _L2:
    def __init__(self, a, b):
        self.r = (a, b)

    def __getitem__(self, idx):
        return self.r[idx[0]][idx[1:]]

    def __setitem__(self, idx, val):
        self.r[idx[0]][idx[1:]] = val


def _aug(y):
    r = lax.broadcasted_iota(jnp.int32, (DA - D, y.shape[1]), 0)
    return jnp.concatenate([y.astype(BF), jnp.where(r < 2, 1.0, 0.0).astype(BF)], axis=0)


def _phi(t):
    return jnp.where(t > 0, t + 1.0, jnp.exp(t)) + PHI_EPS


def _dphi_from_phi(p):
    return jnp.minimum(p - PHI_EPS, 1.0)


def _win(x, g):
    return x[WSTEP * g:WSTEP * g + 128]


def _assemble(parts):
    pieces = [parts[0][:WSTEP]]
    for g in range(NG - 1):
        pieces.append(parts[g][WSTEP:128] + parts[g + 1][0:16])
        pieces.append(parts[g + 1][16:WSTEP] if g + 1 < NG - 1 else parts[g + 1][16:128])
    return jnp.concatenate(pieces, axis=0)


def _head_mask(g):
    r = lax.broadcasted_iota(jnp.int32, (128, 128), 0) + WSTEP * g
    c = lax.broadcasted_iota(jnp.int32, (128, 128), 1) + WSTEP * g
    hr = (r * 3641) >> 16
    hc = (c * 3641) >> 16
    return (hr == hc) & (hr >= HEAD_LO[g]) & (hr <= HEAD_HI[g])


def _lane_fold(x):
    acc = x[:, 0:128]
    for j in range(1, x.shape[1] // 128):
        acc = acc + x[:, 128 * j:128 * (j + 1)]
    return acc


def _lane_tile(x128, n):
    if n == 128:
        return x128
    return jnp.concatenate([x128] * (n // 128), axis=1)


def _gelu_parts(pre):
    x2 = pre * pre
    t = jnp.tanh(pre * (GC0 + (GC0 * GC1) * x2))
    hp = 0.5 + 0.5 * t
    return x2, t, hp


def _cols(s, n):
    if isinstance(s, int):
        return pl.ds(s * n, n)
    return pl.ds(pl.multiple_of(s * n, n), n)


def _kernel(
    x_hbm, wqkv_hbm, wo_hbm, w1_hbm, b1_hbm, w2_hbm, b2_hbm, g_hbm,
    out_hbm, dx_hbm, dwqkv_hbm, dwo_hbm, dw1_hbm, db1_hbm, dw2_hbm, db2_hbm,
    xs, gs, wraw, wx, wT, wo, w1c, w1T, w2c, w2T, b1v, b2v, b2col,
    dw1a, dw2Ta, pre2, stream, u_0, u_1, qk_0, qk_1, rd_0, rd_1, y2_s, y4_s, stat, db1a, dbrow,
    oacc, dyacc, hcar, gcar, fcar,
    kvT, cacc, ctb, zb, mm, mmT, pacc, dctb, dwv_a, dwo_a, db2a, ps0, ps1, dtmp, zs,
    sem_in, sem_out,
):
    wx, wT, w1T, w2c, pre2, hcar, kvT, ctb, mm, mmT, dctb = [
        _Pk(r) for r in (wx, wT, w1T, w2c, pre2, hcar, kvT, ctb, mm, mmT, dctb)]
    u_s = _L2(_Pk(u_0), _Pk(u_1))
    qk_s = _L2(_Pk(qk_0), _Pk(qk_1))
    rd_s = _L2(rd_0, rd_1)
    y4_s, gcar = _Pk(y4_s), _Pk(gcar)

    ALLR = (0, 1, 2, 3, 4)
    env = {'r': ALLR}

    def zero(k):
        if k not in env['r']:
            return 0
        return env['z'] >> (20 + k)

    def _alt(cs, k):
        if k not in env['r']:
            return cs
        return pl.ds(pl.multiple_of(cs.start + (zero(k) << 7), 128), cs.size)

    def home(cs, yref, ys=None, ts=None):
        tref, tc = (stream, cs) if ts is None else (fcar, ts)

        def st(r, v):
            tref[r, tc] = v
        if 3 not in env['r']:
            return st, None, None
        return st, (lambda r: tref[r, _alt(tc, 3)]), (lambda r: yref[r, _alt(ys or cs, 3)])

    zs[0] = 0

    def cp_x(s):
        return pltpu.make_async_copy(x_hbm.at[0, :, _cols(s, TB)], xs.at[:, _cols(s, TB)], sem_in.at[s])

    k0 = NB
    def cp_wpart(lo, hi, k):
        return pltpu.make_async_copy(wqkv_hbm.at[:, pl.ds(lo, hi - lo)], wraw.at[:, pl.ds(lo, hi - lo)], sem_in.at[k])

    def cp_wk(lo, hi, k):
        w = (pl.ds(lo, hi - lo), pl.ds(512, D2 - 512))
        return pltpu.make_async_copy(wqkv_hbm.at[w], wraw.at[w], sem_in.at[k])

    cp_wka = cp_wk(0, 256, k0)
    cp_wkb = cp_wk(256, D, k0 + 11)
    cp_wq = cp_wpart(0, 512, k0 + 9)
    cp_wv = cp_wpart(D2, D3, k0 + 10)
    cp_wo = pltpu.make_async_copy(wo_hbm, wo, sem_in.at[k0 + 1])
    cp_b1 = pltpu.make_async_copy(b1_hbm, b1v, sem_in.at[k0 + 2])
    cp_b2 = pltpu.make_async_copy(b2_hbm, b2v, sem_in.at[k0 + 3])
    cp_w2 = pltpu.make_async_copy(w2_hbm.at[:, pl.ds(0, FQ)], w2T.at[:, pl.ds(0, FQ)], sem_in.at[k0 + 4])
    cp_w2b = pltpu.make_async_copy(w2_hbm.at[:, pl.ds(FQ, F - FQ)], w2T.at[:, pl.ds(FQ, F - FQ)], sem_in.at[k0 + 12])
    cp_g = pltpu.make_async_copy(g_hbm.at[0], gs, sem_in.at[k0 + 5])
    k1 = k0 + 6

    def cp_w1(c):
        return pltpu.make_async_copy(w1_hbm.at[:, _cols(c, W1C)], w1c.at[pl.ds(0, D), _cols(c, W1C)],
                                     sem_in.at[k1 + c])

    cp_x(0).start()
    cp_wka.start()
    cp_wkb.start()
    cp_wq.start()
    cp_x(1).start()
    cp_b1.start()
    cp_b2.start()
    cp_wv.start()
    cp_x(2).start()
    cp_x(3).start()
    for s in range(3):
        cp_w1(s).start()
    cp_wo.start()
    cp_w2.start()
    cp_w2b.start()

    def wrow(ref, g, base=0):
        return ref[base + WSTEP * g:base + WSTEP * g + 128, :]

    def front_a(l, cs, x, link=None, fast=False):
        u, rs, lk = _lnp(x, link, (lambda k: stream[:, _alt(cs, k)]) if l == 1 else None, fast)
        ub = _aug(u)
        u_s[l, :, cs] = ub
        stat[l:l + 1, cs] = rs
        return ub if link is None else lk

    def front_k(l, cs, ub):
        pkb = _phi(_dot5(wT[D:D2, :], ub[0:D], True)).astype(BF)
        qk_s[l, D2:D3, cs] = pkb
        return pkb

    def front_q(l, cs, ub):
        qk_s[l, 0:D, cs] = _phi(_dot5(wT[0:D, :], ub[0:D], True)).astype(BF)

    def front_b(l, cs, ub):
        pkb = front_k(l, cs, ub)
        front_q(l, cs, ub)
        return pkb

    def front_c(pkb, ub, first=False):
        if pkb.shape[1] == T:
            for m in range(4):
                dwv_a[144 * m:144 * m + 144, 512:DA] += _dot_nt(pkb[144 * m:144 * m + 144], ub[512:DA])
            dwv_a[:, 0:512] += _dot_nt(pkb, ub[0:512])
            return
        c = _dot_nt(pkb, ub)
        if first:
            dw1a[:, 0:DA] = c
        else:
            dw1a[:, 0:DA] += c

    def ff_a(l):
        c = dwv_a[...] if l else dw1a[:, 0:DA]
        zb[l] = jnp.broadcast_to(c[:, D:D + 1], (D, 128))
        ct = _from_perm(ps0, c[:, 0:D]).astype(BF)
        ctb[l] = ct
        return ct

    def ff_b(l, ct):
        kvs = []
        for g in range(NG):
            kv = jnp.where(_head_mask(g), _dot_nt(_win(ct, g), wrow(wT, g, D2)), 0.0)
            kvT[l, g] = kv.T.astype(BF)
            kvs.append(kv.astype(BF))
        return kvs

    def ff_c(l, kvs):
        m = _assemble([_dot(kvs[g], wrow(wo, g)) for g in range(NG)])
        mp = _to_perm(ps1, m).astype(BF)
        mm[l] = mp
        mmT[...] = mp.T

    def back_a(l, cs):
        pq = qk_s[l, 0:D, cs].astype(F32)
        rden = 1.0 / (_headsum(pq * zb[l]) + PHI_EPS)
        rd_s[l, :, cs] = rden
        return _headmul(pq, rden).astype(BF)

    def back_b(x, cs, pqn, split=False, fast=False):
        x1 = x + _dot5(mmT[...], pqn, split)
        env['x'] = x1
        if 0 in env['r']:
            stream[:, cs] = x1
            y, rs12 = _ln2(x1, lambda k: stream[:, _alt(cs, k)], fast)
        else:
            y, rs12 = _ln2(x1, lambda k: x1, fast)
        return _aug(y), rs12

    def res(cs):
        return (stream[:, _alt(cs, 2)] if 0 in env['r'] else env['x']) + b2col[...]

    def bwd1_a(l, gb, split=False):
        return gb, _dot5(mm[l], gb, split)

    def bwd1_b(l, cs, gb, dpqn, split=False):
        pq = qk_s[l, 0:D, cs].astype(F32)
        rden = rd_s[l, :, cs]
        z = zb[l]
        rd = rden
        r = None
        pqn = []
        rl = 4 in env['r']
        if rl:
            dtmp[0] = dpqn
        for j in range(DH):
            t = pq[H * j:H * j + H] * rd
            pqn.append(t.astype(BF))
            t = dpqn[H * j:H * j + H] * t
            r = t if r is None else r + t
            rd = _pace(rden, r)
        rb = r.astype(BF)
        for j in range(DH):
            rj = slice(H * j, H * j + H)
            w = _dphi_from_phi(qk_s[l, rj, _alt(cs, 4)].astype(F32) if rl else pq[rj]) * rden
            t = ((dtmp[zero(4), rj, :] if rl else dpqn[rj]) - z[rj] * r) * w
            r = _pace(r, t)
            qk_s[l, rj, cs] = t.astype(BF)
        pqn = jnp.concatenate(pqn, axis=0)
        gr = jnp.concatenate([gb, rb], axis=0)
        pa = pacc if l else cacc
        if split:
            pa[:, 0:512] += _dot_nt(pqn, gr[0:512])
            for m in range(4):
                pa[144 * m:144 * m + 144, 512:DR] += _dot_nt(pqn[144 * m:144 * m + 144], gr[512:DR])
        else:
            pa[...] += _dot_nt(pqn, gr)

    def bf_a(l):
        p = (pacc if l else cacc)[...]
        tl = p[:, 512:DR]
        rr = lax.broadcasted_iota(jnp.int32, tl.shape, 0)
        cc = lax.broadcasted_iota(jnp.int32, tl.shape, 1)
        dz = -jnp.sum(jnp.where(cc - (D - 512) == (rr & (H - 1)), tl, 0.0), axis=1, keepdims=True)
        hi = dz.astype(BF).astype(F32)
        ce = lax.broadcasted_iota(jnp.int32, (D, DA - D), 1)
        dctb[:, D:DA] = jnp.where(ce == 0, hi, jnp.where(ce == 1, dz - hi, 0.0)).astype(BF)
        pb = _from_perm(ps0, p[:, 0:D]).astype(BF)
        return pb

    def acc_l(ref, l, val):
        if l == 1:
            ref[:, 0:D] = val
        else:
            ref[:, 0:D] += val

    def bf_b(l, pb):
        ds_ = [jnp.where(_head_mask(g), _dot_nt(_win(pb, g), wrow(wo, g)), 0.0) for g in range(NG)]
        acc_l(dwo_a, l, _assemble([_dot(kvT[l, g], _win(pb, g)) for g in range(NG)]))
        return ds_

    def bf_c(l, ds_):
        dct = _assemble([_dot(ds_[g].astype(BF), wrow(wT, g, D2)) for g in range(NG)])
        dp = _to_perm(ps1, dct).astype(BF)
        dctb[:, 0:D] = dp
        wx[:, D2:D3] = dp.T
        acc_l(dwv_a, l, _assemble([_dot(ds_[g].T.astype(BF), ctb[l, WSTEP * g:WSTEP * g + 128, :]) for g in range(NG)]))

    def bwd2_a(l, cs, split=False):
        dpk = _dot5(dctb[...], u_s[l, :, cs], split)
        dk = (dpk * _dphi_from_phi(qk_s[l, D2:D3, cs].astype(F32))).astype(BF)
        qk_s[l, D:D2, cs] = dk
        return dk

    def bwd2_b(l, cs, dk=None, keep=True, bal=False, fast=False, ts=None):
        if dk is None:
            rhs = qk_s[l, :, cs]
        else:
            rhs = jnp.concatenate([qk_s[l, 0:D, cs], dk, qk_s[l, D2:D3, cs]], axis=0)
        du = _dot5(wx[...], rhs, bal)
        return _ln2_bwd(stream[:, cs], du, u_s[l, 0:D, cs], stat[l:l + 1, cs], home(cs, u_s.r[l], None, ts), 1.0, keep, fast)

    def hs(h):
        return pl.ds(h * FH, FH)

    def qs(c):
        return pl.ds(c * FQ, FQ)

    def f_pre(y, cs, c):
        pre = _dot5(w1T[qs(c), :], y, True)
        pre2[qs(c), cs] = pre.astype(BF)
        _, _, hp = _gelu_parts(pre)
        return (pre * hp).astype(BF)

    def f_out(hh, c):
        return _dot5(w2T[:, qs(c)], hh, True, True)

    def gelu_bwd(pre):
        x2, t, hp = _gelu_parts(pre)
        hh = (pre * hp).astype(BF)
        gp = hp + (0.5 * pre) * (1.0 - t * t) * (GC0 + (3.0 * GC0 * GC1) * x2)
        return hh, gp

    def gelu_bwd_p(h, cs):
        GR = 64
        hs_, gs_ = [], []
        k = jnp.full((1, T), GC0, F32)
        for c in range(FH // GR):
            pre = pre2[h * FH + c * GR:h * FH + (c + 1) * GR, cs].astype(F32)
            x2 = pre * pre
            t = jnp.tanh(pre * (k + (GC0 * GC1) * x2))
            k = _pace(k, t)
            hp = 0.5 + 0.5 * t
            hs_.append((pre * hp).astype(BF))
            gs_.append(hp + (0.5 * pre) * (1.0 - t * t) * (GC0 + (3.0 * GC0 * GC1) * x2))
        return jnp.concatenate(hs_, axis=0), jnp.concatenate(gs_, axis=0)

    def m_dh(gb, h):
        return _dot5(w2c[hs(h), :], gb, True)

    def m_dhq(gb, c):
        return _dot(w2c[qs(c), :], gb)

    def m_pre(y, h):
        return _dot5(w1T[hs(h), :], y, True)

    def m_dy(dpre, h, bal=False):
        return _dot5(w1c[0:D, hs(h)], dpre, bal, True)

    def m_out(hh, h):
        return _dot(w2T[:, hs(h)], hh)

    def acc_to(ref, sl, val, keep):
        if keep is True:
            ref[:, sl] += val
        elif keep is False:
            ref[:, sl] = val
        else:
            ref[:, sl] = jnp.where(keep, ref[:, sl], 0.0) + val

    def m_w1(y, dpre, h, keep=True):
        acc_to(dw1a, hs(h), _dot_nt(y[0:D], dpre), keep)

    def mk_dpre(dh, gp, h):
        dp = dh * gp
        db1a[hs(h), :] += dp
        return dp.astype(BF)

    def m_w2(gb, hh, h, keep=True):
        acc_to(dw2Ta, hs(h), _dot_nt(gb, hh), keep)

    def m_wq(ref, a, b, c):
        acc_to(ref, qs(c), _dot5_nt(a, b[(c - 2) * FQ:(c - 1) * FQ]), True)

    def m_fin(dst, ref, a, b, sl):
        val = ref[:, sl] + _dot_nt(a, b)
        dst[0:D, sl] = val.astype(BF)

    def m_wq_fin(dst, ref, a, b, c):
        m_fin(dst, ref, a, b[(c - 2) * FQ:(c - 1) * FQ], qs(c))

    def clear(i, carry):
        r = pl.ds(pl.multiple_of(i * 32, 32), 32)
        for ref in (pacc, dwv_a, cacc, db2a):
            ref[r, :] = jnp.zeros((32, ref.shape[1]), F32)
        db1a[pl.ds(pl.multiple_of(i * 256, 256), 256), :] = jnp.zeros((256, T), F32)
        return carry

    lax.fori_loop(0, D // 32, clear, 1)

    def ln0(s, chain=4, lk=None, ks=(0, 1, 2, 3), fast=False):
        for k in ks:
            cs = pl.ds(s * TB + k * T, T)
            if k % chain == 0 and (k or lk is None):
                lk = jnp.zeros((1, T), F32)
            lk = front_a(0, cs, xs[:, cs].astype(F32), lk, fast)
        return lk

    def k_part(s):
        cs = _cols(s, TB)
        qk_s[0, D2:D3, cs] = _phi(_dot(wT[D:D2, :], u_s[0, 0:D, cs])).astype(BF)

    def q_part(lo, hi):
        cs = pl.ds(lo * T, (hi - lo) * T)
        qk_s[0, 0:D, cs] = _phi(_dot(wT[0:D, :], u_s[0, 0:D, cs])).astype(BF)

    def c_part(s):
        cs = _cols(s, TB)
        front_c(qk_s[0, D2:D3, cs], u_s[0, :, cs], s == 0)

    def w1_t(c):
        w1T[_cols(c, W1C), :] = w1c[:, _cols(c, W1C)].T

    cp_x(0).wait()
    ln0(0, 4, None, (0, 1, 2), True)
    cp_wka.wait()
    wta = wraw[0:256, 512:D2].T
    wT[D:D2, 0:256] = _to_perm(ps1, wta[64:640].astype(F32), 0, 2).astype(BF)
    ln0(0, 1, None, (3,), True)
    stream[:, 0:TB] = _dot(wT[D:D2, 0:128], u_s[0, 0:128, 0:TB])
    cp_wkb.wait()
    wtb = wraw[256:D, 512:D2].T
    wT[D:D2, 256:D] = _to_perm(ps1, wtb[64:640].astype(F32), 2, 5).astype(BF)
    qk_s[0, D2:D3, 0:TB] = _phi(
        stream[:, 0:TB] + _dot(wT[D:D2, 128:256], u_s[0, 128:256, 0:TB])
        + _dot(wT[D:D2, 256:D], u_s[0, 256:D, 0:TB])).astype(BF)
    wtk = jnp.concatenate([wta[0:64], wtb[0:64]], axis=1)
    dw1a[:, 0:256] = _dot_nt(qk_s[0, D2:D3, 0:TB], u_s[0, 0:256, 0:TB])
    cp_wq.wait()
    cp_x(1).wait()
    cp_b1.wait()
    cp_b2.wait()
    wtq = jnp.concatenate([wraw[:, 0:512].T, wtk[0:64]], axis=0)
    wT[0:D, :] = _to_perm(ps0, wtq.astype(F32)).astype(BF)
    dw1a[:, 256:DA] = _dot_nt(qk_s[0, D2:D3, 0:TB], u_s[0, 256:DA, 0:TB])
    b2col[...] = jnp.broadcast_to(b2v[...].reshape(1, D).astype(F32), (128, D)).T
    rid = lax.broadcasted_iota(jnp.int32, (DA - D, F), 0)
    w1c[D:DA, :] = jnp.where(
        rid == 0, jnp.broadcast_to(b1v[...].reshape(1, F).astype(F32), (DA - D, F)), 0.0).astype(BF)
    ln0(1)
    q_part(0, 4)
    k_part(1)
    for t_ in (4, 5):
        front_q(0, _cols(t_, T), u_s[0, :, _cols(t_, T)])
    c_part(1)
    cp_wv.wait()
    cp_x(2).wait()
    cp_x(3).wait()
    cp_w1(0).wait()
    cp_w1(1).wait()
    lk = ln0(2)
    for t_ in (6, 7):
        front_q(0, _cols(t_, T), u_s[0, :, _cols(t_, T)])
    wT[D2:D3, :] = wraw[:, D2:D3].T
    w1_t(0)
    ln0(3, 4, lk)
    k_part(2)
    c_part(2)
    w1_t(1)
    k_part(3)
    q_part(8, 12)
    c_part(3)
    cp_w1(2).wait()
    cp_wo.wait()
    cp_w2.wait()

    def step_2(s, first=False, last=False):
        cs = _cols(s, T)
        cn = _cols(s + 1, T)
        pqn = back_a(0, cn)
        if not first:
            y = y2_s[:, cs]
            h2 = f_pre(y, cs, 2)
        yn, rs12 = back_b(xs[:, cn].astype(F32), cn, pqn, True)
        if first:
            q_part(15, 16)
        else:
            o = oacc[...] + f_out(hcar[...], 1)
            h3 = f_pre(y, cs, 3)
            o = o + f_out(h2, 2)
        y2_s[:, cn] = yn
        stat[2:3, cn] = rs12
        h0n = f_pre(yn, cn, 0)
        if not first:
            x2 = o + f_out(h3, 3)
            stream[:, cs] = x2
            ub = front_a(1, cs, x2)
        hcar[...] = f_pre(yn, cn, 1)
        if last:
            pkb = front_k(1, cs, ub)
        oacc[...] = res(cn) + f_out(h0n, 0)
        if last:
            front_c(pkb, ub)
        elif not first:
            front_c(front_b(1, cs, ub), ub)

    env['z'] = zs[0]
    if on('b1'):
        ct = ff_a(0)
        q_part(12, 13)
        ff_c(0, ff_b(0, ct))
        q_part(13, 15)
        w1_t(2)
        step_2(-1, first=True)

    def p2(s, carry):
        env['z'] = s
        for s2 in (2 * s, 2 * s + 1):
            j = pl.ds(pl.multiple_of(jnp.minimum(s2, 11) * 384, 384), 384)
            w2c[j, :] = w2T[:, j].T
            step_2(s2)
        return s

    cp_w2b.wait()
    cp_g.start()
    if on('p2'):
        env['z'] = \
            lax.fori_loop(0, NT_ // 2 - 1, p2, 0)

    cp_g.wait()
    cl = _cols(NT_ - 1, T)
    c0 = _cols(0, T)
    if on('b2'):
        step_2(NT_ - 2, last=True)
        cp_ = _cols(NT_ - 2, T)
        y = y2_s[:, cl]
        gn = gs[:, c0]
        h2 = f_pre(y, cl, 2)
        o = oacc[...] + f_out(hcar[...], 1)
        h3 = f_pre(y, cl, 3)
        o = o + f_out(h2, 2)
        x2 = o + f_out(h3, 3)
        stream[:, cl] = x2
        ub = front_a(1, cl, x2, None, True)
        FE = FH // 8
        dhe = []

        def fill_dh(n):
            e = len(dhe)
            for i in range(e, e + n):
                dhe.append(_dot(w2c[i * FE:(i + 1) * FE, 0:512], gn[0:512]))

        front_q(1, cp_, u_s[1, :, cp_])
        fill_dh(1)
        pkb = front_k(1, cl, ub)
        fill_dh(1)
        front_c(pkb, ub)
        ct = ff_a(1)
        front_q(1, cl, ub)
        kvs = ff_b(1, ct)
        fill_dh(1)
        ff_c(1, kvs)
        dht = jnp.concatenate([_dot(w2c[r, 512:D], gn[512:D]) for r in _rows(FH, 1)], axis=0)
        fill_dh(1)
        yn, rs12 = back_b(stream[:, c0], c0, back_a(1, c0), True, True)
        y4_s[:, c0] = yn
        gcar[...] = gn
        stat[3:4, c0] = rs12
        fill_dh(4)
        hn, gpn = gelu_bwd(m_pre(yn, 0))
        dpren = mk_dpre(jnp.concatenate(dhe, axis=0) + dht, gpn, 0)
        oacc[...] = res(c0) + m_out(hn, 0)
        dyacc[...] = m_dy(dpren, 0)
        m_w1(yn, dpren, 0, False)
        m_w2(gn, hn, 0, False)

    def p3(s, carry):
        env['z'] = s
        env['r'] = R3
        j = pl.ds(pl.multiple_of(jnp.minimum(s, 8) * 128, 128), 128)
        wx[:, j] = wT[j, :].T
        cs = _cols(s, T)
        cn = _cols(s + 1, T)
        gb = gcar[...]
        gn = gs[:, cn]
        pqn = back_a(1, cn)
        dh = m_dh(gb, 1)
        yn, rs12 = back_b(stream[:, cn], cn, pqn, True)
        hh, gp = gelu_bwd(m_pre(y4_s[:, c0], 1))
        stat[3:4, cn] = rs12
        dpre = mk_dpre(dh, gp, 1)
        dy = dyacc[...] + m_dy(dpre, 1)
        g = gb.astype(F32)
        db2a[...] += g
        g3 = _ln2_bwd(g, dy, y4_s[0:D, c0], stat[3:4, cs], home(cs, y4_s, c0))
        xs[:, cs] = (oacc[...] + m_out(hh, 1)).astype(BF)
        m_w1(y4_s[0:D, c0], dpre, 1, s > 0)
        m_w2(gb, hh, 1, s > 0)
        y4_s[:, c0] = yn
        gcar[...] = gn
        dhn = m_dh(gn, 0)
        g3b, dpqn = bwd1_a(1, g3, True)
        hn, gpn = gelu_bwd(m_pre(yn, 0))
        dpren = mk_dpre(dhn, gpn, 0)
        bwd1_b(1, cs, g3b, dpqn, True)
        dyacc[...] = m_dy(dpren, 0)
        oacc[...] = res(cn) + m_out(hn, 0)
        m_w1(yn, dpren, 0)
        m_w2(gn, hn, 0)
        env['r'] = ALLR
        return s

    if on('p3'):
        env['z'] = \
            lax.fori_loop(0, NT_ - 1, p3, 0)

    cp_out = pltpu.make_async_copy(xs, out_hbm.at[0], sem_out.at[0])
    if on('b3'):
        gb = gcar[...]
        y = y4_s[:, c0]
        hh, gp = gelu_bwd(m_pre(y, 1))
        dh = m_dh(gb, 1)
        dpre = mk_dpre(dh, gp, 1)
        dy = dyacc[...] + m_dy(dpre, 1, True)
        g = gb.astype(F32)
        db2a[...] += g
        g3 = _ln2_bwd(g, dy, y[0:D], stat[3:4, cl], home(cl, y4_s, c0), fast=True)
        o = oacc[...] + f_out(hh[0:FQ], 2)
        g3b, dpqn = bwd1_a(1, g3, True)
        m_wq(dw1a, y[0:D], dpre, 2)
        bwd1_b(1, cl, g3b, dpqn, True)
        pb = bf_a(1)
        m_wq(dw1a, y[0:D], dpre, 3)
        bf_c(1, bf_b(1, pb))
        m_wq(dw2Ta, gb, hh, 2)
        dk = bwd2_a(1, c0, True)
        m_wq(dw2Ta, gb, hh, 3)
        gn = bwd2_b(1, c0, dk, True, True, True)
        pacc[:, 0:512] = _dot_nt(u_s[1, 0:D, 0:T], qk_s[1, 0:512, 0:T])
        xs[:, cl] = (o + f_out(hh[FQ:FH], 3)).astype(BF)
        gcar[...] = gn
        hn, gpn = gelu_bwd(pre2[hs(0), c0].astype(F32))
        dhn = m_dh(gn, 0)
        dpren = mk_dpre(dhn, gpn, 0)
        m_w2(gn, hn, 0)
        yn = y2_s[0:D, c0]
        y4_s[0:D, c0] = yn
        m_w1(yn, dpren, 0)
        dyacc[...] = m_dy(dpren, 0, True)
    cp_out.start()

    def p4(s, carry, last=False):
        if not last:
            env['z'] = s
            env['r'] = R4
        cs = _cols(s, T)
        cn = _cols(s + 1, T)
        dk = bwd2_a(1, cn, True)
        gb = gcar[...]
        dh = m_dh(gb, 1)
        db2a[...] += gb.astype(F32)
        gn = bwd2_b(1, cn, dk)
        hh, gp = gelu_bwd_p(1, cs)
        dpre = mk_dpre(dh, gp, 1)
        m_w2(gb, hh, 1)
        gcar[...] = gn
        y = y4_s[0:D, c0]
        dy = dyacc[...] + m_dy(dpre, 1)
        g1 = _ln2_bwd(stream[:, cs], dy, y, stat[2:3, cs], home(cs, y4_s, c0))
        m_w1(y, dpre, 1)
        dhn = m_dh(gn, 0)
        hn, gpn = gelu_bwd_p(0, cn)
        dpren = mk_dpre(dhn, gpn, 0)
        g1b, dpqn = bwd1_a(0, g1)
        if last:
            m_fin(w2T, dw2Ta, gn, hn, hs(0))
        else:
            m_w2(gn, hn, 0)
        bwd1_b(0, cs, g1b, dpqn)
        dyacc[...] = m_dy(dpren, 0)
        yn = y2_s[0:D, cn]
        y4_s[0:D, c0] = yn
        if last:
            m_fin(w1c, dw1a, yn, dpren, hs(0))
        else:
            m_w1(yn, dpren, 0)
        env['r'] = ALLR
        return s

    if on('p4'):
        env['z'] = \
            lax.fori_loop(0, NT_ - 2, p4, 0)

    if on('b4'):
        p4(NT_ - 2, 0, True)
        gb = gcar[...]
        y = y4_s[0:D, c0]
        db2a[...] += gb.astype(F32)
        dh = m_dh(gb, 1)
        hh, gp = gelu_bwd(pre2[hs(1), cl].astype(F32))
        dpre = mk_dpre(dh, gp, 1)
        m_wq_fin(w2T, dw2Ta, gb, hh, 2)
        dy = dyacc[...] + m_dy(dpre, 1)
        g1 = _ln2_bwd(stream[:, cl], dy, y[0:D], stat[2:3, cl], home(cl, y4_s, c0), fast=True)
        m_wq_fin(w2T, dw2Ta, gb, hh, 3)
        g1b, dpqn = bwd1_a(0, g1)
        m_wq_fin(w1c, dw1a, y[0:D], dpre, 2)
        bwd1_b(0, cl, g1b, dpqn)
        pb = bf_a(0)
        m_wq_fin(w1c, dw1a, y[0:D], dpre, 3)
        bf_c(0, bf_b(0, pb))
        dw2Ta[:, 0:512] = pacc[:, 0:512] + _dot_nt(u_s[1, 0:D, T:TB], qk_s[1, 0:512, T:TB])
        dw2Ta[:, 512:D2] = _dot_nt(u_s[1, 0:D, 0:TB], qk_s[1, 512:D2, 0:TB])
        b2v[...] = jnp.sum(db2a[...].T, axis=0, keepdims=True).astype(BF).reshape(D)
        wo[...] = dwo_a[...].astype(BF)
    cp_dw1a = pltpu.make_async_copy(w1c.at[pl.ds(0, D), :], dw1_hbm, sem_out.at[1])
    cp_dw2a = pltpu.make_async_copy(w2T, dw2_hbm, sem_out.at[2])
    cp_db1 = pltpu.make_async_copy(b1v, db1_hbm, sem_out.at[3])
    cp_db2 = pltpu.make_async_copy(b2v, db2_hbm, sem_out.at[4])
    cp_dwo = pltpu.make_async_copy(wo, dwo_hbm, sem_out.at[5])
    cp_dwqkv = pltpu.make_async_copy(wraw, dwqkv_hbm, sem_out.at[6])
    cp_dw1a.start()
    cp_dw2a.start()
    cp_db2.start()
    cp_dwo.start()
    o3 = 7

    def cp_dx(s):
        if isinstance(s, int):
            lo, hi = max(s * TB - T, 0), min(s * TB + TB - T, S)
            w = pl.ds(lo, hi - lo)
        else:
            w = pl.ds(pl.multiple_of(s * TB - T, T), TB)
        return pltpu.make_async_copy(gs.at[:, w], dx_hbm.at[0, :, w], sem_out.at[o3 + s])

    def p5a(s, carry):
        cs = _cols(s, TB)
        ks = pl.ds(pl.multiple_of(TB + s * 384, 128), 384)
        dbrow[0:1, _cols(s, FQ)] = jnp.sum(db1a[_cols(s, FQ), :].T, axis=0, keepdims=True)
        dk = bwd2_a(0, cs)
        dw2Ta[:, 0:D2] += _dot_nt(u_s[1, 0:D, ks], qk_s[1, 0:D2, ks])
        dw2Ta[:, 0:D2] += _dot_nt(u_s[0, 0:D, cs], jnp.concatenate([qk_s[0, 0:D, cs], dk], axis=0))
        return carry

    if on('p5a'):
        lax.fori_loop(0, NB, p5a, 0)

    def sub(s, k):
        if isinstance(s, int):
            return pl.ds(s * TB + k * T, T)
        return pl.ds(pl.multiple_of(s * TB + k * T, T), T)

    def dx_fin(cs, du, fast=False):
        gs[:, cs] = _ln2_bwd(stream[:, cs], du, u_s[0, 0:D, cs], stat[0:1, cs], home(cs, u_s.r[0]), 1.0, False, fast)

    def dx_tile(s, first=False):
        if not first:
            dx_fin(sub(s, -1), dyacc[...])
        for k in range(TB // T - 1):
            dx_fin(sub(s, k), _dot(wx[...], qk_s[0, :, sub(s, k)]))
        dyacc[...] = _dot(wx[...], qk_s[0, :, sub(s, TB // T - 1)])
        cp_dx(s).start()

    env['r'] = ()
    if on('b5'):
        dwt = dw2Ta[:, 0:D2].astype(BF).T.astype(F32)
        dwq = _from_perm(ps0, dwt[0:D]).astype(BF)
        dwk = _from_perm(ps1, dwt[D:D2]).astype(BF)
        wraw[...] = jnp.concatenate([dwq, dwk, dwv_a[:, 0:D].astype(BF)], axis=0).T
        b1v[...] = dbrow[0:1, :].astype(BF).reshape(F)
        dx_tile(0, True)
    else:
        cp_dx(0).start()
    cp_dwqkv.start()
    cp_db1.start()

    def p5b(s, carry):
        env['z'] = s
        dx_tile(s)
        return s

    if on('p5b'):
        for s in range(1, NB):
            dx_tile(s)
        env['r'] = ALLR
        dx_fin(cl, dyacc[...], True)
    else:
        for s in range(1, NB):
            cp_dx(s).start()
    cp_dx(NB).start()

    cp_out.wait()
    cp_dw1a.wait()
    cp_dw2a.wait()
    cp_db1.wait()
    cp_db2.wait()
    cp_dwo.wait()
    cp_dwqkv.wait()
    for s in range(NB + 1):
        cp_dx(s).wait()


@jax.jit
def pallas_interleave_layers__linear_attn_block__mixer_channel_mlp__prompt_kernel(
    A_x: jax.Array,
    A_wqkv: jax.Array,
    A_wo: jax.Array,
    B_x: jax.Array,
    B_w1: jax.Array,
    B_b1: jax.Array,
    B_w2: jax.Array,
    B_b2: jax.Array,
    grad_out: jax.Array,
):
    del B_x
    V = pltpu.VMEM
    n_in = NB + 6 + 3 + 4
    n_out = 7 + NB + 1
    scratch = [
        V((D, S), BF),
        V((D, S), BF),
        V((D, D3), BF),
        V((D // 2, D3), U32),
        V((D3 // 2, D), U32),
        V((D, D), BF),
        V((DA, F), BF),
        V((F // 2, DA), U32),
        V((F // 2, D), U32),
        V((D, F), BF),
        V((F,), BF),
        V((D,), BF),
        V((D, 128), F32),
        V((D, F), F32),
        V((D, F), F32),
        V((F // 2, S), U32),
        V((D, S), F32),
        V((DA // 2, S), U32),
        V((DA // 2, S), U32),
        V((D3 // 2, S), U32),
        V((D3 // 2, S), U32),
        V((H, S), F32),
        V((H, S), F32),
        V((DA, S), BF),
        V((DA // 2, 2 * T), U32),
        V((8, S), F32),
        V((F, T), F32),
        V((8, F), F32),
        V((D, T), F32),
        V((D, T), F32),
        V((FQ // 2, T), U32),
        V((D // 2, T), U32),
        V((D, 3 * T), F32),
        V((2, NG, 64, 128), U32),
        V((D, DR), F32),
        V((2, D // 2, D), U32),
        V((2, D, 128), F32),
        V((2, D // 2, D), U32),
        V((D // 2, D), U32),
        V((D, DR), F32),
        V((D // 2, DA), U32),
        V((D, DA), F32),
        V((D, D), F32),
        V((D, 128), F32),
        V((5, D, 128), F32),
        V((5, D, 128), F32),
        V((2, D, T), F32),
        pltpu.SMEM((1,), jnp.int32),
        pltpu.SemaphoreType.DMA((n_in,)),
        pltpu.SemaphoreType.DMA((n_out,)),
    ]
    any_spec = pl.BlockSpec(memory_space=pl.ANY)
    out_shape = (
        jax.ShapeDtypeStruct((1, D, S), BF),
        jax.ShapeDtypeStruct((1, D, S), BF),
        jax.ShapeDtypeStruct((D, D3), BF),
        jax.ShapeDtypeStruct((D, D), BF),
        jax.ShapeDtypeStruct((D, F), BF),
        jax.ShapeDtypeStruct((F,), BF),
        jax.ShapeDtypeStruct((D, F), BF),
        jax.ShapeDtypeStruct((D,), BF),
    )
    outT, dxT, dwqkv, dwo, dw1, db1, dw2T, db2 = pl.pallas_call(
        _kernel,
        out_shape=out_shape,
        in_specs=[any_spec] * 8,
        out_specs=tuple([any_spec] * 8),
        scratch_shapes=scratch,
        compiler_params=pltpu.CompilerParams(vmem_limit_bytes=127 * 1024 * 1024),
    )(jnp.swapaxes(A_x, 1, 2), A_wqkv, A_wo, B_w1, B_b1, B_w2.T, B_b2, jnp.swapaxes(grad_out, 1, 2))
    return (jnp.swapaxes(outT, 1, 2), jnp.swapaxes(dxT, 1, 2), dwqkv, dwo, dw1, db1, dw2T.T, db2)
```

```python
import jax
import jax.numpy as jnp
from jax import lax
import jax.experimental.pallas as pl
import jax.experimental.pallas.tpu as pltpu

S, D, F = 2048, 576, 4608
H, DH = 32, 18
D3 = 3 * D
DA = 592
T = 128
NT_ = S // T
TB = 512
NB = S // TB
FH = F // 2
FQ = F // 4
D2 = 2 * D
DR = D + H
QA = 512
W1C = F // 3
NG = 5
WSTEP = 112
HEAD_LO = (0, 7, 13, 19, 25)
HEAD_HI = (6, 12, 18, 24, 31)

R3 = ()
R4 = ()
LN_EPS = 1e-5
PHI_EPS = 1e-6
GC0 = 0.7978845608028654
GC1 = 0.044715

BF = jnp.bfloat16


def on(name):
    return True


F32 = jnp.float32
U32 = jnp.uint32
_NN = (((1,), (0,)), ((), ()))
_NT = (((1,), (1,)), ((), ()))


def _dot(a, b):
    return lax.dot_general(a, b, _NN, preferred_element_type=F32)


def _dot_nt(a, b):
    return lax.dot_general(a, b, _NT, preferred_element_type=F32)


def _rows(m, nt):
    p = {1: 4, 2: 2}[nt % 4]
    return [slice(m // p * i, m // p * (i + 1)) for i in range(p)]


def _dot5(a, b, split, head=False):
    k = a.shape[1]
    nt = (k + 127) // 128
    if not split or nt % 4 == 0:
        return _dot(a, b)
    if head:
        odd, main = slice(0, nt % 4 * 128), slice(nt % 4 * 128, k)
    else:
        odd, main = slice(nt // 4 * 512, k), slice(0, nt // 4 * 512)
    tail = [_dot(a[r, odd], b[odd]) for r in _rows(a.shape[0], nt)]
    return _dot(a[:, main], b[main]) + jnp.concatenate(tail, axis=0)


def _dot5_nt(a, b):
    n = b.shape[0]
    nt = (n + 127) // 128
    n0 = nt // 4 * 512
    main = _dot_nt(a, b[0:n0])
    tail = [_dot_nt(a[r], b[n0:n]) for r in _rows(a.shape[0], nt)]
    return jnp.concatenate([main, jnp.concatenate(tail, axis=0)], axis=1)


def _colmean(x):
    n = x.shape[1]
    p = jnp.sum(x.reshape(9, 64, n), axis=0)
    p = p[0:32] + p[32:64]
    p = p[0:16] + p[16:32]
    p = p[0:8] + p[8:16]
    return jnp.sum(p, axis=0, keepdims=True) * (1.0 / D)


def _ln(x):
    m = _colmean(x)
    xc = x - m
    v = _colmean(xc * xc)
    rs = lax.rsqrt(v + LN_EPS)
    return xc * rs, rs


def _ln_bwd(dy, y, rs):
    a = _colmean(dy)
    b = _colmean(dy * y)
    return (dy - a - y * b) * rs


CR = 8
NCH = D // CR
FCR = 32


def _fold(p):
    while p.shape[0] > 8:
        h = p.shape[0] // 2
        p = p[0:h] + p[h:2 * h]
    return jnp.sum(p, axis=0, keepdims=True) * (1.0 / D)


def _ch(x, c, cr=CR):
    return x[c * cr:(c + 1) * cr]


def _nop(c, v):
    return c


PR = 32


_PO = (16, 17) + tuple(range(16))


def _cat(out):
    return jnp.concatenate(out[2:] + out[:2], axis=0)


def _b8(c, rows=PR):
    return jnp.broadcast_to(c, (rows, c.shape[1]))


def _pace(c, v):
    return c + 0.0 * v[0:1]


def _ln2(x, ld, fast=False):
    cr, pace = (FCR, _nop) if fast else (CR, _pace)
    acc = _ch(x, 0, cr)
    for c in range(1, D // cr):
        acc = acc + _ch(x, c, cr)
    m = _fold(acc)
    a1 = a2 = None
    x = ld(0)
    for c in range(D // cr):
        xc = _ch(x, c, cr) - m
        a1 = xc if a1 is None else a1 + xc
        a2 = xc * xc if a2 is None else a2 + xc * xc
    s1 = _fold(a1)
    s2 = _fold(a2)
    rs1 = lax.rsqrt(s2 + LN_EPS)
    m2 = s1 * rs1
    v2 = s2 * rs1 * rs1 - m2 * m2
    rs2 = lax.rsqrt(v2 + LN_EPS)
    rs12 = rs1 * rs2
    mc = _pace(m + s1, rs12)
    out = []
    x = ld(1)
    for c in _PO:
        y = (x[PR * c:PR * c + PR] - mc) * rs12
        mc = pace(mc, y)
        out.append(y.astype(BF))
    return _cat(out), rs12


def _ln2_bwd(g, dy, y, rs12, home, k=1.0 + LN_EPS, keep=True, fast=False):
    st, ld_t, ld_y = home
    a1 = a2 = None
    y = y.astype(F32)
    cr, pace = (FCR, _nop) if fast else (CR, _pace)
    for c in range(D // cr):
        d = _ch(dy, c, cr)
        t = d * _ch(y, c, cr)
        a1 = d if a1 is None else a1 + d
        a2 = t if a2 is None else a2 + t
    t = g + dy * rs12
    if ld_t is None:
        ld_t, ld_y = (lambda r: t[r]), (lambda r: y[r])
    else:
        st(slice(0, D), t)
    a = _fold(a1) * rs12
    b = _fold(a2) * (k * rs12)
    out = []
    for c in _PO:
        r = slice(PR * c, PR * c + PR)
        o = (ld_t(r) - ld_y(r).astype(F32) * b) - a
        b = pace(b, o)
        if keep:
            st(r, o)
        out.append(o.astype(BF))
    return _cat(out)


def _lnp(x, link=None, ld=None, fast=False):
    cr, pace = (FCR, _nop) if fast else (CR, _pace)
    acc = _ch(x, 0, cr)
    if link is not None:
        acc = acc + 0.0 * link
    for c in range(1, D // cr):
        acc = acc + _ch(x, c, cr)
    m = _fold(acc)
    a2 = None
    if ld is not None:
        x = ld(0)
    for c in range(D // cr):
        xc = _ch(x, c, cr) - m
        a2 = xc * xc if a2 is None else a2 + xc * xc
    rs = lax.rsqrt(_fold(a2) + LN_EPS)
    mc = _pace(m, rs)
    out = []
    if ld is not None:
        x = ld(1)
    for c in _PO:
        y = (x[PR * c:PR * c + PR] - mc) * rs
        mc = pace(mc, y)
        out.append(y.astype(BF))
    return _cat(out), rs, jnp.minimum(jnp.abs(y[0:1]), 1.0)


def _headsum(x):
    n = x.shape[1]
    p = x.reshape(DH, H, n)
    p = p[0:9] + p[9:18]
    q = (p[0] + p[1]) + (p[2] + p[3])
    r = (p[4] + p[5]) + (p[6] + p[7])
    return (q + r) + p[8]


def _headmul(x, c):
    n = x.shape[1]
    return (x.reshape(DH, H, n) * c[None]).reshape(D, n)


_LT = ((0, 128), (128, 128), (256, 128), (384, 128), (512, 64))


def _to_perm(scr, val, c0=0, c1=5):
    lt = [(c, o - 128 * c0, w) for c, (o, w) in enumerate(_LT)][c0:c1]
    for c, o, w in lt:
        scr[c, :, 0:w] = val[:, o:o + w]
    return jnp.concatenate(
        [jnp.concatenate([scr[c, pl.ds(j, H, stride=DH), 0:w] for c, o, w in lt], axis=1)
         for j in range(DH)], axis=0)


def _from_perm(scr, val):
    for j in range(DH):
        for c, (o, w) in enumerate(_LT):
            scr[c, pl.ds(j, H, stride=DH), 0:w] = val[H * j:H * j + H, o:o + w]
    return jnp.concatenate([scr[c, :, 0:w] for c, (o, w) in enumerate(_LT)], axis=1)


class _Pk:
    def __init__(self, ref):
        self.ref = ref

    def _idx(self, idx):
        nd = len(self.ref.shape)
        if idx is Ellipsis:
            return idx
        if not isinstance(idx, tuple):
            idx = (idx,)
        idx = list(idx) + [slice(None)] * (nd - len(idx))
        r = idx[nd - 2]
        if isinstance(r, slice):
            if r.start is not None or r.stop is not None:
                r = slice(r.start // 2, r.stop // 2)
        elif isinstance(r.start, int):
            r = pl.ds(r.start // 2, r.size // 2)
        else:
            r = pl.ds(pl.multiple_of(r.start // 2, 8), r.size // 2)
        idx[nd - 2] = r
        return tuple(idx)

    def __getitem__(self, idx):
        return pltpu.bitcast(self.ref[self._idx(idx)], BF)

    def __setitem__(self, idx, val):
        self.ref[self._idx(idx)] = pltpu.bitcast(val, U32)


class _L2:
    def __init__(self, a, b):
        self.r = (a, b)

    def __getitem__(self, idx):
        return self.r[idx[0]][idx[1:]]

    def __setitem__(self, idx, val):
        self.r[idx[0]][idx[1:]] = val


def _aug(y):
    r = lax.broadcasted_iota(jnp.int32, (DA - D, y.shape[1]), 0)
    return jnp.concatenate([y.astype(BF), jnp.where(r < 2, 1.0, 0.0).astype(BF)], axis=0)


def _phi(t):
    return jnp.where(t > 0, t + 1.0, jnp.exp(t)) + PHI_EPS


def _dphi_from_phi(p):
    return jnp.minimum(p - PHI_EPS, 1.0)


def _win(x, g):
    return x[WSTEP * g:WSTEP * g + 128]


def _assemble(parts):
    pieces = [parts[0][:WSTEP]]
    for g in range(NG - 1):
        pieces.append(parts[g][WSTEP:128] + parts[g + 1][0:16])
        pieces.append(parts[g + 1][16:WSTEP] if g + 1 < NG - 1 else parts[g + 1][16:128])
    return jnp.concatenate(pieces, axis=0)


def _head_mask(g):
    r = lax.broadcasted_iota(jnp.int32, (128, 128), 0) + WSTEP * g
    c = lax.broadcasted_iota(jnp.int32, (128, 128), 1) + WSTEP * g
    hr = (r * 3641) >> 16
    hc = (c * 3641) >> 16
    return (hr == hc) & (hr >= HEAD_LO[g]) & (hr <= HEAD_HI[g])


def _lane_fold(x):
    acc = x[:, 0:128]
    for j in range(1, x.shape[1] // 128):
        acc = acc + x[:, 128 * j:128 * (j + 1)]
    return acc


def _lane_tile(x128, n):
    if n == 128:
        return x128
    return jnp.concatenate([x128] * (n // 128), axis=1)


def _gelu_parts(pre):
    x2 = pre * pre
    t = jnp.tanh(pre * (GC0 + (GC0 * GC1) * x2))
    hp = 0.5 + 0.5 * t
    return x2, t, hp


def _cols(s, n):
    if isinstance(s, int):
        return pl.ds(s * n, n)
    return pl.ds(pl.multiple_of(s * n, n), n)


def _kernel(
    x_hbm, wqkv_hbm, wo_hbm, w1_hbm, b1_hbm, w2_hbm, b2_hbm, g_hbm,
    out_hbm, dx_hbm, dwqkv_hbm, dwo_hbm, dw1_hbm, db1_hbm, dw2_hbm, db2_hbm,
    xs, gs, wraw, wx, wT, wo, w1c, w1T, w2c, w2T, b1v, b2v, b2col,
    dw1a, dw2Ta, pre2, stream, u_0, u_1, qk_0, qk_1, rd_0, rd_1, y2_s, y4_s, stat, db1a, dbrow,
    oacc, dyacc, hcar, gcar,
    kvT, cacc, ctb, zb, mm, mmT, pacc, dctb, dwv_a, dwo_a, db2a, ps0, ps1, dtmp, zs,
    sem_in, sem_out,
):
    wx, wT, w1T, w2c, pre2, hcar, kvT, ctb, mm, mmT, dctb = [
        _Pk(r) for r in (wx, wT, w1T, w2c, pre2, hcar, kvT, ctb, mm, mmT, dctb)]
    u_s = _L2(_Pk(u_0), _Pk(u_1))
    qk_s = _L2(_Pk(qk_0), _Pk(qk_1))
    rd_s = _L2(rd_0, rd_1)
    y4_s, gcar = _Pk(y4_s), _Pk(gcar)

    ALLR = (0, 1, 2, 3, 4)
    env = {'r': ALLR}

    def zero(k):
        if k not in env['r']:
            return 0
        return env['z'] >> (20 + k)

    def _alt(cs, k):
        if k not in env['r']:
            return cs
        return pl.ds(pl.multiple_of(cs.start + (zero(k) << 7), 128), cs.size)

    def home(cs, yref, ys=None):
        def st(r, v):
            stream[r, cs] = v
        if 3 not in env['r']:
            return st, None, None
        return st, (lambda r: stream[r, _alt(cs, 3)]), (lambda r: yref[r, _alt(ys or cs, 3)])

    zs[0] = 0

    def cp_x(s):
        return pltpu.make_async_copy(x_hbm.at[0, :, _cols(s, TB)], xs.at[:, _cols(s, TB)], sem_in.at[s])

    k0 = NB
    def cp_wpart(lo, hi, k):
        return pltpu.make_async_copy(wqkv_hbm.at[:, pl.ds(lo, hi - lo)], wraw.at[:, pl.ds(lo, hi - lo)], sem_in.at[k])

    def cp_wk(lo, hi, k):
        w = (pl.ds(lo, hi - lo), pl.ds(512, D2 - 512))
        return pltpu.make_async_copy(wqkv_hbm.at[w], wraw.at[w], sem_in.at[k])

    cp_wka = cp_wk(0, 256, k0)
    cp_wkb = cp_wk(256, D, k0 + 11)
    cp_wq = cp_wpart(0, 512, k0 + 9)
    cp_wv = cp_wpart(D2, D3, k0 + 10)
    cp_wo = pltpu.make_async_copy(wo_hbm, wo, sem_in.at[k0 + 1])
    cp_b1 = pltpu.make_async_copy(b1_hbm, b1v, sem_in.at[k0 + 2])
    cp_b2 = pltpu.make_async_copy(b2_hbm, b2v, sem_in.at[k0 + 3])
    cp_w2 = pltpu.make_async_copy(w2_hbm.at[:, pl.ds(0, FQ)], w2T.at[:, pl.ds(0, FQ)], sem_in.at[k0 + 4])
    cp_w2b = pltpu.make_async_copy(w2_hbm.at[:, pl.ds(FQ, F - FQ)], w2T.at[:, pl.ds(FQ, F - FQ)], sem_in.at[k0 + 12])
    cp_g = pltpu.make_async_copy(g_hbm.at[0], gs, sem_in.at[k0 + 5])
    k1 = k0 + 6

    def cp_w1(c):
        return pltpu.make_async_copy(w1_hbm.at[:, _cols(c, W1C)], w1c.at[pl.ds(0, D), _cols(c, W1C)],
                                     sem_in.at[k1 + c])

    cp_x(0).start()
    cp_wka.start()
    cp_wkb.start()
    cp_wq.start()
    cp_x(1).start()
    cp_b1.start()
    cp_b2.start()
    cp_wv.start()
    cp_x(2).start()
    cp_x(3).start()
    for s in range(3):
        cp_w1(s).start()
    cp_wo.start()
    cp_w2.start()
    cp_w2b.start()

    def wrow(ref, g, base=0):
        return ref[base + WSTEP * g:base + WSTEP * g + 128, :]

    def front_a(l, cs, x, link=None, fast=False):
        u, rs, lk = _lnp(x, link, (lambda k: stream[:, _alt(cs, k)]) if l == 1 else None, fast)
        ub = _aug(u)
        u_s[l, :, cs] = ub
        stat[l:l + 1, cs] = rs
        return ub if link is None else lk

    def front_k(l, cs, ub):
        pkb = _phi(_dot5(wT[D:D2, :], ub[0:D], True)).astype(BF)
        qk_s[l, D2:D3, cs] = pkb
        return pkb

    def front_q(l, cs, ub):
        qk_s[l, 0:D, cs] = _phi(_dot5(wT[0:D, :], ub[0:D], True)).astype(BF)

    def front_b(l, cs, ub):
        pkb = front_k(l, cs, ub)
        front_q(l, cs, ub)
        return pkb

    def front_c(pkb, ub, first=False):
        if pkb.shape[1] == T:
            for m in range(4):
                dwv_a[144 * m:144 * m + 144, 512:DA] += _dot_nt(pkb[144 * m:144 * m + 144], ub[512:DA])
            dwv_a[:, 0:512] += _dot_nt(pkb, ub[0:512])
            return
        c = _dot_nt(pkb, ub)
        if first:
            dw1a[:, 0:DA] = c
        else:
            dw1a[:, 0:DA] += c

    def ff_a(l):
        c = dwv_a[...] if l else dw1a[:, 0:DA]
        zb[l] = jnp.broadcast_to(c[:, D:D + 1], (D, 128))
        ct = _from_perm(ps0, c[:, 0:D]).astype(BF)
        ctb[l] = ct
        return ct

    def ff_b(l, ct):
        kvs = []
        for g in range(NG):
            kv = jnp.where(_head_mask(g), _dot_nt(_win(ct, g), wrow(wT, g, D2)), 0.0)
            kvT[l, g] = kv.T.astype(BF)
            kvs.append(kv.astype(BF))
        return kvs

    def ff_c(l, kvs):
        m = _assemble([_dot(kvs[g], wrow(wo, g)) for g in range(NG)])
        mp = _to_perm(ps1, m).astype(BF)
        mm[l] = mp
        mmT[...] = mp.T

    def back_a(l, cs):
        pq = qk_s[l, 0:D, cs].astype(F32)
        rden = 1.0 / (_headsum(pq * zb[l]) + PHI_EPS)
        rd_s[l, :, cs] = rden
        return _headmul(pq, rden).astype(BF)

    def back_b(x, cs, pqn, split=False, fast=False):
        x1 = x + _dot5(mmT[...], pqn, split)
        env['x'] = x1
        if 0 in env['r']:
            stream[:, cs] = x1
            y, rs12 = _ln2(x1, lambda k: stream[:, _alt(cs, k)], fast)
        else:
            y, rs12 = _ln2(x1, lambda k: x1, fast)
        return _aug(y), rs12

    def res(cs):
        return (stream[:, _alt(cs, 2)] if 0 in env['r'] else env['x']) + b2col[...]

    def bwd1_a(l, gb, split=False):
        return gb, _dot5(mm[l], gb, split)

    def bwd1_b(l, cs, gb, dpqn, split=False):
        pq = qk_s[l, 0:D, cs].astype(F32)
        rden = rd_s[l, :, cs]
        z = zb[l]
        rd = rden
        r = None
        pqn = []
        rl = 4 in env['r']
        if rl:
            dtmp[0] = dpqn
        for j in range(DH):
            t = pq[H * j:H * j + H] * rd
            pqn.append(t.astype(BF))
            t = dpqn[H * j:H * j + H] * t
            r = t if r is None else r + t
            rd = _pace(rden, r)
        rb = r.astype(BF)
        for j in range(DH):
            rj = slice(H * j, H * j + H)
            w = _dphi_from_phi(qk_s[l, rj, _alt(cs, 4)].astype(F32) if rl else pq[rj]) * rden
            t = ((dtmp[zero(4), rj, :] if rl else dpqn[rj]) - z[rj] * r) * w
            r = _pace(r, t)
            qk_s[l, rj, cs] = t.astype(BF)
        pqn = jnp.concatenate(pqn, axis=0)
        gr = jnp.concatenate([gb, rb], axis=0)
        pa = pacc if l else cacc
        if split:
            pa[:, 0:512] += _dot_nt(pqn, gr[0:512])
            for m in range(4):
                pa[144 * m:144 * m + 144, 512:DR] += _dot_nt(pqn[144 * m:144 * m + 144], gr[512:DR])
        else:
            pa[...] += _dot_nt(pqn, gr)

    def bf_a(l):
        p = (pacc if l else cacc)[...]
        tl = p[:, 512:DR]
        rr = lax.broadcasted_iota(jnp.int32, tl.shape, 0)
        cc = lax.broadcasted_iota(jnp.int32, tl.shape, 1)
        dz = -jnp.sum(jnp.where(cc - (D - 512) == (rr & (H - 1)), tl, 0.0), axis=1, keepdims=True)
        hi = dz.astype(BF).astype(F32)
        ce = lax.broadcasted_iota(jnp.int32, (D, DA - D), 1)
        dctb[:, D:DA] = jnp.where(ce == 0, hi, jnp.where(ce == 1, dz - hi, 0.0)).astype(BF)
        pb = _from_perm(ps0, p[:, 0:D]).astype(BF)
        return pb

    def acc_l(ref, l, val):
        if l == 1:
            ref[:, 0:D] = val
        else:
            ref[:, 0:D] += val

    def bf_b(l, pb):
        ds_ = [jnp.where(_head_mask(g), _dot_nt(_win(pb, g), wrow(wo, g)), 0.0) for g in range(NG)]
        acc_l(dwo_a, l, _assemble([_dot(kvT[l, g], _win(pb, g)) for g in range(NG)]))
        return ds_

    def bf_c(l, ds_):
        dct = _assemble([_dot(ds_[g].astype(BF), wrow(wT, g, D2)) for g in range(NG)])
        dp = _to_perm(ps1, dct).astype(BF)
        dctb[:, 0:D] = dp
        wx[:, D2:D3] = dp.T
        acc_l(dwv_a, l, _assemble([_dot(ds_[g].T.astype(BF), ctb[l, WSTEP * g:WSTEP * g + 128, :]) for g in range(NG)]))

    def bwd2_a(l, cs, split=False):
        dpk = _dot5(dctb[...], u_s[l, :, cs], split)
        dk = (dpk * _dphi_from_phi(qk_s[l, D2:D3, cs].astype(F32))).astype(BF)
        qk_s[l, D:D2, cs] = dk
        return dk

    def bwd2_b(l, cs, dk=None, keep=True, bal=False, fast=False):
        if dk is None:
            rhs = qk_s[l, :, cs]
        else:
            rhs = jnp.concatenate([qk_s[l, 0:D, cs], dk, qk_s[l, D2:D3, cs]], axis=0)
        du = _dot5(wx[...], rhs, bal)
        return _ln2_bwd(stream[:, cs], du, u_s[l, 0:D, cs], stat[l:l + 1, cs], home(cs, u_s.r[l]), 1.0, keep, fast)

    def hs(h):
        return pl.ds(h * FH, FH)

    def qs(c):
        return pl.ds(c * FQ, FQ)

    def f_pre(y, cs, c):
        pre = _dot5(w1T[qs(c), :], y, True)
        pre2[qs(c), cs] = pre.astype(BF)
        _, _, hp = _gelu_parts(pre)
        return (pre * hp).astype(BF)

    def f_out(hh, c):
        return _dot5(w2T[:, qs(c)], hh, True, True)

    def gelu_bwd(pre):
        x2, t, hp = _gelu_parts(pre)
        hh = (pre * hp).astype(BF)
        gp = hp + (0.5 * pre) * (1.0 - t * t) * (GC0 + (3.0 * GC0 * GC1) * x2)
        return hh, gp

    def gelu_bwd_p(h, cs):
        GR = 64
        hs_, gs_ = [], []
        k = jnp.full((1, T), GC0, F32)
        for c in range(FH // GR):
            pre = pre2[h * FH + c * GR:h * FH + (c + 1) * GR, cs].astype(F32)
            x2 = pre * pre
            t = jnp.tanh(pre * (k + (GC0 * GC1) * x2))
            k = _pace(k, t)
            hp = 0.5 + 0.5 * t
            hs_.append((pre * hp).astype(BF))
            gs_.append(hp + (0.5 * pre) * (1.0 - t * t) * (GC0 + (3.0 * GC0 * GC1) * x2))
        return jnp.concatenate(hs_, axis=0), jnp.concatenate(gs_, axis=0)

    def m_dh(gb, h):
        return _dot5(w2c[hs(h), :], gb, True)

    def m_dhq(gb, c):
        return _dot(w2c[qs(c), :], gb)

    def m_pre(y, h):
        return _dot5(w1T[hs(h), :], y, True)

    def m_dy(dpre, h, bal=False):
        return _dot5(w1c[0:D, hs(h)], dpre, bal, True)

    def m_out(hh, h):
        return _dot(w2T[:, hs(h)], hh)

    def acc_to(ref, sl, val, keep):
        if keep is True:
            ref[:, sl] += val
        elif keep is False:
            ref[:, sl] = val
        else:
            ref[:, sl] = jnp.where(keep, ref[:, sl], 0.0) + val

    def m_w1(y, dpre, h, keep=True):
        acc_to(dw1a, hs(h), _dot_nt(y[0:D], dpre), keep)

    def mk_dpre(dh, gp, h):
        dp = dh * gp
        db1a[hs(h), :] += dp
        return dp.astype(BF)

    def m_w2(gb, hh, h, keep=True):
        acc_to(dw2Ta, hs(h), _dot_nt(gb, hh), keep)

    def m_wq(ref, a, b, c):
        acc_to(ref, qs(c), _dot5_nt(a, b[(c - 2) * FQ:(c - 1) * FQ]), True)

    def m_fin(dst, ref, a, b, sl):
        val = ref[:, sl] + _dot_nt(a, b)
        dst[0:D, sl] = val.astype(BF)

    def m_wq_fin(dst, ref, a, b, c):
        m_fin(dst, ref, a, b[(c - 2) * FQ:(c - 1) * FQ], qs(c))

    def clear(i, carry):
        r = pl.ds(pl.multiple_of(i * 32, 32), 32)
        for ref in (pacc, dwv_a, cacc, db2a):
            ref[r, :] = jnp.zeros((32, ref.shape[1]), F32)
        db1a[pl.ds(pl.multiple_of(i * 256, 256), 256), :] = jnp.zeros((256, T), F32)
        return carry

    lax.fori_loop(0, D // 32, clear, 1)

    def ln0(s, chain=4, lk=None, ks=(0, 1, 2, 3), fast=False):
        for k in ks:
            cs = pl.ds(s * TB + k * T, T)
            if k % chain == 0 and (k or lk is None):
                lk = jnp.zeros((1, T), F32)
            lk = front_a(0, cs, xs[:, cs].astype(F32), lk, fast)
        return lk

    def k_part(s):
        cs = _cols(s, TB)
        qk_s[0, D2:D3, cs] = _phi(_dot(wT[D:D2, :], u_s[0, 0:D, cs])).astype(BF)

    def q_part(lo, hi):
        cs = pl.ds(lo * T, (hi - lo) * T)
        qk_s[0, 0:D, cs] = _phi(_dot(wT[0:D, :], u_s[0, 0:D, cs])).astype(BF)

    def c_part(s):
        cs = _cols(s, TB)
        front_c(qk_s[0, D2:D3, cs], u_s[0, :, cs], s == 0)

    def w1_t(c):
        w1T[_cols(c, W1C), :] = w1c[:, _cols(c, W1C)].T

    cp_x(0).wait()
    ln0(0, 4, None, (0, 1, 2), True)
    cp_wka.wait()
    wta = wraw[0:256, 512:D2].T
    wT[D:D2, 0:256] = _to_perm(ps1, wta[64:640].astype(F32), 0, 2).astype(BF)
    ln0(0, 1, None, (3,), True)
    stream[:, 0:TB] = _dot(wT[D:D2, 0:128], u_s[0, 0:128, 0:TB])
    cp_wkb.wait()
    wtb = wraw[256:D, 512:D2].T
    wT[D:D2, 256:D] = _to_perm(ps1, wtb[64:640].astype(F32), 2, 5).astype(BF)
    qk_s[0, D2:D3, 0:TB] = _phi(
        stream[:, 0:TB] + _dot(wT[D:D2, 128:256], u_s[0, 128:256, 0:TB])
        + _dot(wT[D:D2, 256:D], u_s[0, 256:D, 0:TB])).astype(BF)
    wtk = jnp.concatenate([wta[0:64], wtb[0:64]], axis=1)
    dw1a[:, 0:256] = _dot_nt(qk_s[0, D2:D3, 0:TB], u_s[0, 0:256, 0:TB])
    cp_wq.wait()
    cp_x(1).wait()
    cp_b1.wait()
    cp_b2.wait()
    wtq = jnp.concatenate([wraw[:, 0:512].T, wtk[0:64]], axis=0)
    wT[0:D, :] = _to_perm(ps0, wtq.astype(F32)).astype(BF)
    dw1a[:, 256:DA] = _dot_nt(qk_s[0, D2:D3, 0:TB], u_s[0, 256:DA, 0:TB])
    b2col[...] = jnp.broadcast_to(b2v[...].reshape(1, D).astype(F32), (128, D)).T
    rid = lax.broadcasted_iota(jnp.int32, (DA - D, F), 0)
    w1c[D:DA, :] = jnp.where(
        rid == 0, jnp.broadcast_to(b1v[...].reshape(1, F).astype(F32), (DA - D, F)), 0.0).astype(BF)
    ln0(1)
    q_part(0, 4)
    k_part(1)
    for t_ in (4, 5):
        front_q(0, _cols(t_, T), u_s[0, :, _cols(t_, T)])
    c_part(1)
    cp_wv.wait()
    cp_x(2).wait()
    cp_x(3).wait()
    cp_w1(0).wait()
    cp_w1(1).wait()
    lk = ln0(2)
    for t_ in (6, 7):
        front_q(0, _cols(t_, T), u_s[0, :, _cols(t_, T)])
    wT[D2:D3, :] = wraw[:, D2:D3].T
    w1_t(0)
    ln0(3, 4, lk)
    k_part(2)
    c_part(2)
    w1_t(1)
    k_part(3)
    q_part(8, 12)
    c_part(3)
    cp_w1(2).wait()
    cp_wo.wait()
    cp_w2.wait()

    def step_2(s, first=False, last=False):
        cs = _cols(s, T)
        cn = _cols(s + 1, T)
        pqn = back_a(0, cn)
        if not first:
            o = oacc[...] + f_out(hcar[...], 1)
        yn, rs12 = back_b(xs[:, cn].astype(F32), cn, pqn, True)
        if first:
            q_part(15, 16)
        else:
            y = y2_s[:, cs]
            h2 = f_pre(y, cs, 2)
            h3 = f_pre(y, cs, 3)
            o = o + f_out(h2, 2)
        y2_s[:, cn] = yn
        stat[2:3, cn] = rs12
        h0n = f_pre(yn, cn, 0)
        if not first:
            x2 = o + f_out(h3, 3)
            stream[:, cs] = x2
            ub = front_a(1, cs, x2)
        hcar[...] = f_pre(yn, cn, 1)
        if last:
            pkb = front_k(1, cs, ub)
        oacc[...] = res(cn) + f_out(h0n, 0)
        if last:
            front_c(pkb, ub)
        elif not first:
            front_c(front_b(1, cs, ub), ub)

    env['z'] = zs[0]
    if on('b1'):
        ct = ff_a(0)
        q_part(12, 13)
        ff_c(0, ff_b(0, ct))
        q_part(13, 15)
        w1_t(2)
        step_2(-1, first=True)

    def p2(s, carry):
        env['z'] = s
        for s2 in (2 * s, 2 * s + 1):
            j = pl.ds(pl.multiple_of(jnp.minimum(s2, 11) * 384, 384), 384)
            w2c[j, :] = w2T[:, j].T
            step_2(s2)
        return s

    cp_w2b.wait()
    cp_g.start()
    if on('p2'):
        env['z'] = \
            lax.fori_loop(0, NT_ // 2 - 1, p2, 0)

    cp_g.wait()
    cl = _cols(NT_ - 1, T)
    c0 = _cols(0, T)
    if on('b2'):
        step_2(NT_ - 2, last=True)
        cp_ = _cols(NT_ - 2, T)
        y = y2_s[:, cl]
        gn = gs[:, c0]
        h2 = f_pre(y, cl, 2)
        o = oacc[...] + f_out(hcar[...], 1)
        h3 = f_pre(y, cl, 3)
        o = o + f_out(h2, 2)
        x2 = o + f_out(h3, 3)
        stream[:, cl] = x2
        ub = front_a(1, cl, x2, None, True)
        FE = FH // 8
        dhe = []

        def fill_dh(n):
            e = len(dhe)
            for i in range(e, e + n):
                dhe.append(_dot(w2c[i * FE:(i + 1) * FE, 0:512], gn[0:512]))

        front_q(1, cp_, u_s[1, :, cp_])
        fill_dh(1)
        pkb = front_k(1, cl, ub)
        fill_dh(1)
        front_c(pkb, ub)
        ct = ff_a(1)
        front_q(1, cl, ub)
        kvs = ff_b(1, ct)
        fill_dh(1)
        ff_c(1, kvs)
        dht = jnp.concatenate([_dot(w2c[r, 512:D], gn[512:D]) for r in _rows(FH, 1)], axis=0)
        fill_dh(1)
        yn, rs12 = back_b(stream[:, c0], c0, back_a(1, c0), True, True)
        y4_s[:, c0] = yn
        gcar[...] = gn
        stat[3:4, c0] = rs12
        fill_dh(4)
        hn, gpn = gelu_bwd(m_pre(yn, 0))
        dpren = mk_dpre(jnp.concatenate(dhe, axis=0) + dht, gpn, 0)
        oacc[...] = res(c0) + m_out(hn, 0)
        dyacc[...] = m_dy(dpren, 0)
        m_w1(yn, dpren, 0, False)
        m_w2(gn, hn, 0, False)

    def p3(s, carry):
        env['z'] = s
        env['r'] = R3
        j = pl.ds(pl.multiple_of(jnp.minimum(s, 8) * 128, 128), 128)
        wx[:, j] = wT[j, :].T
        cs = _cols(s, T)
        cn = _cols(s + 1, T)
        gb = gcar[...]
        gn = gs[:, cn]
        pqn = back_a(1, cn)
        dh = m_dh(gb, 1)
        yn, rs12 = back_b(stream[:, cn], cn, pqn, True)
        hh, gp = gelu_bwd(m_pre(y4_s[:, c0], 1))
        stat[3:4, cn] = rs12
        dpre = mk_dpre(dh, gp, 1)
        dy = dyacc[...] + m_dy(dpre, 1)
        g = gb.astype(F32)
        db2a[...] += g
        g3 = _ln2_bwd(g, dy, y4_s[0:D, c0], stat[3:4, cs], home(cs, y4_s, c0))
        xs[:, cs] = (oacc[...] + m_out(hh, 1)).astype(BF)
        m_w1(y4_s[0:D, c0], dpre, 1, s > 0)
        m_w2(gb, hh, 1, s > 0)
        y4_s[:, c0] = yn
        gcar[...] = gn
        dhn = m_dh(gn, 0)
        g3b, dpqn = bwd1_a(1, g3, True)
        hn, gpn = gelu_bwd(m_pre(yn, 0))
        dpren = mk_dpre(dhn, gpn, 0)
        bwd1_b(1, cs, g3b, dpqn, True)
        dyacc[...] = m_dy(dpren, 0)
        oacc[...] = res(cn) + m_out(hn, 0)
        m_w1(yn, dpren, 0)
        m_w2(gn, hn, 0)
        env['r'] = ALLR
        return s

    if on('p3'):
        env['z'] = \
            lax.fori_loop(0, NT_ - 1, p3, 0)

    cp_out = pltpu.make_async_copy(xs, out_hbm.at[0], sem_out.at[0])
    if on('b3'):
        gb = gcar[...]
        y = y4_s[:, c0]
        hh, gp = gelu_bwd(m_pre(y, 1))
        dh = m_dh(gb, 1)
        dpre = mk_dpre(dh, gp, 1)
        dy = dyacc[...] + m_dy(dpre, 1, True)
        g = gb.astype(F32)
        db2a[...] += g
        g3 = _ln2_bwd(g, dy, y[0:D], stat[3:4, cl], home(cl, y4_s, c0), fast=True)
        o = oacc[...] + f_out(hh[0:FQ], 2)
        g3b, dpqn = bwd1_a(1, g3, True)
        m_wq(dw1a, y[0:D], dpre, 2)
        bwd1_b(1, cl, g3b, dpqn, True)
        pb = bf_a(1)
        m_wq(dw1a, y[0:D], dpre, 3)
        bf_c(1, bf_b(1, pb))
        m_wq(dw2Ta, gb, hh, 2)
        dk = bwd2_a(1, c0, True)
        m_wq(dw2Ta, gb, hh, 3)
        gn = bwd2_b(1, c0, dk, True, True, True)
        pacc[:, 0:512] = _dot_nt(u_s[1, 0:D, 0:T], qk_s[1, 0:512, 0:T])
        xs[:, cl] = (o + f_out(hh[FQ:FH], 3)).astype(BF)
        gcar[...] = gn
        hn, gpn = gelu_bwd(pre2[hs(0), c0].astype(F32))
        dhn = m_dh(gn, 0)
        dpren = mk_dpre(dhn, gpn, 0)
        m_w2(gn, hn, 0)
        yn = y2_s[0:D, c0]
        y4_s[0:D, c0] = yn
        m_w1(yn, dpren, 0)
        dyacc[...] = m_dy(dpren, 0, True)
    cp_out.start()

    def p4(s, carry, last=False):
        if not last:
            env['z'] = s
            env['r'] = R4
        cs = _cols(s, T)
        cn = _cols(s + 1, T)
        dk = bwd2_a(1, cn, True)
        gb = gcar[...]
        dh = m_dh(gb, 1)
        db2a[...] += gb.astype(F32)
        gn = bwd2_b(1, cn, dk)
        hh, gp = gelu_bwd_p(1, cs)
        dpre = mk_dpre(dh, gp, 1)
        m_w2(gb, hh, 1)
        gcar[...] = gn
        y = y4_s[0:D, c0]
        dy = dyacc[...] + m_dy(dpre, 1)
        g1 = _ln2_bwd(stream[:, cs], dy, y, stat[2:3, cs], home(cs, y4_s, c0))
        m_w1(y, dpre, 1)
        dhn = m_dh(gn, 0)
        hn, gpn = gelu_bwd_p(0, cn)
        dpren = mk_dpre(dhn, gpn, 0)
        g1b, dpqn = bwd1_a(0, g1)
        if last:
            m_fin(w2T, dw2Ta, gn, hn, hs(0))
        else:
            m_w2(gn, hn, 0)
        bwd1_b(0, cs, g1b, dpqn)
        dyacc[...] = m_dy(dpren, 0)
        yn = y2_s[0:D, cn]
        y4_s[0:D, c0] = yn
        if last:
            m_fin(w1c, dw1a, yn, dpren, hs(0))
        else:
            m_w1(yn, dpren, 0)
        env['r'] = ALLR
        return s

    if on('p4'):
        env['z'] = \
            lax.fori_loop(0, NT_ - 2, p4, 0)

    if on('b4'):
        p4(NT_ - 2, 0, True)
        gb = gcar[...]
        y = y4_s[0:D, c0]
        db2a[...] += gb.astype(F32)
        dh = m_dh(gb, 1)
        hh, gp = gelu_bwd(pre2[hs(1), cl].astype(F32))
        dpre = mk_dpre(dh, gp, 1)
        m_wq_fin(w2T, dw2Ta, gb, hh, 2)
        dy = dyacc[...] + m_dy(dpre, 1)
        g1 = _ln2_bwd(stream[:, cl], dy, y[0:D], stat[2:3, cl], home(cl, y4_s, c0), fast=True)
        m_wq_fin(w2T, dw2Ta, gb, hh, 3)
        g1b, dpqn = bwd1_a(0, g1)
        m_wq_fin(w1c, dw1a, y[0:D], dpre, 2)
        bwd1_b(0, cl, g1b, dpqn)
        pb = bf_a(0)
        m_wq_fin(w1c, dw1a, y[0:D], dpre, 3)
        bf_c(0, bf_b(0, pb))
        dw2Ta[:, 0:512] = pacc[:, 0:512] + _dot_nt(u_s[1, 0:D, T:TB], qk_s[1, 0:512, T:TB])
        dw2Ta[:, 512:D2] = _dot_nt(u_s[1, 0:D, 0:TB], qk_s[1, 512:D2, 0:TB])
        b2v[...] = jnp.sum(db2a[...].T, axis=0, keepdims=True).astype(BF).reshape(D)
        wo[...] = dwo_a[...].astype(BF)
    cp_dw1a = pltpu.make_async_copy(w1c.at[pl.ds(0, D), :], dw1_hbm, sem_out.at[1])
    cp_dw2a = pltpu.make_async_copy(w2T, dw2_hbm, sem_out.at[2])
    cp_db1 = pltpu.make_async_copy(b1v, db1_hbm, sem_out.at[3])
    cp_db2 = pltpu.make_async_copy(b2v, db2_hbm, sem_out.at[4])
    cp_dwo = pltpu.make_async_copy(wo, dwo_hbm, sem_out.at[5])
    cp_dwqkv = pltpu.make_async_copy(wraw, dwqkv_hbm, sem_out.at[6])
    cp_dw1a.start()
    cp_dw2a.start()
    cp_db2.start()
    cp_dwo.start()
    o3 = 7

    def cp_dx(s):
        if isinstance(s, int):
            lo, hi = max(s * TB - T, 0), min(s * TB + TB - T, S)
            w = pl.ds(lo, hi - lo)
        else:
            w = pl.ds(pl.multiple_of(s * TB - T, T), TB)
        return pltpu.make_async_copy(gs.at[:, w], dx_hbm.at[0, :, w], sem_out.at[o3 + s])

    def p5a(s, carry):
        cs = _cols(s, TB)
        ks = pl.ds(pl.multiple_of(TB + s * 384, 128), 384)
        dbrow[0:1, _cols(s, FQ)] = jnp.sum(db1a[_cols(s, FQ), :].T, axis=0, keepdims=True)
        pre2[0:D, TB:TB + 384] = u_s[1, 0:D, ks]
        pre2[0:D, 0:TB] = u_s[0, 0:D, cs]
        dk = bwd2_a(0, cs)
        dw2Ta[:, 0:D2] += _dot_nt(pre2[0:D, TB:TB + 384], qk_s[1, 0:D2, ks])
        dw2Ta[:, 0:D2] += _dot_nt(pre2[0:D, 0:TB], jnp.concatenate([qk_s[0, 0:D, cs], dk], axis=0))
        return carry

    if on('p5a'):
        lax.fori_loop(0, NB, p5a, 0)

    def sub(s, k):
        if isinstance(s, int):
            return pl.ds(s * TB + k * T, T)
        return pl.ds(pl.multiple_of(s * TB + k * T, T), T)

    def dx_fin(cs, du, fast=False):
        gs[:, cs] = _ln2_bwd(stream[:, cs], du, u_s[0, 0:D, cs], stat[0:1, cs], home(cs, u_s.r[0]), 1.0, False, fast)

    def dx_tile(s, first=False):
        if not first:
            dx_fin(sub(s, -1), dyacc[...])
        for k in range(TB // T - 1):
            dx_fin(sub(s, k), _dot(wx[...], qk_s[0, :, sub(s, k)]))
        dyacc[...] = _dot(wx[...], qk_s[0, :, sub(s, TB // T - 1)])
        cp_dx(s).start()

    env['r'] = ()
    if on('b5'):
        dwt = dw2Ta[:, 0:D2].astype(BF).T.astype(F32)
        dwq = _from_perm(ps0, dwt[0:D]).astype(BF)
        dwk = _from_perm(ps1, dwt[D:D2]).astype(BF)
        wraw[...] = jnp.concatenate([dwq, dwk, dwv_a[:, 0:D].astype(BF)], axis=0).T
        b1v[...] = dbrow[0:1, :].astype(BF).reshape(F)
        dx_tile(0, True)
    else:
        cp_dx(0).start()
    cp_dwqkv.start()
    cp_db1.start()

    def p5b(s, carry):
        env['z'] = s
        dx_tile(s)
        return s

    if on('p5b'):
        for s in range(1, NB):
            dx_tile(s)
        env['r'] = ALLR
        dx_fin(cl, dyacc[...], True)
    else:
        for s in range(1, NB):
            cp_dx(s).start()
    cp_dx(NB).start()

    cp_out.wait()
    cp_dw1a.wait()
    cp_dw2a.wait()
    cp_db1.wait()
    cp_db2.wait()
    cp_dwo.wait()
    cp_dwqkv.wait()
    for s in range(NB + 1):
        cp_dx(s).wait()


@jax.jit
def pallas_interleave_layers__linear_attn_block__mixer_channel_mlp__prompt_kernel(
    A_x: jax.Array,
    A_wqkv: jax.Array,
    A_wo: jax.Array,
    B_x: jax.Array,
    B_w1: jax.Array,
    B_b1: jax.Array,
    B_w2: jax.Array,
    B_b2: jax.Array,
    grad_out: jax.Array,
):
    del B_x
    V = pltpu.VMEM
    n_in = NB + 6 + 3 + 4
    n_out = 7 + NB + 1
    scratch = [
        V((D, S), BF),
        V((D, S), BF),
        V((D, D3), BF),
        V((D // 2, D3), U32),
        V((D3 // 2, D), U32),
        V((D, D), BF),
        V((DA, F), BF),
        V((F // 2, DA), U32),
        V((F // 2, D), U32),
        V((D, F), BF),
        V((F,), BF),
        V((D,), BF),
        V((D, 128), F32),
        V((D, F), F32),
        V((D, F), F32),
        V((F // 2, S), U32),
        V((D, S), F32),
        V((DA // 2, S), U32),
        V((DA // 2, S), U32),
        V((D3 // 2, S), U32),
        V((D3 // 2, S), U32),
        V((H, S), F32),
        V((H, S), F32),
        V((DA, S), BF),
        V((DA // 2, 2 * T), U32),
        V((8, S), F32),
        V((F, T), F32),
        V((8, F), F32),
        V((D, T), F32),
        V((D, T), F32),
        V((FQ // 2, T), U32),
        V((D // 2, T), U32),
        V((2, NG, 64, 128), U32),
        V((D, DR), F32),
        V((2, D // 2, D), U32),
        V((2, D, 128), F32),
        V((2, D // 2, D), U32),
        V((D // 2, D), U32),
        V((D, DR), F32),
        V((D // 2, DA), U32),
        V((D, DA), F32),
        V((D, D), F32),
        V((D, 128), F32),
        V((5, D, 128), F32),
        V((5, D, 128), F32),
        V((2, D, T), F32),
        pltpu.SMEM((1,), jnp.int32),
        pltpu.SemaphoreType.DMA((n_in,)),
        pltpu.SemaphoreType.DMA((n_out,)),
    ]
    any_spec = pl.BlockSpec(memory_space=pl.ANY)
    out_shape = (
        jax.ShapeDtypeStruct((1, D, S), BF),
        jax.ShapeDtypeStruct((1, D, S), BF),
        jax.ShapeDtypeStruct((D, D3), BF),
        jax.ShapeDtypeStruct((D, D), BF),
        jax.ShapeDtypeStruct((D, F), BF),
        jax.ShapeDtypeStruct((F,), BF),
        jax.ShapeDtypeStruct((D, F), BF),
        jax.ShapeDtypeStruct((D,), BF),
    )
    outT, dxT, dwqkv, dwo, dw1, db1, dw2T, db2 = pl.pallas_call(
        _kernel,
        out_shape=out_shape,
        in_specs=[any_spec] * 8,
        out_specs=tuple([any_spec] * 8),
        scratch_shapes=scratch,
        compiler_params=pltpu.CompilerParams(vmem_limit_bytes=127 * 1024 * 1024),
    )(jnp.swapaxes(A_x, 1, 2), A_wqkv, A_wo, B_w1, B_b1, B_w2.T, B_b2, jnp.swapaxes(grad_out, 1, 2))
    return (jnp.swapaxes(outT, 1, 2), jnp.swapaxes(dxT, 1, 2), dwqkv, dwo, dw1, db1, dw2T.T, db2)
```

```python
import jax
import jax.numpy as jnp
from jax import lax
import jax.experimental.pallas as pl
import jax.experimental.pallas.tpu as pltpu

S, D, F = 2048, 576, 4608
H, DH = 32, 18
D3 = 3 * D
DA = 592
T = 128
NT_ = S // T
TB = 512
NB = S // TB
FH = F // 2
FQ = F // 4
D2 = 2 * D
DR = D + H
W1C = F // 3
NG = 5
WSTEP = 112
HEAD_LO = (0, 7, 13, 19, 25)
HEAD_HI = (6, 12, 18, 24, 31)

R3 = ()
R4 = ()
LN_EPS = 1e-5
PHI_EPS = 1e-6
GC0 = 0.7978845608028654
GC1 = 0.044715

BF = jnp.bfloat16


def on(name):
    return True


F32 = jnp.float32
U32 = jnp.uint32
_NN = (((1,), (0,)), ((), ()))
_NT = (((1,), (1,)), ((), ()))


def _dot(a, b):
    return lax.dot_general(a, b, _NN, preferred_element_type=F32)


def _dot_nt(a, b):
    return lax.dot_general(a, b, _NT, preferred_element_type=F32)


def _rows(m, nt):
    p = {1: 4, 2: 2}[nt % 4]
    return [slice(m // p * i, m // p * (i + 1)) for i in range(p)]


def _dot5(a, b, split, head=False):
    k = a.shape[1]
    nt = (k + 127) // 128
    if not split or nt % 4 == 0:
        return _dot(a, b)
    if head:
        odd, main = slice(0, nt % 4 * 128), slice(nt % 4 * 128, k)
    else:
        odd, main = slice(nt // 4 * 512, k), slice(0, nt // 4 * 512)
    tail = [_dot(a[r, odd], b[odd]) for r in _rows(a.shape[0], nt)]
    return _dot(a[:, main], b[main]) + jnp.concatenate(tail, axis=0)


def _dot5_nt(a, b):
    n = b.shape[0]
    nt = (n + 127) // 128
    n0 = nt // 4 * 512
    main = _dot_nt(a, b[0:n0])
    tail = [_dot_nt(a[r], b[n0:n]) for r in _rows(a.shape[0], nt)]
    return jnp.concatenate([main, jnp.concatenate(tail, axis=0)], axis=1)


CR = 8
FCR = 32


def _fold(p):
    while p.shape[0] > 8:
        h = p.shape[0] // 2
        p = p[0:h] + p[h:2 * h]
    return jnp.sum(p, axis=0, keepdims=True) * (1.0 / D)


def _ch(x, c, cr=CR):
    return x[c * cr:(c + 1) * cr]


def _nop(c, v):
    return c


PR = 32


_PO = (16, 17) + tuple(range(16))


def _cat(out):
    return jnp.concatenate(out[2:] + out[:2], axis=0)


def _pace(c, v):
    return c + 0.0 * v[0:1]


def _ln2(x, ld, fast=False):
    cr, pace = (FCR, _nop) if fast else (CR, _pace)
    acc = _ch(x, 0, cr)
    for c in range(1, D // cr):
        acc = acc + _ch(x, c, cr)
    m = _fold(acc)
    a1 = a2 = None
    x = ld(0)
    for c in range(D // cr):
        xc = _ch(x, c, cr) - m
        a1 = xc if a1 is None else a1 + xc
        a2 = xc * xc if a2 is None else a2 + xc * xc
    s1 = _fold(a1)
    s2 = _fold(a2)
    rs1 = lax.rsqrt(s2 + LN_EPS)
    m2 = s1 * rs1
    v2 = s2 * rs1 * rs1 - m2 * m2
    rs2 = lax.rsqrt(v2 + LN_EPS)
    rs12 = rs1 * rs2
    mc = _pace(m + s1, rs12)
    out = []
    x = ld(1)
    for c in _PO:
        y = (x[PR * c:PR * c + PR] - mc) * rs12
        mc = pace(mc, y)
        out.append(y.astype(BF))
    return _cat(out), rs12


def _ln2_bwd(g, dy, y, rs12, home, k=1.0 + LN_EPS, keep=True, fast=False):
    st, ld_t, ld_y = home
    a1 = a2 = None
    y = y.astype(F32)
    cr, pace = (FCR, _nop) if fast else (CR, _pace)
    for c in range(D // cr):
        d = _ch(dy, c, cr)
        t = d * _ch(y, c, cr)
        a1 = d if a1 is None else a1 + d
        a2 = t if a2 is None else a2 + t
    t = g + dy * rs12
    if ld_t is None:
        ld_t, ld_y = (lambda r: t[r]), (lambda r: y[r])
    else:
        st(slice(0, D), t)
    a = _fold(a1) * rs12
    b = _fold(a2) * (k * rs12)
    out = []
    for c in _PO:
        r = slice(PR * c, PR * c + PR)
        o = (ld_t(r) - ld_y(r).astype(F32) * b) - a
        b = pace(b, o)
        if keep:
            st(r, o)
        out.append(o.astype(BF))
    return _cat(out)


def _lnp(x, link=None, ld=None, fast=False):
    cr, pace = (FCR, _nop) if fast else (CR, _pace)
    acc = _ch(x, 0, cr)
    if link is not None:
        acc = acc + 0.0 * link
    for c in range(1, D // cr):
        acc = acc + _ch(x, c, cr)
    m = _fold(acc)
    a2 = None
    if ld is not None:
        x = ld(0)
    for c in range(D // cr):
        xc = _ch(x, c, cr) - m
        a2 = xc * xc if a2 is None else a2 + xc * xc
    rs = lax.rsqrt(_fold(a2) + LN_EPS)
    mc = _pace(m, rs)
    out = []
    if ld is not None:
        x = ld(1)
    for c in _PO:
        y = (x[PR * c:PR * c + PR] - mc) * rs
        mc = pace(mc, y)
        out.append(y.astype(BF))
    return _cat(out), rs, jnp.minimum(jnp.abs(y[0:1]), 1.0)


def _headsum(x):
    n = x.shape[1]
    p = x.reshape(DH, H, n)
    p = p[0:9] + p[9:18]
    q = (p[0] + p[1]) + (p[2] + p[3])
    r = (p[4] + p[5]) + (p[6] + p[7])
    return (q + r) + p[8]


def _headmul(x, c):
    n = x.shape[1]
    return (x.reshape(DH, H, n) * c[None]).reshape(D, n)


_LT = ((0, 128), (128, 128), (256, 128), (384, 128), (512, 64))


def _to_perm(scr, val, c0=0, c1=5):
    lt = [(c, o - 128 * c0, w) for c, (o, w) in enumerate(_LT)][c0:c1]
    for c, o, w in lt:
        scr[c, :, 0:w] = val[:, o:o + w]
    return jnp.concatenate(
        [jnp.concatenate([scr[c, pl.ds(j, H, stride=DH), 0:w] for c, o, w in lt], axis=1)
         for j in range(DH)], axis=0)


def _from_perm(scr, val):
    for j in range(DH):
        for c, (o, w) in enumerate(_LT):
            scr[c, pl.ds(j, H, stride=DH), 0:w] = val[H * j:H * j + H, o:o + w]
    return jnp.concatenate([scr[c, :, 0:w] for c, (o, w) in enumerate(_LT)], axis=1)


class _Pk:
    def __init__(self, ref):
        self.ref = ref

    def _idx(self, idx):
        nd = len(self.ref.shape)
        if idx is Ellipsis:
            return idx
        if not isinstance(idx, tuple):
            idx = (idx,)
        idx = list(idx) + [slice(None)] * (nd - len(idx))
        r = idx[nd - 2]
        if isinstance(r, slice):
            if r.start is not None or r.stop is not None:
                r = slice(r.start // 2, r.stop // 2)
        elif isinstance(r.start, int):
            r = pl.ds(r.start // 2, r.size // 2)
        else:
            r = pl.ds(pl.multiple_of(r.start // 2, 8), r.size // 2)
        idx[nd - 2] = r
        return tuple(idx)

    def __getitem__(self, idx):
        return pltpu.bitcast(self.ref[self._idx(idx)], BF)

    def __setitem__(self, idx, val):
        self.ref[self._idx(idx)] = pltpu.bitcast(val, U32)


class _L2:
    def __init__(self, a, b):
        self.r = (a, b)

    def __getitem__(self, idx):
        return self.r[idx[0]][idx[1:]]

    def __setitem__(self, idx, val):
        self.r[idx[0]][idx[1:]] = val


def _aug(y):
    r = lax.broadcasted_iota(jnp.int32, (DA - D, y.shape[1]), 0)
    return jnp.concatenate([y.astype(BF), jnp.where(r < 2, 1.0, 0.0).astype(BF)], axis=0)


def _phi(t):
    return jnp.where(t > 0, t + 1.0, jnp.exp(t)) + PHI_EPS


def _dphi_from_phi(p):
    return jnp.minimum(p - PHI_EPS, 1.0)


def _win(x, g):
    return x[WSTEP * g:WSTEP * g + 128]


def _assemble(parts):
    pieces = [parts[0][:WSTEP]]
    for g in range(NG - 1):
        pieces.append(parts[g][WSTEP:128] + parts[g + 1][0:16])
        pieces.append(parts[g + 1][16:WSTEP] if g + 1 < NG - 1 else parts[g + 1][16:128])
    return jnp.concatenate(pieces, axis=0)


def _head_mask(g):
    r = lax.broadcasted_iota(jnp.int32, (128, 128), 0) + WSTEP * g
    c = lax.broadcasted_iota(jnp.int32, (128, 128), 1) + WSTEP * g
    hr = (r * 3641) >> 16
    hc = (c * 3641) >> 16
    return (hr == hc) & (hr >= HEAD_LO[g]) & (hr <= HEAD_HI[g])


def _gelu_parts(pre):
    x2 = pre * pre
    t = jnp.tanh(pre * (GC0 + (GC0 * GC1) * x2))
    hp = 0.5 + 0.5 * t
    return x2, t, hp


def _cols(s, n):
    if isinstance(s, int):
        return pl.ds(s * n, n)
    return pl.ds(pl.multiple_of(s * n, n), n)


def _kernel(
    x_hbm, wqkv_hbm, wo_hbm, w1_hbm, b1_hbm, w2_hbm, b2_hbm, g_hbm,
    out_hbm, dx_hbm, dwqkv_hbm, dwo_hbm, dw1_hbm, db1_hbm, dw2_hbm, db2_hbm,
    xs, gs, wraw, wx, wT, wo, w1c, w1T, w2c, w2T, b1v, b2v, b2col,
    dw1a, dw2Ta, pre2, stream, u_0, u_1, qk_0, qk_1, rd_0, rd_1, y2_s, y4_s, stat, db1a, dbrow,
    oacc, dyacc, hcar, gcar,
    kvT, cacc, ctb, zb, mm, mmT, pacc, dctb, dwv_a, dwo_a, db2a, ps0, ps1, dtmp, zs,
    sem_in, sem_out,
):
    wx, wT, w1T, w2c, pre2, hcar, kvT, ctb, mm, mmT, dctb = [
        _Pk(r) for r in (wx, wT, w1T, w2c, pre2, hcar, kvT, ctb, mm, mmT, dctb)]
    u_s = _L2(_Pk(u_0), _Pk(u_1))
    qk_s = _L2(_Pk(qk_0), _Pk(qk_1))
    rd_s = _L2(rd_0, rd_1)
    y4_s, gcar = _Pk(y4_s), _Pk(gcar)

    ALLR = (0, 1, 2, 3, 4)
    env = {'r': ALLR}

    def zero(k):
        if k not in env['r']:
            return 0
        return env['z'] >> (20 + k)

    def _alt(cs, k):
        if k not in env['r']:
            return cs
        return pl.ds(pl.multiple_of(cs.start + (zero(k) << 7), 128), cs.size)

    def home(cs, yref, ys=None):
        def st(r, v):
            stream[r, cs] = v
        if 3 not in env['r']:
            return st, None, None
        return st, (lambda r: stream[r, _alt(cs, 3)]), (lambda r: yref[r, _alt(ys or cs, 3)])

    zs[0] = 0

    def cp_x(s):
        return pltpu.make_async_copy(x_hbm.at[0, :, _cols(s, TB)], xs.at[:, _cols(s, TB)], sem_in.at[s])

    k0 = NB
    def cp_wpart(lo, hi, k):
        return pltpu.make_async_copy(wqkv_hbm.at[:, pl.ds(lo, hi - lo)], wraw.at[:, pl.ds(lo, hi - lo)], sem_in.at[k])

    def cp_wk(lo, hi, k):
        w = (pl.ds(lo, hi - lo), pl.ds(512, D2 - 512))
        return pltpu.make_async_copy(wqkv_hbm.at[w], wraw.at[w], sem_in.at[k])

    cp_wka = cp_wk(0, 256, k0)
    cp_wkb = cp_wk(256, D, k0 + 11)
    cp_wq = cp_wpart(0, 512, k0 + 9)
    cp_wv = cp_wpart(D2, D3, k0 + 10)
    cp_wo = pltpu.make_async_copy(wo_hbm, wo, sem_in.at[k0 + 1])
    cp_b1 = pltpu.make_async_copy(b1_hbm, b1v, sem_in.at[k0 + 2])
    cp_b2 = pltpu.make_async_copy(b2_hbm, b2v, sem_in.at[k0 + 3])
    cp_w2 = pltpu.make_async_copy(w2_hbm.at[:, pl.ds(0, FQ)], w2T.at[:, pl.ds(0, FQ)], sem_in.at[k0 + 4])
    cp_w2b = pltpu.make_async_copy(w2_hbm.at[:, pl.ds(FQ, F - FQ)], w2T.at[:, pl.ds(FQ, F - FQ)], sem_in.at[k0 + 12])
    cp_g = pltpu.make_async_copy(g_hbm.at[0], gs, sem_in.at[k0 + 5])
    k1 = k0 + 6

    def cp_w1(c):
        return pltpu.make_async_copy(w1_hbm.at[:, _cols(c, W1C)], w1c.at[pl.ds(0, D), _cols(c, W1C)],
                                     sem_in.at[k1 + c])

    cp_x(0).start()
    cp_wka.start()
    cp_wkb.start()
    cp_wq.start()
    cp_x(1).start()
    cp_b1.start()
    cp_b2.start()
    cp_wv.start()
    cp_x(2).start()
    cp_x(3).start()
    for s in range(3):
        cp_w1(s).start()
    cp_wo.start()
    cp_w2.start()
    cp_w2b.start()

    def wrow(ref, g, base=0):
        return ref[base + WSTEP * g:base + WSTEP * g + 128, :]

    def front_a(l, cs, x, link=None, fast=False):
        u, rs, lk = _lnp(x, link, (lambda k: stream[:, _alt(cs, k)]) if l == 1 else None, fast)
        ub = _aug(u)
        u_s[l, :, cs] = ub
        stat[l:l + 1, cs] = rs
        return ub if link is None else lk

    def front_k(l, cs, ub):
        pkb = _phi(_dot5(wT[D:D2, :], ub[0:D], True)).astype(BF)
        qk_s[l, D2:D3, cs] = pkb
        return pkb

    def front_q(l, cs, ub):
        qk_s[l, 0:D, cs] = _phi(_dot5(wT[0:D, :], ub[0:D], True)).astype(BF)

    def front_b(l, cs, ub):
        pkb = front_k(l, cs, ub)
        front_q(l, cs, ub)
        return pkb

    def front_c(pkb, ub, first=False):
        if pkb.shape[1] == T:
            for m in range(4):
                dwv_a[144 * m:144 * m + 144, 512:DA] += _dot_nt(pkb[144 * m:144 * m + 144], ub[512:DA])
            dwv_a[:, 0:512] += _dot_nt(pkb, ub[0:512])
            return
        c = _dot_nt(pkb, ub)
        if first:
            dw1a[:, 0:DA] = c
        else:
            dw1a[:, 0:DA] += c

    def ff_a(l):
        c = dwv_a[...] if l else dw1a[:, 0:DA]
        zb[l] = jnp.broadcast_to(c[:, D:D + 1], (D, 128))
        ct = _from_perm(ps0, c[:, 0:D]).astype(BF)
        ctb[l] = ct
        return ct

    def ff_b(l, ct):
        kvs = []
        for g in range(NG):
            kv = jnp.where(_head_mask(g), _dot_nt(_win(ct, g), wrow(wT, g, D2)), 0.0)
            kvT[l, g] = kv.T.astype(BF)
            kvs.append(kv.astype(BF))
        return kvs

    def ff_c(l, kvs):
        m = _assemble([_dot(kvs[g], wrow(wo, g)) for g in range(NG)])
        mp = _to_perm(ps1, m).astype(BF)
        mm[l] = mp
        mmT[...] = mp.T

    def back_a(l, cs):
        pq = qk_s[l, 0:D, cs].astype(F32)
        rden = 1.0 / (_headsum(pq * zb[l]) + PHI_EPS)
        rd_s[l, :, cs] = rden
        return _headmul(pq, rden).astype(BF)

    def back_b(x, cs, pqn, split=False, fast=False):
        x1 = x + _dot5(mmT[...], pqn, split)
        env['x'] = x1
        if 0 in env['r']:
            stream[:, cs] = x1
            y, rs12 = _ln2(x1, lambda k: stream[:, _alt(cs, k)], fast)
        else:
            y, rs12 = _ln2(x1, lambda k: x1, fast)
        return _aug(y), rs12

    def res(cs):
        return (stream[:, _alt(cs, 2)] if 0 in env['r'] else env['x']) + b2col[...]

    def bwd1_a(l, gb, split=False):
        return gb, _dot5(mm[l], gb, split)

    def bwd1_b(l, cs, gb, dpqn, split=False):
        pq = qk_s[l, 0:D, cs].astype(F32)
        rden = rd_s[l, :, cs]
        z = zb[l]
        rd = rden
        r = None
        pqn = []
        rl = 4 in env['r']
        if rl:
            dtmp[0] = dpqn
        for j in range(DH):
            t = pq[H * j:H * j + H] * rd
            pqn.append(t.astype(BF))
            t = dpqn[H * j:H * j + H] * t
            r = t if r is None else r + t
            rd = _pace(rden, r)
        rb = r.astype(BF)
        for j in range(DH):
            rj = slice(H * j, H * j + H)
            w = _dphi_from_phi(qk_s[l, rj, _alt(cs, 4)].astype(F32) if rl else pq[rj]) * rden
            t = ((dtmp[zero(4), rj, :] if rl else dpqn[rj]) - z[rj] * r) * w
            r = _pace(r, t)
            qk_s[l, rj, cs] = t.astype(BF)
        pqn = jnp.concatenate(pqn, axis=0)
        gr = jnp.concatenate([gb, rb], axis=0)
        pa = pacc if l else cacc
        if split:
            pa[:, 0:512] += _dot_nt(pqn, gr[0:512])
            for m in range(4):
                pa[144 * m:144 * m + 144, 512:DR] += _dot_nt(pqn[144 * m:144 * m + 144], gr[512:DR])
        else:
            pa[...] += _dot_nt(pqn, gr)

    def bf_a(l):
        p = (pacc if l else cacc)[...]
        tl = p[:, 512:DR]
        rr = lax.broadcasted_iota(jnp.int32, tl.shape, 0)
        cc = lax.broadcasted_iota(jnp.int32, tl.shape, 1)
        dz = -jnp.sum(jnp.where(cc - (D - 512) == (rr & (H - 1)), tl, 0.0), axis=1, keepdims=True)
        hi = dz.astype(BF).astype(F32)
        ce = lax.broadcasted_iota(jnp.int32, (D, DA - D), 1)
        dctb[:, D:DA] = jnp.where(ce == 0, hi, jnp.where(ce == 1, dz - hi, 0.0)).astype(BF)
        pb = _from_perm(ps0, p[:, 0:D]).astype(BF)
        return pb

    def acc_l(ref, l, val):
        if l == 1:
            ref[:, 0:D] = val
        else:
            ref[:, 0:D] += val

    def bf_b(l, pb):
        ds_ = [jnp.where(_head_mask(g), _dot_nt(_win(pb, g), wrow(wo, g)), 0.0) for g in range(NG)]
        acc_l(dwo_a, l, _assemble([_dot(kvT[l, g], _win(pb, g)) for g in range(NG)]))
        return ds_

    def bf_c(l, ds_):
        dct = _assemble([_dot(ds_[g].astype(BF), wrow(wT, g, D2)) for g in range(NG)])
        dp = _to_perm(ps1, dct).astype(BF)
        dctb[:, 0:D] = dp
        wx[:, D2:D3] = dp.T
        acc_l(dwv_a, l, _assemble([_dot(ds_[g].T.astype(BF), ctb[l, WSTEP * g:WSTEP * g + 128, :]) for g in range(NG)]))

    def bwd2_a(l, cs, split=False):
        dpk = _dot5(dctb[...], u_s[l, :, cs], split)
        dk = (dpk * _dphi_from_phi(qk_s[l, D2:D3, cs].astype(F32))).astype(BF)
        qk_s[l, D:D2, cs] = dk
        return dk

    def bwd2_b(l, cs, dk=None, keep=True, bal=False, fast=False):
        if dk is None:
            rhs = qk_s[l, :, cs]
        else:
            rhs = jnp.concatenate([qk_s[l, 0:D, cs], dk, qk_s[l, D2:D3, cs]], axis=0)
        du = _dot5(wx[...], rhs, bal)
        return _ln2_bwd(stream[:, cs], du, u_s[l, 0:D, cs], stat[l:l + 1, cs], home(cs, u_s.r[l]), 1.0, keep, fast)

    def hs(h):
        return pl.ds(h * FH, FH)

    def qs(c):
        return pl.ds(c * FQ, FQ)

    def f_pre(y, cs, c):
        pre = _dot5(w1T[qs(c), :], y, True)
        pre2[qs(c), cs] = pre.astype(BF)
        _, _, hp = _gelu_parts(pre)
        return (pre * hp).astype(BF)

    def f_out(hh, c):
        return _dot5(w2T[:, qs(c)], hh, True, True)

    def gelu_bwd(pre):
        x2, t, hp = _gelu_parts(pre)
        hh = (pre * hp).astype(BF)
        gp = hp + (0.5 * pre) * (1.0 - t * t) * (GC0 + (3.0 * GC0 * GC1) * x2)
        return hh, gp

    def gelu_bwd_p(h, cs):
        GR = 64
        hs_, gs_ = [], []
        k = jnp.full((1, T), GC0, F32)
        for c in range(FH // GR):
            pre = pre2[h * FH + c * GR:h * FH + (c + 1) * GR, cs].astype(F32)
            x2 = pre * pre
            t = jnp.tanh(pre * (k + (GC0 * GC1) * x2))
            k = _pace(k, t)
            hp = 0.5 + 0.5 * t
            hs_.append((pre * hp).astype(BF))
            gs_.append(hp + (0.5 * pre) * (1.0 - t * t) * (GC0 + (3.0 * GC0 * GC1) * x2))
        return jnp.concatenate(hs_, axis=0), jnp.concatenate(gs_, axis=0)

    def m_dh(gb, h):
        return _dot5(w2c[hs(h), :], gb, True)

    def m_pre(y, h):
        return _dot5(w1T[hs(h), :], y, True)

    def m_dy(dpre, h, bal=False):
        return _dot5(w1c[0:D, hs(h)], dpre, bal, True)

    def m_out(hh, h):
        return _dot(w2T[:, hs(h)], hh)

    def acc_to(ref, sl, val, keep):
        if keep is True:
            ref[:, sl] += val
        elif keep is False:
            ref[:, sl] = val
        else:
            ref[:, sl] = jnp.where(keep, ref[:, sl], 0.0) + val

    def m_w1(y, dpre, h, keep=True):
        acc_to(dw1a, hs(h), _dot_nt(y[0:D], dpre), keep)

    def mk_dpre(dh, gp, h):
        dp = dh * gp
        db1a[hs(h), :] += dp
        return dp.astype(BF)

    def m_w2(gb, hh, h, keep=True):
        acc_to(dw2Ta, hs(h), _dot_nt(gb, hh), keep)

    def m_wq(ref, a, b, c):
        acc_to(ref, qs(c), _dot5_nt(a, b[(c - 2) * FQ:(c - 1) * FQ]), True)

    def m_fin(dst, ref, a, b, sl):
        val = ref[:, sl] + _dot_nt(a, b)
        dst[0:D, sl] = val.astype(BF)

    def m_wq_fin(dst, ref, a, b, c):
        m_fin(dst, ref, a, b[(c - 2) * FQ:(c - 1) * FQ], qs(c))

    def clear(i, carry):
        r = pl.ds(pl.multiple_of(i * 32, 32), 32)
        for ref in (pacc, dwv_a, cacc, db2a):
            ref[r, :] = jnp.zeros((32, ref.shape[1]), F32)
        db1a[pl.ds(pl.multiple_of(i * 256, 256), 256), :] = jnp.zeros((256, T), F32)
        return carry

    lax.fori_loop(0, D // 32, clear, 1)

    def ln0(s, chain=4, lk=None, ks=(0, 1, 2, 3), fast=False):
        for k in ks:
            cs = pl.ds(s * TB + k * T, T)
            if k % chain == 0 and (k or lk is None):
                lk = jnp.zeros((1, T), F32)
            lk = front_a(0, cs, xs[:, cs].astype(F32), lk, fast)
        return lk

    def k_part(s):
        cs = _cols(s, TB)
        qk_s[0, D2:D3, cs] = _phi(_dot(wT[D:D2, :], u_s[0, 0:D, cs])).astype(BF)

    def q_part(lo, hi):
        cs = pl.ds(lo * T, (hi - lo) * T)
        qk_s[0, 0:D, cs] = _phi(_dot(wT[0:D, :], u_s[0, 0:D, cs])).astype(BF)

    def c_part(s):
        cs = _cols(s, TB)
        front_c(qk_s[0, D2:D3, cs], u_s[0, :, cs], s == 0)

    def w1_t(c):
        w1T[_cols(c, W1C), :] = w1c[:, _cols(c, W1C)].T

    cp_x(0).wait()
    ln0(0, 4, None, (0, 1, 2), True)
    cp_wka.wait()
    wta = wraw[0:256, 512:D2].T
    wT[D:D2, 0:256] = _to_perm(ps1, wta[64:640].astype(F32), 0, 2).astype(BF)
    ln0(0, 1, None, (3,), True)
    stream[:, 0:TB] = _dot(wT[D:D2, 0:128], u_s[0, 0:128, 0:TB])
    cp_wkb.wait()
    wtb = wraw[256:D, 512:D2].T
    wT[D:D2, 256:D] = _to_perm(ps1, wtb[64:640].astype(F32), 2, 5).astype(BF)
    qk_s[0, D2:D3, 0:TB] = _phi(
        stream[:, 0:TB] + _dot(wT[D:D2, 128:256], u_s[0, 128:256, 0:TB])
        + _dot(wT[D:D2, 256:D], u_s[0, 256:D, 0:TB])).astype(BF)
    wtk = jnp.concatenate([wta[0:64], wtb[0:64]], axis=1)
    dw1a[:, 0:256] = _dot_nt(qk_s[0, D2:D3, 0:TB], u_s[0, 0:256, 0:TB])
    cp_wq.wait()
    cp_x(1).wait()
    cp_b1.wait()
    cp_b2.wait()
    wtq = jnp.concatenate([wraw[:, 0:512].T, wtk[0:64]], axis=0)
    wT[0:D, :] = _to_perm(ps0, wtq.astype(F32)).astype(BF)
    dw1a[:, 256:DA] = _dot_nt(qk_s[0, D2:D3, 0:TB], u_s[0, 256:DA, 0:TB])
    b2col[...] = jnp.broadcast_to(b2v[...].reshape(1, D).astype(F32), (128, D)).T
    rid = lax.broadcasted_iota(jnp.int32, (DA - D, F), 0)
    w1c[D:DA, :] = jnp.where(
        rid == 0, jnp.broadcast_to(b1v[...].reshape(1, F).astype(F32), (DA - D, F)), 0.0).astype(BF)
    ln0(1)
    q_part(0, 4)
    k_part(1)
    for t_ in (4, 5):
        front_q(0, _cols(t_, T), u_s[0, :, _cols(t_, T)])
    c_part(1)
    cp_wv.wait()
    cp_x(2).wait()
    cp_x(3).wait()
    cp_w1(0).wait()
    cp_w1(1).wait()
    lk = ln0(2)
    for t_ in (6, 7):
        front_q(0, _cols(t_, T), u_s[0, :, _cols(t_, T)])
    wT[D2:D3, :] = wraw[:, D2:D3].T
    w1_t(0)
    ln0(3, 4, lk)
    k_part(2)
    c_part(2)
    w1_t(1)
    k_part(3)
    q_part(8, 12)
    c_part(3)
    cp_w1(2).wait()
    cp_wo.wait()
    cp_w2.wait()

    def step_2(s, first=False, last=False):
        cs = _cols(s, T)
        cn = _cols(s + 1, T)
        pqn = back_a(0, cn)
        if not first:
            o = oacc[...] + f_out(hcar[...], 1)
        yn, rs12 = back_b(xs[:, cn].astype(F32), cn, pqn, True)
        if first:
            q_part(15, 16)
        else:
            y = y2_s[:, cs]
            h2 = f_pre(y, cs, 2)
            h3 = f_pre(y, cs, 3)
            o = o + f_out(h2, 2)
        y2_s[:, cn] = yn
        stat[2:3, cn] = rs12
        h0n = f_pre(yn, cn, 0)
        if not first:
            x2 = o + f_out(h3, 3)
            stream[:, cs] = x2
            ub = front_a(1, cs, x2)
        hcar[...] = f_pre(yn, cn, 1)
        if last:
            pkb = front_k(1, cs, ub)
        oacc[...] = res(cn) + f_out(h0n, 0)
        if last:
            front_c(pkb, ub)
        elif not first:
            front_c(front_b(1, cs, ub), ub)

    env['z'] = zs[0]
    if on('b1'):
        ct = ff_a(0)
        q_part(12, 13)
        ff_c(0, ff_b(0, ct))
        q_part(13, 15)
        w1_t(2)
        step_2(-1, first=True)

    def p2(s, carry):
        env['z'] = s
        for s2 in (2 * s, 2 * s + 1):
            j = pl.ds(pl.multiple_of(jnp.minimum(s2, 11) * 384, 384), 384)
            w2c[j, :] = w2T[:, j].T
            step_2(s2)
        return s

    cp_w2b.wait()
    cp_g.start()
    if on('p2'):
        env['z'] = \
            lax.fori_loop(0, NT_ // 2 - 1, p2, 0)

    cp_g.wait()
    cl = _cols(NT_ - 1, T)
    c0 = _cols(0, T)
    if on('b2'):
        step_2(NT_ - 2, last=True)
        cp_ = _cols(NT_ - 2, T)
        y = y2_s[:, cl]
        gn = gs[:, c0]
        h2 = f_pre(y, cl, 2)
        o = oacc[...] + f_out(hcar[...], 1)
        h3 = f_pre(y, cl, 3)
        o = o + f_out(h2, 2)
        x2 = o + f_out(h3, 3)
        stream[:, cl] = x2
        ub = front_a(1, cl, x2, None, True)
        FE = FH // 8
        dhe = []

        def fill_dh(n):
            e = len(dhe)
            for i in range(e, e + n):
                dhe.append(_dot(w2c[i * FE:(i + 1) * FE, 0:512], gn[0:512]))

        front_q(1, cp_, u_s[1, :, cp_])
        fill_dh(1)
        pkb = front_k(1, cl, ub)
        fill_dh(1)
        front_c(pkb, ub)
        ct = ff_a(1)
        front_q(1, cl, ub)
        kvs = ff_b(1, ct)
        fill_dh(1)
        ff_c(1, kvs)
        dht = jnp.concatenate([_dot(w2c[r, 512:D], gn[512:D]) for r in _rows(FH, 1)], axis=0)
        fill_dh(1)
        yn, rs12 = back_b(stream[:, c0], c0, back_a(1, c0), True, True)
        y4_s[:, c0] = yn
        gcar[...] = gn
        stat[3:4, c0] = rs12
        fill_dh(4)
        hn, gpn = gelu_bwd(m_pre(yn, 0))
        dpren = mk_dpre(jnp.concatenate(dhe, axis=0) + dht, gpn, 0)
        oacc[...] = res(c0) + m_out(hn, 0)
        dyacc[...] = m_dy(dpren, 0)
        m_w1(yn, dpren, 0, False)
        m_w2(gn, hn, 0, False)

    def p3(s, carry):
        env['z'] = s
        env['r'] = R3
        j = pl.ds(pl.multiple_of(jnp.minimum(s, 8) * 128, 128), 128)
        wx[:, j] = wT[j, :].T
        cs = _cols(s, T)
        cn = _cols(s + 1, T)
        gb = gcar[...]
        gn = gs[:, cn]
        pqn = back_a(1, cn)
        dh = m_dh(gb, 1)
        yn, rs12 = back_b(stream[:, cn], cn, pqn, True)
        hh, gp = gelu_bwd(m_pre(y4_s[:, c0], 1))
        stat[3:4, cn] = rs12
        dpre = mk_dpre(dh, gp, 1)
        dy = dyacc[...] + m_dy(dpre, 1)
        g = gb.astype(F32)
        db2a[...] += g
        g3 = _ln2_bwd(g, dy, y4_s[0:D, c0], stat[3:4, cs], home(cs, y4_s, c0))
        xs[:, cs] = (oacc[...] + m_out(hh, 1)).astype(BF)
        m_w1(y4_s[0:D, c0], dpre, 1, s > 0)
        m_w2(gb, hh, 1, s > 0)
        y4_s[:, c0] = yn
        gcar[...] = gn
        dhn = m_dh(gn, 0)
        g3b, dpqn = bwd1_a(1, g3, True)
        hn, gpn = gelu_bwd(m_pre(yn, 0))
        dpren = mk_dpre(dhn, gpn, 0)
        bwd1_b(1, cs, g3b, dpqn, True)
        dyacc[...] = m_dy(dpren, 0)
        oacc[...] = res(cn) + m_out(hn, 0)
        m_w1(yn, dpren, 0)
        m_w2(gn, hn, 0)
        env['r'] = ALLR
        return s

    if on('p3'):
        env['z'] = \
            lax.fori_loop(0, NT_ - 1, p3, 0)

    cp_out = pltpu.make_async_copy(xs, out_hbm.at[0], sem_out.at[0])
    if on('b3'):
        gb = gcar[...]
        y = y4_s[:, c0]
        hh, gp = gelu_bwd(m_pre(y, 1))
        dh = m_dh(gb, 1)
        dpre = mk_dpre(dh, gp, 1)
        dy = dyacc[...] + m_dy(dpre, 1, True)
        g = gb.astype(F32)
        db2a[...] += g
        g3 = _ln2_bwd(g, dy, y[0:D], stat[3:4, cl], home(cl, y4_s, c0), fast=True)
        o = oacc[...] + f_out(hh[0:FQ], 2)
        g3b, dpqn = bwd1_a(1, g3, True)
        m_wq(dw1a, y[0:D], dpre, 2)
        bwd1_b(1, cl, g3b, dpqn, True)
        pb = bf_a(1)
        m_wq(dw1a, y[0:D], dpre, 3)
        bf_c(1, bf_b(1, pb))
        m_wq(dw2Ta, gb, hh, 2)
        dk = bwd2_a(1, c0, True)
        m_wq(dw2Ta, gb, hh, 3)
        gn = bwd2_b(1, c0, dk, True, True, True)
        pacc[:, 0:512] = _dot_nt(u_s[1, 0:D, 0:T], qk_s[1, 0:512, 0:T])
        xs[:, cl] = (o + f_out(hh[FQ:FH], 3)).astype(BF)
        gcar[...] = gn
        hn, gpn = gelu_bwd(pre2[hs(0), c0].astype(F32))
        dhn = m_dh(gn, 0)
        dpren = mk_dpre(dhn, gpn, 0)
        m_w2(gn, hn, 0)
        yn = y2_s[0:D, c0]
        y4_s[0:D, c0] = yn
        m_w1(yn, dpren, 0)
        dyacc[...] = m_dy(dpren, 0, True)
    cp_out.start()

    def p4(s, carry, last=False):
        if not last:
            env['z'] = s
            env['r'] = R4
        cs = _cols(s, T)
        cn = _cols(s + 1, T)
        dk = bwd2_a(1, cn, True)
        gb = gcar[...]
        dh = m_dh(gb, 1)
        db2a[...] += gb.astype(F32)
        gn = bwd2_b(1, cn, dk)
        hh, gp = gelu_bwd_p(1, cs)
        dpre = mk_dpre(dh, gp, 1)
        m_w2(gb, hh, 1)
        gcar[...] = gn
        y = y4_s[0:D, c0]
        dy = dyacc[...] + m_dy(dpre, 1)
        g1 = _ln2_bwd(stream[:, cs], dy, y, stat[2:3, cs], home(cs, y4_s, c0))
        m_w1(y, dpre, 1)
        dhn = m_dh(gn, 0)
        hn, gpn = gelu_bwd_p(0, cn)
        dpren = mk_dpre(dhn, gpn, 0)
        g1b, dpqn = bwd1_a(0, g1)
        if last:
            m_fin(w2T, dw2Ta, gn, hn, hs(0))
        else:
            m_w2(gn, hn, 0)
        bwd1_b(0, cs, g1b, dpqn)
        dyacc[...] = m_dy(dpren, 0)
        yn = y2_s[0:D, cn]
        y4_s[0:D, c0] = yn
        if last:
            m_fin(w1c, dw1a, yn, dpren, hs(0))
        else:
            m_w1(yn, dpren, 0)
        env['r'] = ALLR
        return s

    if on('p4'):
        env['z'] = \
            lax.fori_loop(0, NT_ - 2, p4, 0)

    if on('b4'):
        p4(NT_ - 2, 0, True)
        gb = gcar[...]
        y = y4_s[0:D, c0]
        db2a[...] += gb.astype(F32)
        dh = m_dh(gb, 1)
        hh, gp = gelu_bwd(pre2[hs(1), cl].astype(F32))
        dpre = mk_dpre(dh, gp, 1)
        m_wq_fin(w2T, dw2Ta, gb, hh, 2)
        dy = dyacc[...] + m_dy(dpre, 1)
        g1 = _ln2_bwd(stream[:, cl], dy, y[0:D], stat[2:3, cl], home(cl, y4_s, c0), fast=True)
        m_wq_fin(w2T, dw2Ta, gb, hh, 3)
        g1b, dpqn = bwd1_a(0, g1)
        m_wq_fin(w1c, dw1a, y[0:D], dpre, 2)
        bwd1_b(0, cl, g1b, dpqn)
        pb = bf_a(0)
        m_wq_fin(w1c, dw1a, y[0:D], dpre, 3)
        bf_c(0, bf_b(0, pb))
        dw2Ta[:, 0:512] = pacc[:, 0:512] + _dot_nt(u_s[1, 0:D, T:TB], qk_s[1, 0:512, T:TB])
        dw2Ta[:, 512:D2] = _dot_nt(u_s[1, 0:D, 0:TB], qk_s[1, 512:D2, 0:TB])
        b2v[...] = jnp.sum(db2a[...].T, axis=0, keepdims=True).astype(BF).reshape(D)
        wo[...] = dwo_a[...].astype(BF)
    cp_dw1a = pltpu.make_async_copy(w1c.at[pl.ds(0, D), :], dw1_hbm, sem_out.at[1])
    cp_dw2a = pltpu.make_async_copy(w2T, dw2_hbm, sem_out.at[2])
    cp_db1 = pltpu.make_async_copy(b1v, db1_hbm, sem_out.at[3])
    cp_db2 = pltpu.make_async_copy(b2v, db2_hbm, sem_out.at[4])
    cp_dwo = pltpu.make_async_copy(wo, dwo_hbm, sem_out.at[5])
    cp_dwqkv = pltpu.make_async_copy(wraw, dwqkv_hbm, sem_out.at[6])
    cp_dw1a.start()
    cp_dw2a.start()
    cp_db2.start()
    cp_dwo.start()
    o3 = 7

    def cp_dx(s):
        if isinstance(s, int):
            lo, hi = max(s * TB - T, 0), min(s * TB + TB - T, S)
            w = pl.ds(lo, hi - lo)
        else:
            w = pl.ds(pl.multiple_of(s * TB - T, T), TB)
        return pltpu.make_async_copy(gs.at[:, w], dx_hbm.at[0, :, w], sem_out.at[o3 + s])

    def p5a(s, carry):
        cs = pl.ds(pl.multiple_of(s * 640, 128), 640)
        ks = pl.ds(pl.multiple_of(TB + s * 768, 128), 768)
        dbrow[0:1, _cols(s, FH)] = jnp.sum(db1a[_cols(s, FH), :].T, axis=0, keepdims=True)
        pre2[0:D, 640:1408] = u_s[1, 0:D, ks]
        pre2[0:D, 0:640] = u_s[0, 0:D, cs]
        dk = bwd2_a(0, cs)
        dw2Ta[:, 0:D2] += _dot_nt(pre2[0:D, 640:1408], qk_s[1, 0:D2, ks])
        dw2Ta[:, 0:D2] += _dot_nt(pre2[0:D, 0:640], jnp.concatenate([qk_s[0, 0:D, cs], dk], axis=0))
        return carry

    if on('p5a'):
        lax.fori_loop(0, 2, p5a, 0)

    def sub(s, k):
        if isinstance(s, int):
            return pl.ds(s * TB + k * T, T)
        return pl.ds(pl.multiple_of(s * TB + k * T, T), T)

    def dx_fin(cs, du, fast=False):
        gs[:, cs] = _ln2_bwd(stream[:, cs], du, u_s[0, 0:D, cs], stat[0:1, cs], home(cs, u_s.r[0]), 1.0, False, fast)

    def dx_tile(s, first=False):
        if not first:
            dx_fin(sub(s, -1), dyacc[...])
        for k in range(1 if first else 0, TB // T - 1):
            dx_fin(sub(s, k), _dot(wx[...], qk_s[0, :, sub(s, k)]))
        dyacc[...] = _dot(wx[...], qk_s[0, :, sub(s, TB // T - 1)])
        cp_dx(s).start()

    env['r'] = ()
    if on('b5'):
        c2 = pl.ds(S - 6 * T, 6 * T)
        dk = bwd2_a(0, c2)
        dx_fin(c0, _dot(wx[...], qk_s[0, :, c0]))
        dwt = dw2Ta[:, 0:D2] + _dot_nt(u_s[0, 0:D, c2], jnp.concatenate([qk_s[0, 0:D, c2], dk], axis=0))
        dwt = dwt.astype(BF).T.astype(F32)
        dwq = _from_perm(ps0, dwt[0:D]).astype(BF)
        dwk = _from_perm(ps1, dwt[D:D2]).astype(BF)
        wraw[...] = jnp.concatenate([dwq, dwk, dwv_a[:, 0:D].astype(BF)], axis=0).T
        b1v[...] = dbrow[0:1, :].astype(BF).reshape(F)
        dx_tile(0, True)
    else:
        cp_dx(0).start()
    cp_dwqkv.start()
    cp_db1.start()

    if on('p5b'):
        for s in range(1, NB):
            dx_tile(s)
        env['r'] = ALLR
        dx_fin(cl, dyacc[...], True)
    else:
        for s in range(1, NB):
            cp_dx(s).start()
    cp_dx(NB).start()

    cp_out.wait()
    cp_dw1a.wait()
    cp_dw2a.wait()
    cp_db1.wait()
    cp_db2.wait()
    cp_dwo.wait()
    cp_dwqkv.wait()
    for s in range(NB + 1):
        cp_dx(s).wait()


@jax.jit
def pallas_interleave_layers__linear_attn_block__mixer_channel_mlp__prompt_kernel(
    A_x: jax.Array,
    A_wqkv: jax.Array,
    A_wo: jax.Array,
    B_x: jax.Array,
    B_w1: jax.Array,
    B_b1: jax.Array,
    B_w2: jax.Array,
    B_b2: jax.Array,
    grad_out: jax.Array,
):
    del B_x
    V = pltpu.VMEM
    n_in = NB + 6 + 3 + 4
    n_out = 7 + NB + 1
    scratch = [
        V((D, S), BF),
        V((D, S), BF),
        V((D, D3), BF),
        V((D // 2, D3), U32),
        V((D3 // 2, D), U32),
        V((D, D), BF),
        V((DA, F), BF),
        V((F // 2, DA), U32),
        V((F // 2, D), U32),
        V((D, F), BF),
        V((F,), BF),
        V((D,), BF),
        V((D, 128), F32),
        V((D, F), F32),
        V((D, F), F32),
        V((F // 2, S), U32),
        V((D, S), F32),
        V((DA // 2, S), U32),
        V((DA // 2, S), U32),
        V((D3 // 2, S), U32),
        V((D3 // 2, S), U32),
        V((H, S), F32),
        V((H, S), F32),
        V((DA, S), BF),
        V((DA // 2, 2 * T), U32),
        V((8, S), F32),
        V((F, T), F32),
        V((8, F), F32),
        V((D, T), F32),
        V((D, T), F32),
        V((FQ // 2, T), U32),
        V((D // 2, T), U32),
        V((2, NG, 64, 128), U32),
        V((D, DR), F32),
        V((2, D // 2, D), U32),
        V((2, D, 128), F32),
        V((2, D // 2, D), U32),
        V((D // 2, D), U32),
        V((D, DR), F32),
        V((D // 2, DA), U32),
        V((D, DA), F32),
        V((D, D), F32),
        V((D, 128), F32),
        V((5, D, 128), F32),
        V((5, D, 128), F32),
        V((2, D, T), F32),
        pltpu.SMEM((1,), jnp.int32),
        pltpu.SemaphoreType.DMA((n_in,)),
        pltpu.SemaphoreType.DMA((n_out,)),
    ]
    any_spec = pl.BlockSpec(memory_space=pl.ANY)
    out_shape = (
        jax.ShapeDtypeStruct((1, D, S), BF),
        jax.ShapeDtypeStruct((1, D, S), BF),
        jax.ShapeDtypeStruct((D, D3), BF),
        jax.ShapeDtypeStruct((D, D), BF),
        jax.ShapeDtypeStruct((D, F), BF),
        jax.ShapeDtypeStruct((F,), BF),
        jax.ShapeDtypeStruct((D, F), BF),
        jax.ShapeDtypeStruct((D,), BF),
    )
    outT, dxT, dwqkv, dwo, dw1, db1, dw2T, db2 = pl.pallas_call(
        _kernel,
        out_shape=out_shape,
        in_specs=[any_spec] * 8,
        out_specs=tuple([any_spec] * 8),
        scratch_shapes=scratch,
        compiler_params=pltpu.CompilerParams(vmem_limit_bytes=127 * 1024 * 1024),
    )(jnp.swapaxes(A_x, 1, 2), A_wqkv, A_wo, B_w1, B_b1, B_w2.T, B_b2, jnp.swapaxes(grad_out, 1, 2))
    return (jnp.swapaxes(outT, 1, 2), jnp.swapaxes(dxT, 1, 2), dwqkv, dwo, dw1, db1, dw2T.T, db2)
```
